```python
import jax
import jax.numpy as jnp

def _softmax(x, axis=-1):
    return jax.nn.softmax(x, axis=axis)
def _gelu(x):
    return jax.nn.gelu(x, approximate=True)
def _silu(x):
    return jax.nn.silu(x)
def _sigmoid(x):
    return jax.nn.sigmoid(x)
def _layernorm(x, axis=-1, eps=1e-5):
    m = jnp.mean(x, axis=axis, keepdims=True)
    v = jnp.var(x, axis=axis, keepdims=True)
    return (x - m) / jnp.sqrt(v + eps)
def _scatter_add(tgt, idx, src, axis=0):
    return tgt.at[idx].add(src)
def _segment_sum(src, seg, n):
    return jax.ops.segment_sum(src, seg, n)
class _Rng:
    def __init__(self, key):
        self._k = key
    def _next(self):
        self._k, sub = jax.random.split(self._k)
        return sub
    def normal(self, shape):
        return jax.random.normal(self._next(), shape, dtype=jnp.bfloat16)
    def randint(self, lo, hi, shape):
        return jax.random.randint(self._next(), shape, lo, hi, dtype=jnp.int32)
    def uniform(self, shape, lo=0.0, hi=1.0):
        return jax.random.uniform(self._next(), shape, jnp.bfloat16, lo, hi)
    def permutation(self, n):
        return jax.random.permutation(self._next(), n)


kernel_name = 'interleave_layers__sliding_local_dilated__glu_gated_swiglu__prompt'

def setup_inputs():
    _rng = _Rng(jax.random.key(int.from_bytes(__import__("os").urandom(4), "little")))
    _w = (lambda a: (lambda t: t.astype(jnp.bfloat16) if jnp.issubdtype(t.dtype, jnp.floating) else t)(jnp.asarray(a)))
    def _A_setup():
        B, S, D = 1, 2048, 1024
        return {
            "x": _w((lambda *s: _rng.normal(s) * 0.05)(B, S, D)),
            "wqkv": _w((lambda *s: _rng.normal(s) * 0.05)(D, 3 * D)),
            "wo": _w((lambda *s: _rng.normal(s) * 0.05)(D, D)),
        }
    _A_in = _A_setup()

    def _B_setup():
        B, S, D, F = 1, 2048, 1024, 3584
        return {
            "x": _w((lambda *s: _rng.normal(s) * 0.05)(B, S, D)),
            "w1": _w((lambda *s: _rng.normal(s) * 0.05)(D, F) * (2.0 / D) ** 0.5),
            "w3": _w((lambda *s: _rng.normal(s) * 0.05)(D, F) * (2.0 / D) ** 0.5),
            "w2": _w((lambda *s: _rng.normal(s) * 0.05)(F, D) * (2.0 / F) ** 0.5),
        }
    _B_in = _B_setup()

    return {
        "A_x": _A_in["x"],
        "A_wqkv": _A_in["wqkv"],
        "A_wo": _A_in["wo"],
        "B_x": _B_in["x"],
        "B_w1": _B_in["w1"],
        "B_w3": _B_in["w3"],
        "B_w2": _B_in["w2"],
    }

def reference(A_x, A_wqkv, A_wo, B_x, B_w1, B_w3, B_w2):
    def _A_ref(x, wqkv, wo):
        B, S, D = x.shape
        H = 32; Dh = D // H
        W, dil = 8, 2
        qkv = (lambda x, *d: x.transpose(*d))((x @ wqkv).reshape(B, S, 3, H, Dh), 2, 0, 3, 1, 4)
        q, k, v = qkv[0], qkv[1], qkv[2]
        scale = Dh ** -0.5
        pos = jnp.arange(S)
        off = jnp.arange(W) * dil
        idx = pos[:, None] - off[None, :]
        mask = idx >= 0
        idx_c = jnp.where(mask, idx, 0).reshape(-1)
        kg = k[:, :, idx_c, :].reshape(B, H, S, W, Dh)
        vg = v[:, :, idx_c, :].reshape(B, H, S, W, Dh)
        logits = jnp.einsum("bhsd,bhswd->bhsw", q, kg) * scale
        logits = jnp.where(mask[None, None, :, :], logits, -1e9)
        attn = _softmax(logits, axis=-1)
        o = jnp.einsum("bhsw,bhswd->bhsd", attn, vg)
        return (lambda x, *d: x.transpose(*d))(o, 0, 2, 1, 3).reshape(B, S, D) @ wo

    def _B_ref(x, w1, w3, w2):
        gate = jnp.einsum("bsd,df->bsf", x, w1)
        up = jnp.einsum("bsd,df->bsf", x, w3)
        h = _silu(gate) * up
        out = jnp.einsum("bsf,fd->bsd", h, w2)
        return out

    x = A_x
    x = x + _A_ref(_layernorm(x, axis=-1), A_wqkv, A_wo)
    x = x + _B_ref(_layernorm(x, axis=-1), B_w1, B_w3, B_w2)
    x = x + _A_ref(_layernorm(x, axis=-1), A_wqkv, A_wo)
    x = x + _B_ref(_layernorm(x, axis=-1), B_w1, B_w3, B_w2)
    return x
```

```python
import functools
import jax
import jax.numpy as jnp
from jax import lax
import jax.experimental.pallas as pl
import jax.experimental.pallas.tpu as pltpu

S, D, H, DH, WIN, DIL, F = 2048, 1024, 32, 32, 8, 2, 3584
NB = D // 128
SH = 8 * DIL
HALO = (WIN - 1) * SH
f32, bf16 = jnp.float32, jnp.bfloat16


def _dot(a, b):
    return jnp.dot(a, b, preferred_element_type=f32)


def _ln(x):
    m = jnp.mean(x, axis=-1, keepdims=True)
    xc = x - m
    v = jnp.mean(xc * xc, axis=-1, keepdims=True)
    return xc * lax.rsqrt(v + 1e-5)


def _dst(src, i):
    g = (src >> 2) & 7
    return (src & 3) * 32 + (g ^ i) * 4 + (src >> 5)


def _butterfly(blocks, g):
    for b in range(3):
        m = ((g >> b) & 1) == 1
        blocks = [jnp.where(m, blocks[j ^ (1 << b)], blocks[j]) for j in range(NB)]
    return blocks


def _permute_cols(src_ref, dst_ref, j):
    RC = 256
    r = lax.broadcasted_iota(jnp.int32, (128, 128), 0)
    c = lax.broadcasted_iota(jnp.int32, (128, 128), 1)
    g = (lax.broadcasted_iota(jnp.int32, (RC // 2, 128), 1) >> 2) & 7
    def body(it, carry):
        rows = pl.ds(pl.multiple_of(it * RC, RC), RC)
        blocks = [pltpu.bitcast(src_ref[j, rows, 128 * b:128 * (b + 1)], jnp.uint32) for b in range(NB)]
        blocks = _butterfly(blocks, g)
        for i in range(NB):
            p = jnp.where(c == _dst(r, i), 1.0, 0.0).astype(bf16)
            t = pltpu.bitcast(blocks[i], bf16)
            dst_ref[j, rows, 128 * i:128 * (i + 1)] = _dot(t, p).astype(bf16)
        return carry
    lax.fori_loop(0, D // RC, body, 0)


def _permute_rows(src_ref, dst_ref):
    CC = 256
    r = lax.broadcasted_iota(jnp.int32, (128, 128), 0)
    c = lax.broadcasted_iota(jnp.int32, (128, 128), 1)
    g = (lax.broadcasted_iota(jnp.int32, (64, CC), 0) >> 1) & 7
    def body(it, carry):
        cols = pl.ds(pl.multiple_of(it * CC, CC), CC)
        blocks = [pltpu.bitcast(src_ref[128 * b:128 * (b + 1), cols], jnp.uint32) for b in range(NB)]
        blocks = _butterfly(blocks, g)
        for i in range(NB):
            pt = jnp.where(r == _dst(c, i), 1.0, 0.0).astype(bf16)
            t = pltpu.bitcast(blocks[i], bf16)
            dst_ref[128 * i:128 * (i + 1), cols] = _dot(pt, t).astype(bf16)
        return carry
    lax.fori_loop(0, D // CC, body, 0)


def _roll_in_groups(x):
    n = x.shape[0] // 8
    return pltpu.roll(x.reshape(n, 8, x.shape[1]), 1, 1).reshape(x.shape)


def make(TM=128, FC=512, AR=16, PRE=1, PAD=1, flags=None, SUB=1, order=0, nrun=None):
    G = TM // 8
    GP = G + PAD
    T = S // TM
    NS = 2 * T + 1
    NC = F // FC

    def kern(x0_ref, x_ref, wqkv_h, wo_h, w1_h, w3_h, w2_h, o_ref,
             wqkv_r, wo_r, wqkv, wo, w1, w3, w2, sem_a, sem_f,
             pbuf, qbuf, xn1, xn2, qkv_s, hk, hv, o_s, h_s, acc):
        s = pl.program_id(0)
        slot = s & 1
        l_att = (s >> 1) & 1
        fresh = jnp.logical_or(s == 0, s == 2)

        def cp_qkv(j):
            return pltpu.make_async_copy(wqkv_h.at[:, pl.ds(pl.multiple_of(j * D, D), D)], wqkv_r.at[j], sem_a.at[j])

        cp_wo = pltpu.make_async_copy(wo_h, wo_r, sem_a.at[3])

        def cp_ffn(c):
            cols = pl.ds(pl.multiple_of(c * FC, FC), FC)
            return (pltpu.make_async_copy(w1_h.at[:, cols], w1.at[c], sem_f.at[0, c]),
                    pltpu.make_async_copy(w3_h.at[:, cols], w3.at[c], sem_f.at[1, c]),
                    pltpu.make_async_copy(w2_h.at[cols, :], w2.at[cols, :], sem_f.at[2, c]))

        def load_x(ref):
            for c in range(8):
                for i in range(NB):
                    pbuf[i, GP * c:GP * c + G, :] = ref[G * c:G * (c + 1), 128 * i:128 * (i + 1)].astype(f32)

        def store_out():
            for c in range(8):
                for i in range(NB):
                    o_ref[G * c:G * (c + 1), 128 * i:128 * (i + 1)] = pbuf[i, GP * c:GP * c + G, :].astype(bf16)

        def p_rows(m0, n):
            return jnp.concatenate(
                [jnp.concatenate([pbuf[i, pl.ds(m0 + m, 8, stride=GP), :] for i in range(NB)], axis=1) for m in range(n)], axis=0)

        def ln1():
            for m in range(0, G, 2):
                xn1[8 * m:8 * m + 16, :] = _ln(p_rows(m, 2)).astype(bf16)

        def proj(j):
            qkv_s[j, HALO:, :] = _dot(xn1[...], wqkv[j])

        def halo():
            c0 = (lax.broadcasted_iota(jnp.int32, (HALO, D), 0) & 7) == 0
            for j, hal in ((1, hk), (2, hv)):
                cur = _roll_in_groups(qkv_s[j, TM:, :])
                prev = jnp.where(fresh, jnp.broadcast_to(qkv_s[j, HALO:HALO + 1, :], (HALO, D)), hal[l_att])
                qkv_s[j, 0:HALO, :] = jnp.where(c0, prev, cur)
                hal[l_att] = cur

        def attn_rows(r0):
            static = isinstance(r0, int)
            scale = DH ** -0.5
            def rows(w):
                b = HALO + r0 - SH * w
                return pl.ds(b if static else pl.multiple_of(b, 8), AR)
            q = [qkv_s[0, rows(0), 128 * i:128 * (i + 1)] for i in range(NB)]
            lg = []
            for w in range(WIN):
                a = q[0] * qkv_s[1, rows(w), 0:128]
                for i in range(1, NB):
                    a = a + q[i] * qkv_s[1, rows(w), 128 * i:128 * (i + 1)]
                a = a + pltpu.roll(a, 64, 1)
                a = a + pltpu.roll(a, 32, 1)
                a = a * scale
                if w > 0 and (not static or r0 < SH * w):
                    row = lax.broadcasted_iota(jnp.int32, (AR, 128), 0) + r0
                    bad = jnp.logical_and(jnp.logical_and(row < SH * w, (row & 7) == 0), fresh)
                    a = jnp.where(bad, -1e9, a)
                lg.append(a)
            mx = functools.reduce(jnp.maximum, lg)
            e = [jnp.exp(a - mx) for a in lg]
            inv = 1.0 / functools.reduce(lambda a, b: a + b, e)
            p = [a * inv for a in e]
            for i in range(NB):
                o = p[0] * qkv_s[2, rows(0), 128 * i:128 * (i + 1)]
                for w in range(1, WIN):
                    o = o + p[w] * qkv_s[2, rows(w), 128 * i:128 * (i + 1)]
                o_s[pl.ds(r0 if static else pl.multiple_of(r0, AR), AR), 128 * i:128 * (i + 1)] = o.astype(bf16)

        def proj_ln2():
            z = _dot(o_s[...], wo[...])
            for m in range(0, G, 2):
                x1 = p_rows(m, 2) + z[8 * m:8 * m + 16, :]
                qbuf[slot, 8 * m:8 * m + 16, :] = x1
                xn2[slot, 8 * m:8 * m + 16, :] = _ln(x1).astype(bf16)

        def gate_up(c):
            xn = xn2[1 - slot]
            gt = _dot(xn, w1[c])
            up = _dot(xn, w3[c])
            return (gt * jax.nn.sigmoid(gt) * up).astype(bf16)

        def finish(y):
            for m in range(G):
                x2 = qbuf[1 - slot, 8 * m:8 * m + 8, :] + y[8 * m:8 * m + 8, :]
                for i in range(NB):
                    pbuf[i, pl.ds(m, 8, stride=GP), :] = x2[:, 128 * i:128 * (i + 1)]

        @pl.when(s == 0)
        def _():
            cp_qkv(0).start()
            cp_qkv(1).start()
            hk[...] = jnp.zeros(hk.shape, f32)
            hv[...] = jnp.zeros(hv.shape, f32)
            load_x(x0_ref)

        def start_ffn(cs):
            for c in cs:
                for cp in cp_ffn(c):
                    cp.start()

        @pl.when(s <= 1)
        def _():
            ln1()
            def body(j, carry):
                @pl.when(s == 0)
                def _():
                    cp_qkv(j).wait()
                    pl.when(j == 0)(lambda: cp_qkv(2).start())
                    pl.when(j == 1)(lambda: cp_wo.start())
                    pl.when(j == 2)(lambda: start_ffn([0]))
                    _permute_cols(wqkv_r, wqkv, j)
                proj(j)
                return carry
            lax.fori_loop(0, 3, body, 0)
            halo()
            lax.fori_loop(0, TM // AR, lambda j, c: (attn_rows(j * AR), c)[1], 0)

            @pl.when(s == 0)
            def _():
                cp_wo.wait()
                start_ffn([1, 2])
                _permute_rows(wo_r, wo)
            proj_ln2()
            pl.when(s == 0)(lambda: start_ffn(range(3, NC)))

        @pl.when(jnp.logical_or(s == 1, s == NS - 1))
        def _():
            acc[...] = jnp.zeros(acc.shape, f32)
            def body(c, carry):
                @pl.when(s == 1)
                def _():
                    for cp in cp_ffn(c):
                        cp.wait()
                acc[...] += _dot(gate_up(c), w2[pl.ds(pl.multiple_of(c * FC, FC), FC), :])
                return carry
            lax.fori_loop(0, NC, body, 0)
            finish(acc[...])

        @pl.when(jnp.logical_and(s > 1, s < NS - 1))
        def _():
            rows = list(range(0, TM, AR))
            def gu(c):
                h_s[:, FC * c:FC * (c + 1)] = gate_up(c)
            for c in range(PRE):
                gu(c)
            ln1()
            for j in range(3):
                proj(j)
            halo()
            n = NC - PRE
            for j in range(n):
                gu(PRE + j)
                for r0 in rows[len(rows) * j // n:len(rows) * (j + 1) // n]:
                    attn_rows(r0)
            proj_ln2()
            finish(_dot(h_s[...], w2[...]))

        swap = jnp.logical_or((s & 3) == 3, (s & 3) == 0)

        @pl.when(jnp.logical_and(swap, s > 0))
        def _():
            store_out()

        @pl.when(jnp.logical_and(swap, s < NS - 1))
        def _():
            load_x(x_ref)

    def x_idx(s):
        return (jnp.minimum(2 * (s >> 2) + jnp.where((s & 3) == 0, 1, 2), T - 1), 0)

    def o_idx(s):
        return (jnp.where(s == 0, 0, 2 * ((s - 1) >> 2) + jnp.where((s & 3) == 0, 1, 0)), 0)

    @jax.jit
    def fn(A_x, A_wqkv, A_wo, B_x, B_w1, B_w3, B_w2):
        x = A_x.reshape(S, D)
        anyspec = pl.BlockSpec(memory_space=pl.ANY)
        out = pl.pallas_call(
            kern,
            grid=(nrun or NS,),
            in_specs=[pl.BlockSpec((TM, D), lambda s: (0, 0)), pl.BlockSpec((TM, D), x_idx)] + [anyspec] * 5,
            out_specs=pl.BlockSpec((TM, D), o_idx),
            out_shape=jax.ShapeDtypeStruct((S, D), bf16),
            scratch_shapes=[
                pltpu.VMEM((3, D, D), bf16), pltpu.VMEM((D, D), bf16),
                pltpu.VMEM((3, D, D), bf16), pltpu.VMEM((D, D), bf16),
                pltpu.VMEM((NC, D, FC), bf16), pltpu.VMEM((NC, D, FC), bf16), pltpu.VMEM((F, D), bf16),
                pltpu.SemaphoreType.DMA((4,)), pltpu.SemaphoreType.DMA((3, NC)),
                pltpu.VMEM((NB, 8 * GP, 128), f32), pltpu.VMEM((2, TM, D), f32),
                pltpu.VMEM((TM, D), bf16), pltpu.VMEM((2, TM, D), bf16),
                pltpu.VMEM((3, TM + HALO, D), f32),
                pltpu.VMEM((2, HALO, D), f32), pltpu.VMEM((2, HALO, D), f32),
                pltpu.VMEM((TM, D), bf16), pltpu.VMEM((TM, F), bf16), pltpu.VMEM((TM, D), f32),
            ],
            compiler_params=pltpu.CompilerParams(
                dimension_semantics=("arbitrary",),
                vmem_limit_bytes=110 * 1024 * 1024, flags=flags),
        )(x, x, A_wqkv, A_wo, B_w1, B_w3, B_w2)
        return out.reshape(1, S, D)
    return fn


_kernel = make()


def pallas_interleave_layers__sliding_local_dilated__glu_gated_swiglu__prompt_kernel(A_x, A_wqkv, A_wo, B_x, B_w1, B_w3, B_w2):
    return _kernel(A_x, A_wqkv, A_wo, B_x, B_w1, B_w3, B_w2)
```

```python
import functools
import jax
import jax.numpy as jnp
from jax import lax
import jax.experimental.pallas as pl
import jax.experimental.pallas.tpu as pltpu

S, D, H, DH, WIN, DIL, F = 2048, 1024, 32, 32, 8, 2, 3584
NB = D // 128
SH = 8 * DIL
HALO = (WIN - 1) * SH
f32, bf16 = jnp.float32, jnp.bfloat16


def _dot(a, b):
    return jnp.dot(a, b, preferred_element_type=f32)


def _ln(x):
    m = jnp.mean(x, axis=-1, keepdims=True)
    xc = x - m
    v = jnp.mean(xc * xc, axis=-1, keepdims=True)
    return xc * lax.rsqrt(v + 1e-5)


def _dst(src, i):
    g = (src >> 2) & 7
    return (src & 3) * 32 + (g ^ i) * 4 + (src >> 5)


def _butterfly(blocks, g):
    for b in range(3):
        m = ((g >> b) & 1) == 1
        blocks = [jnp.where(m, blocks[j ^ (1 << b)], blocks[j]) for j in range(NB)]
    return blocks


def _permute_cols(src_ref, dst_ref, j):
    RC = 256
    r = lax.broadcasted_iota(jnp.int32, (128, 128), 0)
    c = lax.broadcasted_iota(jnp.int32, (128, 128), 1)
    g = (lax.broadcasted_iota(jnp.int32, (RC // 2, 128), 1) >> 2) & 7
    def body(it, carry):
        rows = pl.ds(pl.multiple_of(it * RC, RC), RC)
        blocks = [pltpu.bitcast(src_ref[j, rows, 128 * b:128 * (b + 1)], jnp.uint32) for b in range(NB)]
        blocks = _butterfly(blocks, g)
        for i in range(NB):
            p = jnp.where(c == _dst(r, i), 1.0, 0.0).astype(bf16)
            t = pltpu.bitcast(blocks[i], bf16)
            dst_ref[j, rows, 128 * i:128 * (i + 1)] = _dot(t, p).astype(bf16)
        return carry
    lax.fori_loop(0, D // RC, body, 0)


def _permute_rows(src_ref, dst_ref):
    CC = 256
    r = lax.broadcasted_iota(jnp.int32, (128, 128), 0)
    c = lax.broadcasted_iota(jnp.int32, (128, 128), 1)
    g = (lax.broadcasted_iota(jnp.int32, (64, CC), 0) >> 1) & 7
    def body(it, carry):
        cols = pl.ds(pl.multiple_of(it * CC, CC), CC)
        blocks = [pltpu.bitcast(src_ref[128 * b:128 * (b + 1), cols], jnp.uint32) for b in range(NB)]
        blocks = _butterfly(blocks, g)
        for i in range(NB):
            pt = jnp.where(r == _dst(c, i), 1.0, 0.0).astype(bf16)
            t = pltpu.bitcast(blocks[i], bf16)
            dst_ref[128 * i:128 * (i + 1), cols] = _dot(pt, t).astype(bf16)
        return carry
    lax.fori_loop(0, D // CC, body, 0)


def _roll_in_groups(x):
    n = x.shape[0] // 8
    return pltpu.roll(x.reshape(n, 8, x.shape[1]), 1, 1).reshape(x.shape)


def make(TM=128, FC=512, AR=8, PRE=2, PAD=1, flags=None, SUB=2, order=2, nrun=None, FS=256, dbg=0, ARL=32):
    G = TM // 8
    GP = G + PAD
    T = S // TM
    NS = 2 * T + 1
    NC = F // FC

    def kern(x_h, wqkv_h, wo_h, w1_h, w3_h, w2_h, out_h,
             wqkv_r, wo_r, wqkv, wo, w1, w3, w2, sem_a, sem_f,
             pbuf, qbuf, xn1, xn2, qkv_s, hk, hv, o_s, h_s, acc, x_ref, o_ref, sem_io):

        def cp_qkv(j):
            return pltpu.make_async_copy(wqkv_h.at[:, pl.ds(pl.multiple_of(j * D, D), D)], wqkv_r.at[j], sem_a.at[j])

        cp_wo = pltpu.make_async_copy(wo_h, wo_r, sem_a.at[3])

        def cp_ffn(c):
            cols = pl.ds(pl.multiple_of(c * FC, FC), FC)
            return (pltpu.make_async_copy(w1_h.at[:, cols], w1.at[c], sem_f.at[0, c]),
                    pltpu.make_async_copy(w3_h.at[:, cols], w3.at[c], sem_f.at[1, c]),
                    pltpu.make_async_copy(w2_h.at[cols, :], w2.at[cols, :], sem_f.at[2, c]))

        def load_x():
            for c in range(8):
                for i in range(NB):
                    pbuf[i, GP * c:GP * c + G, :] = x_ref[G * c:G * (c + 1), 128 * i:128 * (i + 1)].astype(f32)

        def store_out():
            for c in range(8):
                for i in range(NB):
                    o_ref[G * c:G * (c + 1), 128 * i:128 * (i + 1)] = pbuf[i, GP * c:GP * c + G, :].astype(bf16)

        def prow(m):
            return pl.ds(8 * m, 8) if dbg & 2 else pl.ds(m, 8, stride=GP)

        def p_rows(m0, n):
            return jnp.concatenate(
                [jnp.concatenate([pbuf[i, prow(m0 + m), :] for i in range(NB)], axis=1) for m in range(n)], axis=0)

        def ln1():
            for m in range(0, G, 2):
                xn1[8 * m:8 * m + 16, :] = _ln(p_rows(m, 2)).astype(bf16)

        def proj(j):
            qkv_s[j, HALO:, :] = _dot(xn1[...], wqkv[j])

        def halo(s):
            l_att = (s >> 1) & 1
            fresh = jnp.logical_or(s == 0, s == 2)
            c0 = (lax.broadcasted_iota(jnp.int32, (HALO, D), 0) & 7) == 0
            for j, hal in ((1, hk), (2, hv)):
                cur = _roll_in_groups(qkv_s[j, TM:, :])
                prev = jnp.where(fresh, jnp.broadcast_to(qkv_s[j, HALO:HALO + 1, :], (HALO, D)), hal[l_att])
                qkv_s[j, 0:HALO, :] = jnp.where(c0, prev, cur)
                hal[l_att] = cur

        def attn_rows(s, r0, AR):
            fresh = jnp.logical_or(s == 0, s == 2)
            static = isinstance(r0, int)
            scale = DH ** -0.5
            def rows(w):
                b = HALO + r0 - SH * w
                return pl.ds(b if static else pl.multiple_of(b, 8), AR)
            q = [qkv_s[0, rows(0), 128 * i:128 * (i + 1)] for i in range(NB)]
            lg = []
            for w in range(WIN):
                a = q[0] * qkv_s[1, rows(w), 0:128]
                for i in range(1, NB):
                    a = a + q[i] * qkv_s[1, rows(w), 128 * i:128 * (i + 1)]
                a = a + pltpu.roll(a, 64, 1)
                a = a + pltpu.roll(a, 32, 1)
                a = a * scale
                if w > 0 and (not static or r0 < SH * w):
                    row = lax.broadcasted_iota(jnp.int32, (AR, 128), 0) + r0
                    bad = jnp.logical_and(jnp.logical_and(row < SH * w, (row & 7) == 0), fresh)
                    a = jnp.where(bad, -1e9, a)
                lg.append(a)
            mx = functools.reduce(jnp.maximum, lg)
            e = [jnp.exp(a - mx) for a in lg]
            inv = 1.0 / functools.reduce(lambda a, b: a + b, e)
            p = [a * inv for a in e]
            for i in range(NB):
                o = p[0] * qkv_s[2, rows(0), 128 * i:128 * (i + 1)]
                for w in range(1, WIN):
                    o = o + p[w] * qkv_s[2, rows(w), 128 * i:128 * (i + 1)]
                o_s[pl.ds(r0 if static else pl.multiple_of(r0, AR), AR), 128 * i:128 * (i + 1)] = o.astype(bf16)

        def proj_ln2(s):
            slot = s & 1
            z = _dot(o_s[...], wo[...])
            for m in range(0, G, 2):
                x1 = p_rows(m, 2) + z[8 * m:8 * m + 16, :]
                qbuf[slot, 8 * m:8 * m + 16, :] = x1
                xn2[slot, 8 * m:8 * m + 16, :] = _ln(x1).astype(bf16)

        def gate_up(s, c):
            xn = xn2[1 - (s & 1)]
            gt = _dot(xn, w1[c])
            up = _dot(xn, w3[c])
            return (gt * jax.nn.sigmoid(gt) * up).astype(bf16)

        def finish(s, y):
            slot = s & 1
            for m in range(G):
                x2 = qbuf[1 - slot, 8 * m:8 * m + 8, :] + y[8 * m:8 * m + 8, :]
                for i in range(NB):
                    pbuf[i, prow(m), :] = x2[:, 128 * i:128 * (i + 1)]

        def cp_x(t):
            return pltpu.make_async_copy(x_h.at[pl.ds(pl.multiple_of(t * TM, TM), TM), :], x_ref, sem_io.at[0])

        def cp_out(t):
            return pltpu.make_async_copy(o_ref, out_h.at[pl.ds(pl.multiple_of(t * TM, TM), TM), :], sem_io.at[1])

        def next_x(t):
            cp_x(t).wait()
            load_x()
            pl.when(t + 1 < T)(lambda: cp_x(t + 1).start())

        def start_ffn(cs):
            for c in cs:
                for cp in cp_ffn(c):
                    cp.start()

        def att_only(s, carry):
            next_x(s)
            ln1()
            def body(j, carry):
                @pl.when(s == 0)
                def _():
                    cp_qkv(j).wait()
                    pl.when(j == 0)(lambda: cp_qkv(2).start())
                    pl.when(j == 1)(lambda: cp_wo.start())
                    pl.when(j == 2)(lambda: start_ffn([0]))
                    _permute_cols(wqkv_r, wqkv, j)
                proj(j)
                return carry
            lax.fori_loop(0, 3, body, 0)
            halo(s)
            lax.fori_loop(0, TM // ARL, lambda j, c: (attn_rows(s, j * ARL, ARL), c)[1], 0)

            @pl.when(s == 0)
            def _():
                cp_wo.wait()
                start_ffn([1, 2])
                _permute_rows(wo_r, wo)
            proj_ln2(s)
            pl.when(s == 0)(lambda: start_ffn(range(3, NC)))
            return carry

        def ffn_only(s):
            acc[...] = jnp.zeros(acc.shape, f32)
            def body(c, carry):
                @pl.when(s == 1)
                def _():
                    for cp in cp_ffn(c):
                        cp.wait()
                acc[...] += _dot(gate_up(s, c), w2[pl.ds(pl.multiple_of(c * FC, FC), FC), :])
                return carry
            lax.fori_loop(0, NC, body, 0)
            finish(s, acc[...])

        def steady(s, carry):
            rows = list(range(0, TM, AR))
            zero = pl.multiple_of((s >> 10) * 8, 8)
            def gate(val):
                qkv_s[0, pl.ds(zero, 8), 0:128] = val[TM - 8:TM, val.shape[1] - 128:]
            n = F // FS - PRE
            npt = (2 * n if SUB == 2 else n) - order
            def attn_part(j):
                for r0 in rows[len(rows) * j // npt:len(rows) * (j + 1) // npt]:
                    if not dbg & 4:
                        attn_rows(s, r0, AR)
            def gu(c, j=None):
                xn = xn2[1 - (s & 1)]
                cw, cs = (FS * c) // FC, pl.ds((FS * c) % FC, FS)
                gt = _dot(xn, w1[cw, :, cs])
                if j is not None and SUB == 2:
                    gate(gt)
                    attn_part(2 * j)
                up = _dot(xn, w3[cw, :, cs])
                if j is not None:
                    if SUB:
                        gate(up)
                    attn_part(2 * j + 1 if SUB == 2 else j)
                h_s[:, FS * c:FS * (c + 1)] = (gt * jax.nn.sigmoid(gt) * up).astype(bf16)
            for c in range(PRE):
                gu(c)
            ln1()
            for j in range(3):
                proj(j)
            halo(s)
            for j in range(n):
                gu(PRE + j, j)
            proj_ln2(s)
            finish(s, _dot(h_s[...], w2[...]))

            @pl.when(jnp.logical_or((s & 3) == 3, (s & 3) == 0))
            def _():
                t = (s - 2) >> 1
                pl.when(t > 0)(lambda: cp_out(t - 1).wait())
                store_out()
                cp_out(t).start()
                pl.when(t + 2 < T)(lambda: next_x(t + 2))
            return carry

        cp_x(0).start()
        cp_qkv(0).start()
        cp_qkv(1).start()
        hk[...] = jnp.zeros(hk.shape, f32)
        hv[...] = jnp.zeros(hv.shape, f32)
        lax.fori_loop(0, 2, att_only, 0)

        def phase(p, carry):
            ffn_only(1 + p * (NS - 2))

            @pl.when(p == 0)
            def _():
                lax.fori_loop(2, nrun or (NS - 1), steady, 0)
            return carry
        lax.fori_loop(0, 2, phase, 0)
        if nrun is None:
            cp_out(T - 2).wait()
        else:
            cp_out(0).wait()
            cp_x(0).wait()
        store_out()
        cp_out(T - 1).start()
        cp_out(T - 1).wait()

    @jax.jit
    def fn(A_x, A_wqkv, A_wo, B_x, B_w1, B_w3, B_w2):
        x = A_x.reshape(S, D)
        anyspec = pl.BlockSpec(memory_space=pl.ANY)
        out = pl.pallas_call(
            kern,
            in_specs=[anyspec] * 6,
            out_specs=anyspec,
            out_shape=jax.ShapeDtypeStruct((S, D), bf16),
            scratch_shapes=[
                pltpu.VMEM((3, D, D), bf16), pltpu.VMEM((D, D), bf16),
                pltpu.VMEM((3, D, D), bf16), pltpu.VMEM((D, D), bf16),
                pltpu.VMEM((NC, D, FC), bf16), pltpu.VMEM((NC, D, FC), bf16), pltpu.VMEM((F, D), bf16),
                pltpu.SemaphoreType.DMA((4,)), pltpu.SemaphoreType.DMA((3, NC)),
                pltpu.VMEM((NB, 8 * GP, 128), f32), pltpu.VMEM((2, TM, D), f32),
                pltpu.VMEM((TM, D), bf16), pltpu.VMEM((2, TM, D), bf16),
                pltpu.VMEM((3, TM + HALO, D), f32),
                pltpu.VMEM((2, HALO, D), f32), pltpu.VMEM((2, HALO, D), f32),
                pltpu.VMEM((TM, D), bf16), pltpu.VMEM((TM, F), bf16), pltpu.VMEM((TM, D), f32),
                pltpu.VMEM((TM, D), bf16), pltpu.VMEM((TM, D), bf16), pltpu.SemaphoreType.DMA((2,)),
            ],
            compiler_params=pltpu.CompilerParams(
                vmem_limit_bytes=110 * 1024 * 1024, flags=flags),
        )(x, A_wqkv, A_wo, B_w1, B_w3, B_w2)
        return out.reshape(1, S, D)
    return fn


_kernel = make()


def pallas_interleave_layers__sliding_local_dilated__glu_gated_swiglu__prompt_kernel(A_x, A_wqkv, A_wo, B_x, B_w1, B_w3, B_w2):
    return _kernel(A_x, A_wqkv, A_wo, B_x, B_w1, B_w3, B_w2)
```

```python
import functools
import jax
import jax.numpy as jnp
from jax import lax
import jax.experimental.pallas as pl
import jax.experimental.pallas.tpu as pltpu

S, D, H, DH, WIN, DIL, F = 2048, 1024, 32, 32, 8, 2, 3584
NB = D // 128
SH = 8 * DIL
HALO = (WIN - 1) * SH
f32, bf16 = jnp.float32, jnp.bfloat16


def _dot(a, b):
    return jnp.dot(a, b, preferred_element_type=f32)


def _ln(x):
    m = jnp.mean(x, axis=-1, keepdims=True)
    xc = x - m
    v = jnp.mean(xc * xc, axis=-1, keepdims=True)
    return xc * lax.rsqrt(v + 1e-5)


def _swiglu(g, u, th):
    if th:
        hg = 0.5 * g
        return ((hg + hg * jnp.tanh(hg)) * u).astype(bf16)
    return (g * jax.nn.sigmoid(g) * u).astype(bf16)


def _tree(t):
    while len(t) > 1:
        t = [t[j] + t[j + 1] for j in range(0, len(t), 2)]
    return t[0]


def _dst(src, i):
    g = (src >> 2) & 7
    return (src & 3) * 32 + (g ^ i) * 4 + (src >> 5)


def _butterfly(blocks, g):
    for b in range(3):
        m = ((g >> b) & 1) == 1
        blocks = [jnp.where(m, blocks[j ^ (1 << b)], blocks[j]) for j in range(NB)]
    return blocks


def _permute_cols(src_ref, dst_ref, j):
    RC = 256
    r = lax.broadcasted_iota(jnp.int32, (128, 128), 0)
    c = lax.broadcasted_iota(jnp.int32, (128, 128), 1)
    g = (lax.broadcasted_iota(jnp.int32, (RC // 2, 128), 1) >> 2) & 7
    def body(it, carry):
        rows = pl.ds(pl.multiple_of(it * RC, RC), RC)
        blocks = [pltpu.bitcast(src_ref[j, rows, 128 * b:128 * (b + 1)], jnp.uint32) for b in range(NB)]
        blocks = _butterfly(blocks, g)
        for i in range(NB):
            p = jnp.where(c == _dst(r, i), 1.0, 0.0).astype(bf16)
            t = pltpu.bitcast(blocks[i], bf16)
            dst_ref[j, rows, 128 * i:128 * (i + 1)] = _dot(t, p).astype(bf16)
        return carry
    lax.fori_loop(0, D // RC, body, 0)


def _permute_rows(src_ref, dst_ref):
    CC = 256
    r = lax.broadcasted_iota(jnp.int32, (128, 128), 0)
    c = lax.broadcasted_iota(jnp.int32, (128, 128), 1)
    g = (lax.broadcasted_iota(jnp.int32, (64, CC), 0) >> 1) & 7
    def body(it, carry):
        cols = pl.ds(pl.multiple_of(it * CC, CC), CC)
        blocks = [pltpu.bitcast(src_ref[128 * b:128 * (b + 1), cols], jnp.uint32) for b in range(NB)]
        blocks = _butterfly(blocks, g)
        for i in range(NB):
            pt = jnp.where(r == _dst(c, i), 1.0, 0.0).astype(bf16)
            t = pltpu.bitcast(blocks[i], bf16)
            dst_ref[128 * i:128 * (i + 1), cols] = _dot(pt, t).astype(bf16)
        return carry
    lax.fori_loop(0, D // CC, body, 0)


def _roll_in_groups(x):
    n = x.shape[0] // 8
    return pltpu.roll(x.reshape(n, 8, x.shape[1]), 1, 1).reshape(x.shape)


def make(TM=128, FC=512, AR=8, PRE=2, PAD=1, flags=None, SUB=2, order=2, nrun=None, FS=256, dbg=0, ARL=32, SER=1, TH=True, GATE=True):
    G = TM // 8
    GP = G + PAD
    T = S // TM
    NS = 2 * T + 1
    NC = F // FC

    def kern(x_h, wqkv_h, wo_h, w1_h, w3_h, w2_h, out_h,
             wqkv_r, wo_r, wqkv, wo, w1, w3, w2, sem_a, sem_f,
             pbuf, qbuf, xn1, xn2, qkv_s, hk, hv, h_s, acc, x_ref, o_ref, sem_io):

        def cp_qkv(j):
            return pltpu.make_async_copy(wqkv_h.at[:, pl.ds(pl.multiple_of(j * D, D), D)], wqkv_r.at[j], sem_a.at[j])

        cp_wo = pltpu.make_async_copy(wo_h, wo_r, sem_a.at[3])

        def cp_ffn(c):
            cols = pl.ds(pl.multiple_of(c * FC, FC), FC)
            return (pltpu.make_async_copy(w1_h.at[:, cols], w1.at[c], sem_f.at[0, c]),
                    pltpu.make_async_copy(w3_h.at[:, cols], w3.at[c], sem_f.at[1, c]),
                    pltpu.make_async_copy(w2_h.at[cols, :], w2.at[cols, :], sem_f.at[2, c]))

        def load_x():
            for c in range(8):
                for i in range(NB):
                    pbuf[i, GP * c:GP * c + G, :] = x_ref[G * c:G * (c + 1), 128 * i:128 * (i + 1)].astype(f32)

        def store_out():
            for c in range(8):
                for i in range(NB):
                    o_ref[G * c:G * (c + 1), 128 * i:128 * (i + 1)] = pbuf[i, GP * c:GP * c + G, :].astype(bf16)

        def prow(m):
            return pl.ds(8 * m, 8) if dbg & 2 else pl.ds(m, 8, stride=GP)

        def p_rows(m0, n):
            return jnp.concatenate(
                [jnp.concatenate([pbuf[i, prow(m0 + m), :] for i in range(NB)], axis=1) for m in range(n)], axis=0)

        def ln1():
            for m in range(0, G, 2):
                xn1[8 * m:8 * m + 16, :] = _ln(p_rows(m, 2)).astype(bf16)

        def proj(j):
            qkv_s[j, HALO:, :] = _dot(xn1[...], wqkv[j])

        def halo(s):
            l_att = (s >> 1) & 1
            fresh = jnp.logical_or(s == 0, s == 2)
            c0 = (lax.broadcasted_iota(jnp.int32, (HALO, D), 0) & 7) == 0
            for j, hal in ((1, hk), (2, hv)):
                cur = _roll_in_groups(qkv_s[j, TM:, :])
                prev = jnp.where(fresh, jnp.broadcast_to(qkv_s[j, HALO:HALO + 1, :], (HALO, D)), hal[l_att])
                qkv_s[j, 0:HALO, :] = jnp.where(c0, prev, cur)
                hal[l_att] = cur

        def attn_rows(s, r0, AR, ser=0):
            fresh = jnp.logical_or(s == 0, s == 2)
            static = isinstance(r0, int)
            scale = DH ** -0.5
            zero = (s >> 10) * 8
            def rows(w, z=0):
                b = HALO + r0 - SH * w + z
                return pl.ds(b if isinstance(b, int) else pl.multiple_of(b, 8), AR)
            q = [qkv_s[0, rows(0), 128 * i:128 * (i + 1)] for i in range(NB)]
            l = []
            for w in range(WIN):
                t = [q[i] * qkv_s[1, rows(w), 128 * i:128 * (i + 1)] for i in range(NB)]
                a = _tree(t)
                if ser and w % ser == ser - 1:
                    qkv_s[0, pl.ds(pl.multiple_of(zero, 8), AR), 0:128] = a
                a = a + pltpu.roll(a, 64, 1)
                a = a + pltpu.roll(a, 32, 1)
                a = a * scale
                if w > 0 and (not static or r0 < SH * w):
                    row = lax.broadcasted_iota(jnp.int32, (AR, 128), 0) + r0
                    bad = jnp.logical_and(jnp.logical_and(row < SH * w, (row & 7) == 0), fresh)
                    a = jnp.where(bad, -1e9, a)
                l.append(a)
            mx = functools.reduce(jnp.maximum, l)
            e = [jnp.exp(a - mx) for a in l]
            inv = 1.0 / _tree(e)
            p = [a * inv for a in e]
            for i in range(NB):
                cols = slice(128 * i, 128 * (i + 1))
                o = _tree([p[w] * qkv_s[2, rows(w), cols] for w in range(WIN)])
                qkv_s[0, rows(0, zero if ser and i % ser == ser - 1 else 0), cols] = o

        def proj_ln2(s):
            slot = s & 1
            z = _dot(qkv_s[0, HALO:, :].astype(bf16), wo[...])
            for m in range(0, G, 2):
                x1 = p_rows(m, 2) + z[8 * m:8 * m + 16, :]
                qbuf[slot, 8 * m:8 * m + 16, :] = x1
                xn2[slot, 8 * m:8 * m + 16, :] = _ln(x1).astype(bf16)

        def gate_up(s, c):
            xn = xn2[1 - (s & 1)]
            gt = _dot(xn, w1[c])
            up = _dot(xn, w3[c])
            return _swiglu(gt, up, TH)

        def finish(s, y):
            slot = s & 1
            for m in range(G):
                x2 = qbuf[1 - slot, 8 * m:8 * m + 8, :] + y[8 * m:8 * m + 8, :]
                for i in range(NB):
                    pbuf[i, prow(m), :] = x2[:, 128 * i:128 * (i + 1)]

        def cp_x(t):
            return pltpu.make_async_copy(x_h.at[pl.ds(pl.multiple_of(t * TM, TM), TM), :], x_ref, sem_io.at[0])

        def cp_out(t):
            return pltpu.make_async_copy(o_ref, out_h.at[pl.ds(pl.multiple_of(t * TM, TM), TM), :], sem_io.at[1])

        def next_x(t):
            cp_x(t).wait()
            load_x()
            pl.when(t + 1 < T)(lambda: cp_x(t + 1).start())

        def start_ffn(cs):
            for c in ([] if dbg & 8 else cs):
                for cp in cp_ffn(c):
                    cp.start()

        def att_only(s, carry):
            next_x(s)
            ln1()
            def body(j, carry):
                @pl.when(s == 0)
                def _():
                    cp_qkv(j).wait()
                    pl.when(j == 0)(lambda: cp_qkv(2).start())
                    pl.when(j == 1)(lambda: cp_wo.start())
                    pl.when(j == 2)(lambda: start_ffn([0]))
                    _permute_cols(wqkv_r, wqkv, j)
                proj(j)
                return carry
            lax.fori_loop(0, 3, body, 0)
            halo(s)
            lax.fori_loop(0, TM // ARL, lambda j, c: (attn_rows(s, j * ARL, ARL), c)[1], 0)

            @pl.when(s == 0)
            def _():
                cp_wo.wait()
                start_ffn([1, 2])
                _permute_rows(wo_r, wo)
            proj_ln2(s)
            pl.when(s == 0)(lambda: start_ffn(range(3, NC)))
            return carry

        def ffn_only(s):
            acc[...] = jnp.zeros(acc.shape, f32)
            def body(c, carry):
                @pl.when(s == 1)
                def _():
                    for cp in ([] if dbg & 8 else cp_ffn(c)):
                        cp.wait()
                acc[...] += _dot(gate_up(s, c), w2[pl.ds(pl.multiple_of(c * FC, FC), FC), :])
                return carry
            lax.fori_loop(0, NC, body, 0)
            finish(s, acc[...])

        def steady(s, carry):
            rows = list(range(0, TM, AR))
            zero = pl.multiple_of((s >> 10) * 8, 8)
            def gate(val):
                if GATE:
                    qkv_s[0, pl.ds(zero, 8), 0:128] = val[TM - 8:TM, val.shape[1] - 128:]
            n = F // FS - PRE
            npt = (2 * n if SUB == 2 else n) - order
            def attn_part(j):
                for r0 in rows[len(rows) * j // npt:len(rows) * (j + 1) // npt]:
                    if not dbg & 4:
                        attn_rows(s, r0, AR, SER)
            def gu(c, j=None):
                xn = xn2[1 - (s & 1)]
                cw, cs = (FS * c) // FC, pl.ds((FS * c) % FC, FS)
                gt = _dot(xn, w1[cw, :, cs])
                if j is not None and SUB == 2:
                    gate(gt)
                    attn_part(2 * j)
                up = _dot(xn, w3[cw, :, cs])
                if j is not None:
                    if SUB:
                        gate(up)
                    attn_part(2 * j + 1 if SUB == 2 else j)
                h_s[:, FS * c:FS * (c + 1)] = _swiglu(gt, up, TH)
            for c in range(PRE):
                gu(c)
            ln1()
            for j in range(3):
                proj(j)
            halo(s)
            for j in range(n):
                gu(PRE + j, j)
            proj_ln2(s)
            finish(s, _dot(h_s[...], w2[...]))

            @pl.when(jnp.logical_or((s & 3) == 3, (s & 3) == 0))
            def _():
                t = (s - 2) >> 1
                pl.when(t > 0)(lambda: cp_out(t - 1).wait())
                store_out()
                cp_out(t).start()
                pl.when(t + 2 < T)(lambda: next_x(t + 2))
            return carry

        cp_x(0).start()
        cp_qkv(0).start()
        cp_qkv(1).start()
        hk[...] = jnp.zeros(hk.shape, f32)
        hv[...] = jnp.zeros(hv.shape, f32)
        lax.fori_loop(0, 2, att_only, 0)

        def phase(p, carry):
            ffn_only(1 + p * (NS - 2))

            @pl.when(p == 0)
            def _():
                lax.fori_loop(2, nrun or (NS - 1), steady, 0)
            return carry
        lax.fori_loop(0, 2, phase, 0)
        if nrun is None:
            cp_out(T - 2).wait()
        else:
            cp_out(0).wait()
            cp_x(0).wait()
        store_out()
        cp_out(T - 1).start()
        cp_out(T - 1).wait()

    @jax.jit
    def fn(A_x, A_wqkv, A_wo, B_x, B_w1, B_w3, B_w2):
        x = A_x.reshape(S, D)
        anyspec = pl.BlockSpec(memory_space=pl.ANY)
        out = pl.pallas_call(
            kern,
            in_specs=[anyspec] * 6,
            out_specs=anyspec,
            out_shape=jax.ShapeDtypeStruct((S, D), bf16),
            scratch_shapes=[
                pltpu.VMEM((3, D, D), bf16), pltpu.VMEM((D, D), bf16),
                pltpu.VMEM((3, D, D), bf16), pltpu.VMEM((D, D), bf16),
                pltpu.VMEM((NC, D, FC), bf16), pltpu.VMEM((NC, D, FC), bf16), pltpu.VMEM((F, D), bf16),
                pltpu.SemaphoreType.DMA((4,)), pltpu.SemaphoreType.DMA((3, NC)),
                pltpu.VMEM((NB, 8 * GP, 128), f32), pltpu.VMEM((2, TM, D), f32),
                pltpu.VMEM((TM, D), bf16), pltpu.VMEM((2, TM, D), bf16),
                pltpu.VMEM((3, TM + HALO, D), f32),
                pltpu.VMEM((2, HALO, D), f32), pltpu.VMEM((2, HALO, D), f32),
                pltpu.VMEM((TM, F), bf16), pltpu.VMEM((TM, D), f32),
                pltpu.VMEM((TM, D), bf16), pltpu.VMEM((TM, D), bf16), pltpu.SemaphoreType.DMA((2,)),
            ],
            compiler_params=pltpu.CompilerParams(
                vmem_limit_bytes=110 * 1024 * 1024, flags=flags),
        )(x, A_wqkv, A_wo, B_w1, B_w3, B_w2)
        return out.reshape(1, S, D)
    return fn


_kernel = make()


def pallas_interleave_layers__sliding_local_dilated__glu_gated_swiglu__prompt_kernel(A_x, A_wqkv, A_wo, B_x, B_w1, B_w3, B_w2):
    return _kernel(A_x, A_wqkv, A_wo, B_x, B_w1, B_w3, B_w2)
```

```python
import functools
import jax
import jax.numpy as jnp
from jax import lax
import jax.experimental.pallas as pl
import jax.experimental.pallas.tpu as pltpu

S, D, H, DH, WIN, DIL, F = 2048, 1024, 32, 32, 8, 2, 3584
NB = D // 128
SH = 8 * DIL
HALO = (WIN - 1) * SH
f32, bf16 = jnp.float32, jnp.bfloat16


def _dot(a, b):
    return jnp.dot(a, b, preferred_element_type=f32)


def _ln(x):
    m = jnp.mean(x, axis=-1, keepdims=True)
    xc = x - m
    v = jnp.mean(xc * xc, axis=-1, keepdims=True)
    return xc * lax.rsqrt(v + 1e-5)


def _swiglu(g, u, th):
    if th:
        hg = 0.5 * g
        return (hg + hg * jnp.tanh(hg)) * u
    return g * jax.nn.sigmoid(g) * u


def _tree(t):
    while len(t) > 1:
        t = [t[j] + t[j + 1] for j in range(0, len(t), 2)]
    return t[0]


def _a_terms(a11, a12, a21, a22):
    return (a11 + a22, a21 + a22, a11, a22, a11 + a12, a21 - a11, a12 - a22)


def _b_terms(b11, b12, b21, b22):
    return (b11 + b22, b11, b12 - b22, b21 - b11, b22, b11 + b12, b21 + b22)


def _strassen(prod):
    m1 = prod(0)
    m2 = prod(1)
    t22 = m1 - m2
    m4 = prod(3)
    c21 = m2 + m4
    t11 = m1 + m4 + prod(6)
    m5 = prod(4)
    c11 = t11 - m5
    m3 = prod(2)
    c12 = m3 + m5
    c22 = t22 + m3 + prod(5)
    return c11, c12, c21, c22


def _dst(src, i):
    g = (src >> 2) & 7
    return (src & 3) * 32 + (g ^ i) * 4 + (src >> 5)


def _butterfly(blocks, g):
    for b in range(3):
        m = ((g >> b) & 1) == 1
        blocks = [jnp.where(m, blocks[j ^ (1 << b)], blocks[j]) for j in range(NB)]
    return blocks


def _permute_cols(src_ref, dst_ref, j):
    RC = 256
    r = lax.broadcasted_iota(jnp.int32, (128, 128), 0)
    c = lax.broadcasted_iota(jnp.int32, (128, 128), 1)
    g = (lax.broadcasted_iota(jnp.int32, (RC // 2, 128), 1) >> 2) & 7
    def body(it, carry):
        rows = pl.ds(pl.multiple_of(it * RC, RC), RC)
        blocks = [pltpu.bitcast(src_ref[j, rows, 128 * b:128 * (b + 1)], jnp.uint32) for b in range(NB)]
        blocks = _butterfly(blocks, g)
        for i in range(NB):
            p = jnp.where(c == _dst(r, i), 1.0, 0.0).astype(bf16)
            t = pltpu.bitcast(blocks[i], bf16)
            dst_ref[rows, 128 * i:128 * (i + 1)] = _dot(t, p).astype(bf16)
        return carry
    lax.fori_loop(0, D // RC, body, 0)


def _permute_rows(src_ref, dst_ref):
    CC = 256
    r = lax.broadcasted_iota(jnp.int32, (128, 128), 0)
    c = lax.broadcasted_iota(jnp.int32, (128, 128), 1)
    g = (lax.broadcasted_iota(jnp.int32, (64, CC), 0) >> 1) & 7
    def body(it, carry):
        cols = pl.ds(pl.multiple_of(it * CC, CC), CC)
        blocks = [pltpu.bitcast(src_ref[128 * b:128 * (b + 1), cols], jnp.uint32) for b in range(NB)]
        blocks = _butterfly(blocks, g)
        for i in range(NB):
            pt = jnp.where(r == _dst(c, i), 1.0, 0.0).astype(bf16)
            t = pltpu.bitcast(blocks[i], bf16)
            dst_ref[128 * i:128 * (i + 1), cols] = _dot(pt, t).astype(bf16)
        return carry
    lax.fori_loop(0, D // CC, body, 0)


def _roll_in_groups(x):
    n = x.shape[0] // 8
    return pltpu.roll(x.reshape(n, 8, x.shape[1]), 1, 1).reshape(x.shape)


def make(TM=128, FC=512, AR=8, PRE=1, PAD=1, flags=None, SUB=2, order=6, nrun=None, FS=256, dbg=0, ARL=32, SER=2, TH=True, GATE=True, PR=16):
    G = TM // 8
    GP = G + PAD
    T = S // TM
    NS = 2 * T + 1
    NC = F // FC
    HM, HD, HF = TM // 2, D // 2, FC // 2

    def kern(x_h, wqkv_h, wo_h, w1_h, w3_h, w2_h, out_h,
             wqkv_r, wo_r, wp, w1, w3, w2, sem_a, sem_f,
             pbuf, qbuf, qkv_s, hk, hv, x_ref, o_ref, sem_io,
             wa_c, w1_c, w3_c, w2_c, x1c, x2c, oc, hc):

        def cp_qkv(j):
            return pltpu.make_async_copy(wqkv_h.at[:, pl.ds(pl.multiple_of(j * D, D), D)], wqkv_r.at[j], sem_a.at[j])

        cp_wo = pltpu.make_async_copy(wo_h, wo_r, sem_a.at[3])

        def cp_ffn(c):
            cols = pl.ds(pl.multiple_of(c * FC, FC), FC)
            return (pltpu.make_async_copy(w1_h.at[:, cols], w1.at[c], sem_f.at[0, c]),
                    pltpu.make_async_copy(w3_h.at[:, cols], w3.at[c], sem_f.at[1, c]),
                    pltpu.make_async_copy(w2_h.at[cols, :], w2.at[cols, :], sem_f.at[2, c]))

        def load_x():
            for c in range(8):
                for i in range(NB):
                    pbuf[i, GP * c:GP * c + G, :] = x_ref[G * c:G * (c + 1), 128 * i:128 * (i + 1)].astype(f32)

        def store_out():
            for c in range(8):
                for i in range(NB):
                    o_ref[G * c:G * (c + 1), 128 * i:128 * (i + 1)] = pbuf[i, GP * c:GP * c + G, :].astype(bf16)

        def prow(m):
            return pl.ds(8 * m, 8) if dbg & 2 else pl.ds(m, 8, stride=GP)

        def p_rows(m0, n):
            return jnp.concatenate(
                [jnp.concatenate([pbuf[i, prow(m0 + m), :] for i in range(NB)], axis=1) for m in range(n)], axis=0)

        def halo(s):
            l_att = (s >> 1) & 1
            fresh = jnp.logical_or(s == 0, s == 2)
            c0 = (lax.broadcasted_iota(jnp.int32, (HALO, D), 0) & 7) == 0
            for j, hal in ((1, hk), (2, hv)):
                cur = _roll_in_groups(qkv_s[j, TM:, :])
                prev = jnp.where(fresh, jnp.broadcast_to(qkv_s[j, HALO:HALO + 1, :], (HALO, D)), hal[l_att])
                qkv_s[j, 0:HALO, :] = jnp.where(c0, prev, cur)
                hal[l_att] = cur

        def attn_rows(s, r0, AR, ser=0):
            fresh = jnp.logical_or(s == 0, s == 2)
            static = isinstance(r0, int)
            scale = DH ** -0.5
            zero = (s >> 10) * 8
            def rows(w, z=0):
                b = HALO + r0 - SH * w + z
                return pl.ds(b if isinstance(b, int) else pl.multiple_of(b, 8), AR)
            q = [qkv_s[0, rows(0), 128 * i:128 * (i + 1)] for i in range(NB)]
            l = []
            for w in range(WIN):
                t = [q[i] * qkv_s[1, rows(w), 128 * i:128 * (i + 1)] for i in range(NB)]
                a = _tree(t)
                if ser and w % ser == ser - 1:
                    qkv_s[0, pl.ds(pl.multiple_of(zero, 8), AR), 0:128] = a
                a = a + pltpu.roll(a, 64, 1)
                a = a + pltpu.roll(a, 32, 1)
                a = a * scale
                if w > 0 and (not static or r0 < SH * w):
                    row = lax.broadcasted_iota(jnp.int32, (AR, 128), 0) + r0
                    bad = jnp.logical_and(jnp.logical_and(row < SH * w, (row & 7) == 0), fresh)
                    a = jnp.where(bad, -1e9, a)
                l.append(a)
            mx = functools.reduce(jnp.maximum, l)
            e = [jnp.exp(a - mx) for a in l]
            inv = 1.0 / _tree(e)
            p = [a * inv for a in e]
            for i in range(NB):
                cols = slice(128 * i, 128 * (i + 1))
                o = _tree([p[w] * qkv_s[2, rows(w), cols] for w in range(WIN)])
                qkv_s[0, rows(0, zero if ser and i % ser == ser - 1 else 0), cols] = o

        def finish(s, y):
            slot = s & 1
            for m in range(G):
                x2 = qbuf[1 - slot, 8 * m:8 * m + 8, :] + y[8 * m:8 * m + 8, :]
                for i in range(NB):
                    pbuf[i, prow(m), :] = x2[:, 128 * i:128 * (i + 1)]

        def prep(dst, get, rows):
            for r in range(0, rows, PR):
                blk = [get(i, j, r) for i in range(2) for j in range(2)]
                terms = _b_terms(*[v.astype(f32) for v in blk])
                for t in range(7):
                    dst(t, r, blk[0] if t == 1 else blk[3] if t == 4 else terms[t].astype(bf16))

        def prep_att(j):
            def dst(t, r, v):
                wa_c[j, t, r:r + PR, :] = v
            prep(dst, lambda a, b, r: wp[HD * a + r:HD * a + r + PR, HD * b:HD * (b + 1)], HD)

        def prep_up(c, w, wc):
            def dst(t, r, v):
                wc[c, t, r:r + PR, :] = v
            prep(dst, lambda a, b, r: w[c, HD * a + r:HD * a + r + PR, HF * b:HF * (b + 1)], HD)

        def prep_down(c):
            def dst(t, r, v):
                w2_c[t, pl.ds(pl.multiple_of(c * HF + r, PR), PR), :] = v
            prep(dst, lambda a, b, r: w2[pl.ds(pl.multiple_of(c * FC + HF * a + r, PR), PR), HD * b:HD * (b + 1)], HF)

        def put_terms(dst, r, top, bot):
            n = top.shape[0]
            for t, v in enumerate(_a_terms(top[:, :HD], top[:, HD:], bot[:, :HD], bot[:, HD:])):
                dst[t, r:r + n, :] = v.astype(bf16)

        def ln1_s():
            for m in range(0, G // 2, 2):
                put_terms(x1c, 8 * m, _ln(p_rows(m, 2)), _ln(p_rows(G // 2 + m, 2)))

        def proj_s(j):
            c11, c12, c21, c22 = _strassen(lambda t: _dot(x1c[t], wa_c[j, t]))
            qkv_s[j, HALO:HALO + HM, :HD] = c11
            qkv_s[j, HALO:HALO + HM, HD:] = c12
            qkv_s[j, HALO + HM:, :HD] = c21
            qkv_s[j, HALO + HM:, HD:] = c22

        def proj_ln2_s(s):
            slot = s & 1
            for r in range(0, HM, 16):
                put_terms(oc, r, qkv_s[0, HALO + r:HALO + r + 16, :], qkv_s[0, HALO + HM + r:HALO + HM + r + 16, :])
            c11, c12, c21, c22 = _strassen(lambda t: _dot(oc[t], wa_c[3, t]))
            for m in range(0, G // 2, 2):
                r = slice(8 * m, 8 * m + 16)
                top = p_rows(m, 2) + jnp.concatenate([c11[r], c12[r]], axis=1)
                bot = p_rows(G // 2 + m, 2) + jnp.concatenate([c21[r], c22[r]], axis=1)
                qbuf[slot, 8 * m:8 * m + 16, :] = top
                qbuf[slot, HM + 8 * m:HM + 8 * m + 16, :] = bot
                put_terms(x2c, 8 * m, _ln(top), _ln(bot))

        def gate_up(c, hook):
            g = _strassen(lambda t: hook(_dot(x2c[t], w1_c[c, t])))
            u = _strassen(lambda t: hook(_dot(x2c[t], w3_c[c, t])))
            h = [_swiglu(a, b, TH) for a, b in zip(g, u)]
            cols = pl.ds(HF * c if isinstance(c, int) else pl.multiple_of(HF * c, HF), HF)
            for t, v in enumerate(_a_terms(*h)):
                hc[t, :, cols] = v.astype(bf16)

        def down(s):
            c11, c12, c21, c22 = _strassen(lambda t: _dot(hc[t], w2_c[t]))
            finish(s, jnp.concatenate([jnp.concatenate([c11, c12], axis=1), jnp.concatenate([c21, c22], axis=1)], axis=0))

        def cp_x(t):
            return pltpu.make_async_copy(x_h.at[pl.ds(pl.multiple_of(t * TM, TM), TM), :], x_ref, sem_io.at[0])

        def cp_out(t):
            return pltpu.make_async_copy(o_ref, out_h.at[pl.ds(pl.multiple_of(t * TM, TM), TM), :], sem_io.at[1])

        def next_x(t):
            cp_x(t).wait()
            load_x()
            pl.when(t + 1 < T)(lambda: cp_x(t + 1).start())

        def start_ffn(cs):
            for c in ([] if dbg & 8 else cs):
                for cp in cp_ffn(c):
                    cp.start()

        def att_head(s):
            next_x(s)
            ln1_s()
            def body(j, carry):
                @pl.when(s == 0)
                def _():
                    cp_qkv(j).wait()
                    pl.when(j == 0)(lambda: cp_qkv(2).start())
                    pl.when(j == 1)(lambda: cp_wo.start())
                    pl.when(j == 2)(lambda: start_ffn([0]))
                    _permute_cols(wqkv_r, wp, j)
                    prep_att(j)
                proj_s(j)
                return carry
            lax.fori_loop(0, 3, body, 0)
            halo(s)
            lax.fori_loop(0, TM // ARL, lambda j, c: (attn_rows(s, j * ARL, ARL), c)[1], 0)

            @pl.when(s == 0)
            def _():
                cp_wo.wait()
                start_ffn(range(1, NC))
                _permute_rows(wo_r, wp)
                prep_att(3)

        def ffn_head(s):
            def body(c, carry):
                @pl.when(s == 1)
                def _():
                    for cp in cp_ffn(c):
                        cp.wait()
                    prep_up(c, w1, w1_c)
                    prep_up(c, w3, w3_c)
                    prep_down(c)
                gate_up(c, lambda v: v)
                return carry
            lax.fori_loop(0, NC, body, 0)

        def steady(s, carry):
            rows = list(range(0, TM, AR))
            zero = pl.multiple_of((s >> 10) * 8, 8)
            def gate(val):
                if GATE:
                    qkv_s[0, pl.ds(zero, 8), 0:128] = val[val.shape[0] - 8:, val.shape[1] - 128:]
            npt = 14 * (NC - PRE) - order
            pt = [0]
            def gated(val):
                j = pt[0]
                pt[0] += 1
                part = rows[len(rows) * j // npt:len(rows) * (j + 1) // npt]
                if part:
                    gate(val)
                    for r0 in part:
                        attn_rows(s, r0, AR, SER)
                return val
            for c in range(PRE):
                gate_up(c, lambda v: v)
            ln1_s()
            for j in range(3):
                proj_s(j)
            halo(s)
            for c in range(PRE, NC):
                gate_up(c, gated)
            proj_ln2_s(s)
            down(s)

            @pl.when(jnp.logical_or((s & 3) == 3, (s & 3) == 0))
            def _():
                t = (s - 2) >> 1
                pl.when(t > 0)(lambda: cp_out(t - 1).wait())
                store_out()
                cp_out(t).start()
                pl.when(t + 2 < T)(lambda: next_x(t + 2))
            return carry

        cp_x(0).start()
        cp_qkv(0).start()
        cp_qkv(1).start()
        hk[...] = jnp.zeros(hk.shape, f32)
        hv[...] = jnp.zeros(hv.shape, f32)

        def edge(p, carry):
            s = jnp.where(p == 2, NS - 1, p)
            pl.when(p < 2)(lambda: att_head(s))
            pl.when(p > 0)(lambda: ffn_head(s))
            pl.when(p < 2)(lambda: proj_ln2_s(s))
            pl.when(p > 0)(lambda: down(s))

            @pl.when(p == 1)
            def _():
                lax.fori_loop(2, nrun or (NS - 1), steady, 0)
            return carry
        lax.fori_loop(0, 3, edge, 0)
        if nrun is None:
            cp_out(T - 2).wait()
        else:
            cp_out(0).wait()
            cp_x(0).wait()
        store_out()
        cp_out(T - 1).start()
        cp_out(T - 1).wait()

    @jax.jit
    def fn(A_x, A_wqkv, A_wo, B_x, B_w1, B_w3, B_w2):
        x = A_x.reshape(S, D)
        anyspec = pl.BlockSpec(memory_space=pl.ANY)
        out = pl.pallas_call(
            kern,
            in_specs=[anyspec] * 6,
            out_specs=anyspec,
            out_shape=jax.ShapeDtypeStruct((S, D), bf16),
            scratch_shapes=[
                pltpu.VMEM((3, D, D), bf16), pltpu.VMEM((D, D), bf16), pltpu.VMEM((D, D), bf16),
                pltpu.VMEM((NC, D, FC), bf16), pltpu.VMEM((NC, D, FC), bf16), pltpu.VMEM((F, D), bf16),
                pltpu.SemaphoreType.DMA((4,)), pltpu.SemaphoreType.DMA((3, NC)),
                pltpu.VMEM((NB, 8 * GP, 128), f32), pltpu.VMEM((2, TM, D), f32),
                pltpu.VMEM((3, TM + HALO, D), f32),
                pltpu.VMEM((2, HALO, D), f32), pltpu.VMEM((2, HALO, D), f32),
                pltpu.VMEM((TM, D), bf16), pltpu.VMEM((TM, D), bf16), pltpu.SemaphoreType.DMA((2,)),
                pltpu.VMEM((4, 7, HD, HD), bf16), pltpu.VMEM((NC, 7, HD, HF), bf16), pltpu.VMEM((NC, 7, HD, HF), bf16),
                pltpu.VMEM((7, F // 2, HD), bf16),
                pltpu.VMEM((7, HM, HD), bf16), pltpu.VMEM((7, HM, HD), bf16), pltpu.VMEM((7, HM, HD), bf16),
                pltpu.VMEM((7, HM, F // 2), bf16),
            ],
            compiler_params=pltpu.CompilerParams(
                vmem_limit_bytes=120 * 1024 * 1024, flags=flags),
        )(x, A_wqkv, A_wo, B_w1, B_w3, B_w2)
        return out.reshape(1, S, D)
    return fn


_kernel = make()


def pallas_interleave_layers__sliding_local_dilated__glu_gated_swiglu__prompt_kernel(A_x, A_wqkv, A_wo, B_x, B_w1, B_w3, B_w2):
    return _kernel(A_x, A_wqkv, A_wo, B_x, B_w1, B_w3, B_w2)
```

```python
import functools
import jax
import jax.numpy as jnp
from jax import lax
import jax.experimental.pallas as pl
import jax.experimental.pallas.tpu as pltpu

S, D, H, DH, WIN, DIL, F = 2048, 1024, 32, 32, 8, 2, 3584
NB = D // 128
SH = 8 * DIL
HALO = (WIN - 1) * SH
f32, bf16, u32 = jnp.float32, jnp.bfloat16, jnp.uint32


def _dot(a, b):
    return jnp.dot(a, b, preferred_element_type=f32)


def _ln(x):
    m = jnp.mean(x, axis=-1, keepdims=True)
    xc = x - m
    v = jnp.mean(xc * xc, axis=-1, keepdims=True)
    return xc * lax.rsqrt(v + 1e-5)


def _swiglu(g, u, th):
    if th:
        hg = 0.5 * g
        return (hg + hg * jnp.tanh(hg)) * u
    return g * jax.nn.sigmoid(g) * u


def _tree(t):
    while len(t) > 1:
        t = [t[j] + t[j + 1] for j in range(0, len(t), 2)]
    return t[0]


def _pack(v):
    return pltpu.bitcast(v.astype(bf16), jnp.uint32)


def _pdot(a, b):
    return _dot(pltpu.bitcast(a, bf16), pltpu.bitcast(b, bf16))


def _a_terms(a11, a12, a21, a22):
    return (a11 + a22, a21 + a22, a11, a22, a11 + a12, a21 - a11, a12 - a22)


def _b_terms(b11, b12, b21, b22):
    return (b11 + b22, b11, b12 - b22, b21 - b11, b22, b11 + b12, b21 + b22)


def _strassen(prod):
    m1 = prod(0)
    m2 = prod(1)
    t22 = m1 - m2
    m4 = prod(3)
    c21 = m2 + m4
    t11 = m1 + m4 + prod(6)
    m5 = prod(4)
    c11 = t11 - m5
    m3 = prod(2)
    c12 = m3 + m5
    c22 = t22 + m3 + prod(5)
    return c11, c12, c21, c22


def _dst(src, i):
    g = (src >> 2) & 7
    return (src & 3) * 32 + (g ^ i) * 4 + (src >> 5)


def _butterfly(blocks, g):
    for b in range(3):
        m = ((g >> b) & 1) == 1
        blocks = [jnp.where(m, blocks[j ^ (1 << b)], blocks[j]) for j in range(NB)]
    return blocks


def _prep_proj(src, dst, it):
    RC, HD = 128, D // 2
    r = lax.broadcasted_iota(jnp.int32, (128, 128), 0)
    c = lax.broadcasted_iota(jnp.int32, (128, 128), 1)
    g = (lax.broadcasted_iota(jnp.int32, (RC, 128), 1) >> 2) & 7
    top, bot = (pl.ds(pl.multiple_of(h + it * RC, RC), RC) for h in (0, HD))
    blocks = [pltpu.bitcast(jnp.concatenate([src[top, 128 * b:128 * (b + 1)], src[bot, 128 * b:128 * (b + 1)]], axis=0), u32)
              for b in range(NB)]
    blocks = _butterfly(blocks, g)

    def perm(i):
        p = jnp.where(c == _dst(r, i), 1.0, 0.0).astype(bf16)
        return _dot(pltpu.bitcast(blocks[i], bf16), p)

    rows = pl.ds(pl.multiple_of(it * (RC // 2), RC // 2), RC // 2)
    for i in range(NB // 2):
        lo, hi = perm(i), perm(i + NB // 2)
        for t, v in enumerate(_b_terms(lo[:RC], hi[:RC], lo[RC:], hi[RC:])):
            dst[t, rows, 128 * i:128 * (i + 1)] = _pack(v)


def _prep_out(src, dst, it):
    CC, HD = 128, D // 2
    r = lax.broadcasted_iota(jnp.int32, (128, 128), 0)
    c = lax.broadcasted_iota(jnp.int32, (128, 128), 1)
    g = (lax.broadcasted_iota(jnp.int32, (64, 2 * CC), 0) >> 1) & 7
    left, right = (pl.ds(pl.multiple_of(h + it * CC, CC), CC) for h in (0, HD))
    blocks = [pltpu.bitcast(jnp.concatenate([src[128 * b:128 * (b + 1), left], src[128 * b:128 * (b + 1), right]], axis=1), u32)
              for b in range(NB)]
    blocks = _butterfly(blocks, g)

    def perm(i):
        pt = jnp.where(r == _dst(c, i), 1.0, 0.0).astype(bf16)
        return _dot(pt, pltpu.bitcast(blocks[i], bf16))

    for i in range(NB // 2):
        up, dn = perm(i), perm(i + NB // 2)
        for t, v in enumerate(_b_terms(up[:, :CC], up[:, CC:], dn[:, :CC], dn[:, CC:])):
            dst[t, 64 * i:64 * (i + 1), left] = _pack(v)


def _roll_in_groups(x):
    n = x.shape[0] // 8
    return pltpu.roll(x.reshape(n, 8, x.shape[1]), 1, 1).reshape(x.shape)


def make(TM=128, FC=512, AR=8, PRE=1, PAD=1, flags=None, SUB=2, order=12, nrun=None, FS=256, dbg=0, ARL=32, SER=2, TH=True, GATE=True, PR=16):
    G = TM // 8
    GP = G + PAD
    T = S // TM
    NS = 2 * T + 1
    NC = F // FC
    ln = (lambda v: v) if dbg & 16 else _ln
    HM, HD, HF = TM // 2, D // 2, FC // 2

    def kern(x_h, wqkv_h, wo_h, w1_h, w3_h, w2_h, out_h,
             wqkv_r, wo_r, w1, w3, w2, sem_a, sem_f,
             pbuf, qbuf, qkv_s, hk, hv, x_ref, o_ref, sem_io,
             wa_c, w1_c, w3_c, w2_c, x1c, x2c, oc, hc):

        def cp_qkv(j, it):
            cols = pl.ds(pl.multiple_of(j * D, D), D)
            rows = [pl.ds(pl.multiple_of(h + it * 128, 128), 128) for h in (0, HD)]
            return [pltpu.make_async_copy(wqkv_h.at[r, cols], wqkv_r.at[j, r], sem_a.at[j, it]) for r in rows]

        def start_qkv(j):
            for it in range(4):
                for cp in cp_qkv(j, it):
                    cp.start()

        cp_wo = pltpu.make_async_copy(wo_h, wo_r, sem_a.at[3, 0])

        def cp_ffn(c):
            cols = pl.ds(pl.multiple_of(c * FC, FC), FC)
            return (pltpu.make_async_copy(w1_h.at[:, cols], w1.at[c], sem_f.at[0, c]),
                    pltpu.make_async_copy(w3_h.at[:, cols], w3.at[c], sem_f.at[1, c]),
                    pltpu.make_async_copy(w2_h.at[cols, :], w2.at[cols, :], sem_f.at[2, c]))

        def load_x():
            for c in range(8):
                for i in range(NB):
                    pbuf[i, GP * c:GP * c + G, :] = x_ref[G * c:G * (c + 1), 128 * i:128 * (i + 1)].astype(f32)

        def store_out():
            for c in range(8):
                for i in range(NB):
                    o_ref[G * c:G * (c + 1), 128 * i:128 * (i + 1)] = pbuf[i, GP * c:GP * c + G, :].astype(bf16)

        def prow(m):
            return pl.ds(8 * m, 8) if dbg & 2 else pl.ds(m, 8, stride=GP)

        def p_rows(m0, n):
            return jnp.concatenate(
                [jnp.concatenate([pbuf[i, prow(m0 + m), :] for i in range(NB)], axis=1) for m in range(n)], axis=0)

        def halo(s):
            l_att = (s >> 1) & 1
            fresh = jnp.logical_or(s == 0, s == 2)
            c0 = (lax.broadcasted_iota(jnp.int32, (HALO, D), 0) & 7) == 0
            for j, hal in ((1, hk), (2, hv)):
                cur = _roll_in_groups(qkv_s[j, TM:, :])
                prev = jnp.where(fresh, jnp.broadcast_to(qkv_s[j, HALO:HALO + 1, :], (HALO, D)), hal[l_att])
                qkv_s[j, 0:HALO, :] = jnp.where(c0, prev, cur)
                hal[l_att] = cur

        def attn_rows(s, r0, AR, ser=0):
            fresh = jnp.logical_or(s == 0, s == 2)
            static = isinstance(r0, int)
            scale = DH ** -0.5
            zero = (s >> 10) * 8
            def rows(w, z=0):
                b = HALO + r0 - SH * w + z
                return pl.ds(b if isinstance(b, int) else pl.multiple_of(b, 8), AR)
            q = [qkv_s[0, rows(0), 128 * i:128 * (i + 1)] for i in range(NB)]
            l = []
            for w in range(WIN):
                t = [q[i] * qkv_s[1, rows(w), 128 * i:128 * (i + 1)] for i in range(NB)]
                a = _tree(t)
                if ser and w % ser == ser - 1:
                    qkv_s[0, pl.ds(pl.multiple_of(zero, 8), AR), 0:128] = a
                a = a + pltpu.roll(a, 64, 1)
                a = a + pltpu.roll(a, 32, 1)
                a = a * scale
                if w > 0 and (not static or r0 < SH * w):
                    row = lax.broadcasted_iota(jnp.int32, (AR, 128), 0) + r0
                    bad = jnp.logical_and(jnp.logical_and(row < SH * w, (row & 7) == 0), fresh)
                    a = jnp.where(bad, -1e9, a)
                l.append(a)
            mx = functools.reduce(jnp.maximum, l)
            e = [jnp.exp(a - mx) for a in l]
            inv = 1.0 / _tree(e)
            p = [a * inv for a in e]
            for i in range(NB):
                cols = slice(128 * i, 128 * (i + 1))
                o = _tree([p[w] * qkv_s[2, rows(w), cols] for w in range(WIN)])
                qkv_s[0, rows(0, zero if ser and i % ser == ser - 1 else 0), cols] = o

        def finish(s, y):
            slot = s & 1
            for m in range(G):
                x2 = qbuf[1 - slot, 8 * m:8 * m + 8, :] + y[8 * m:8 * m + 8, :]
                for i in range(NB):
                    pbuf[i, prow(m), :] = x2[:, 128 * i:128 * (i + 1)]

        def prep(dst, get, rows):
            for r in range(0, rows, PR):
                blk = [get(i, j, r) for i in range(2) for j in range(2)]
                terms = _b_terms(*[v.astype(f32) for v in blk])
                for t in range(7):
                    dst(t, r // 2, _pack(blk[0] if t == 1 else blk[3] if t == 4 else terms[t]))

        def prep_up(c, w, wc):
            def dst(t, r, v):
                wc[c, t, r:r + PR // 2, :] = v
            prep(dst, lambda a, b, r: w[c, HD * a + r:HD * a + r + PR, HF * b:HF * (b + 1)], HD)

        def prep_down(c):
            def dst(t, r, v):
                w2_c[t, pl.ds(pl.multiple_of(c * (HF // 2) + r, PR // 2), PR // 2), :] = v
            prep(dst, lambda a, b, r: w2[pl.ds(pl.multiple_of(c * FC + HF * a + r, PR), PR), HD * b:HD * (b + 1)], HF)

        def put_terms(dst, r, top, bot):
            n = top.shape[0]
            for t, v in enumerate(_a_terms(top[:, :HD], top[:, HD:], bot[:, :HD], bot[:, HD:])):
                dst[t, r // 2:(r + n) // 2, :] = _pack(v)

        def ln1_s():
            for m in range(0, G // 2, 2):
                put_terms(x1c, 8 * m, ln(p_rows(m, 2)), ln(p_rows(G // 2 + m, 2)))

        def proj_s(j):
            c11, c12, c21, c22 = _strassen(lambda t: _pdot(x1c[t], wa_c[j, t]))
            qkv_s[j, HALO:HALO + HM, :HD] = c11
            qkv_s[j, HALO:HALO + HM, HD:] = c12
            qkv_s[j, HALO + HM:, :HD] = c21
            qkv_s[j, HALO + HM:, HD:] = c22

        def proj_ln2_s(s):
            slot = s & 1
            for r in range(0, HM, 16):
                put_terms(oc, r, qkv_s[0, HALO + r:HALO + r + 16, :], qkv_s[0, HALO + HM + r:HALO + HM + r + 16, :])
            c11, c12, c21, c22 = _strassen(lambda t: _pdot(oc[t], wa_c[3, t]))
            for m in range(0, G // 2, 2):
                r = slice(8 * m, 8 * m + 16)
                top = p_rows(m, 2) + jnp.concatenate([c11[r], c12[r]], axis=1)
                bot = p_rows(G // 2 + m, 2) + jnp.concatenate([c21[r], c22[r]], axis=1)
                qbuf[slot, 8 * m:8 * m + 16, :] = top
                qbuf[slot, HM + 8 * m:HM + 8 * m + 16, :] = bot
                put_terms(x2c, 8 * m, ln(top), ln(bot))

        def gate_up(c, hook):
            g = _strassen(lambda t: hook(_pdot(x2c[t], w1_c[c, t])))
            u = _strassen(lambda t: hook(_pdot(x2c[t], w3_c[c, t])))
            h = [a + b if dbg & 64 else _swiglu(a, b, TH) for a, b in zip(g, u)]
            cols = pl.ds(HF * c if isinstance(c, int) else pl.multiple_of(HF * c, HF), HF)
            for t, v in enumerate(_a_terms(*h)):
                hc[t, :, cols] = _pack(v)

        def down(s):
            c11, c12, c21, c22 = _strassen(lambda t: _pdot(hc[t], w2_c[t]))
            finish(s, jnp.concatenate([jnp.concatenate([c11, c12], axis=1), jnp.concatenate([c21, c22], axis=1)], axis=0))

        def cp_x(t):
            return pltpu.make_async_copy(x_h.at[pl.ds(pl.multiple_of(t * TM, TM), TM), :], x_ref, sem_io.at[0])

        def cp_out(t):
            return pltpu.make_async_copy(o_ref, out_h.at[pl.ds(pl.multiple_of(t * TM, TM), TM), :], sem_io.at[1])

        def next_x(t):
            cp_x(t).wait()
            load_x()
            pl.when(t + 1 < T)(lambda: cp_x(t + 1).start())

        def start_ffn(cs):
            for c in cs:
                for cp in cp_ffn(c):
                    cp.start()

        def att_head(s):
            next_x(s)
            ln1_s()
            def body(j, carry):
                @pl.when(s == 0)
                def _():
                    def strip(it, carry):
                        for cp in cp_qkv(j, it):
                            cp.wait()

                        @pl.when(it == 1)
                        def _():
                            pl.when(j < 2)(lambda: start_qkv(j + 1))
                            pl.when(j == 1)(lambda: cp_wo.start())
                            pl.when(j == 2)(lambda: start_ffn([0]))
                        _prep_proj(wqkv_r.at[j], wa_c.at[j], it)
                        return carry
                    lax.fori_loop(0, 4, strip, 0)
                proj_s(j)
                return carry
            lax.fori_loop(0, 3, body, 0)
            halo(s)
            lax.fori_loop(0, TM // ARL, lambda j, c: (attn_rows(s, j * ARL, ARL), c)[1], 0)

            @pl.when(s == 0)
            def _():
                cp_wo.wait()
                start_ffn(range(1, NC))
                lax.fori_loop(0, 4, lambda it, c: (_prep_out(wo_r, wa_c.at[3], it), c)[1], 0)

        def ffn_head(s):
            def body(c, carry):
                @pl.when(s == 1)
                def _():
                    for cp in cp_ffn(c):
                        cp.wait()
                    prep_up(c, w1, w1_c)
                    prep_up(c, w3, w3_c)
                    prep_down(c)
                gate_up(c, lambda v: v)
                return carry
            lax.fori_loop(0, NC, body, 0)

        def steady(s, carry):
            rows = list(range(0, TM, AR))
            zero = pl.multiple_of((s >> 10) * 8, 8)
            def gate(val):
                if GATE:
                    qkv_s[0, pl.ds(zero, 8), 0:128] = val[val.shape[0] - 8:, val.shape[1] - 128:]
            npt = 14 * (NC - PRE) - order
            pt = [0]
            def gated(val):
                j = pt[0]
                pt[0] += 1
                part = rows[len(rows) * j // npt:len(rows) * (j + 1) // npt]
                if part:
                    gate(val)
                    for r0 in ([] if dbg & 4 else part):
                        attn_rows(s, r0, AR, SER)
                return val
            for c in range(PRE):
                gate_up(c, lambda v: v)
            ln1_s()
            for j in range(3):
                proj_s(j)
            if not dbg & 32:
                halo(s)
            for c in range(PRE, NC):
                gate_up(c, gated)
            proj_ln2_s(s)
            down(s)

            @pl.when(jnp.logical_or((s & 3) == 3, (s & 3) == 0))
            def _():
                t = (s - 2) >> 1
                pl.when(t > 0)(lambda: cp_out(t - 1).wait())
                store_out()
                cp_out(t).start()
                pl.when(t + 2 < T)(lambda: next_x(t + 2))
            return carry

        cp_x(0).start()
        start_qkv(0)
        hk[...] = jnp.zeros(hk.shape, f32)
        hv[...] = jnp.zeros(hv.shape, f32)

        def edge(p, carry):
            s = jnp.where(p == 2, NS - 1, p)
            pl.when(p < 2)(lambda: att_head(s))
            pl.when(p > 0)(lambda: ffn_head(s))
            pl.when(p < 2)(lambda: proj_ln2_s(s))
            pl.when(p > 0)(lambda: down(s))

            @pl.when(p == 1)
            def _():
                lax.fori_loop(2, nrun or (NS - 1), steady, 0)
            return carry
        lax.fori_loop(0, 3, edge, 0)
        if nrun is None:
            cp_out(T - 2).wait()
        else:
            cp_out(0).wait()
            cp_x(0).wait()
        store_out()
        cp_out(T - 1).start()
        cp_out(T - 1).wait()

    @jax.jit
    def fn(A_x, A_wqkv, A_wo, B_x, B_w1, B_w3, B_w2):
        x = A_x.reshape(S, D)
        anyspec = pl.BlockSpec(memory_space=pl.ANY)
        out = pl.pallas_call(
            kern,
            in_specs=[anyspec] * 6,
            out_specs=anyspec,
            out_shape=jax.ShapeDtypeStruct((S, D), bf16),
            scratch_shapes=[
                pltpu.VMEM((3, D, D), bf16), pltpu.VMEM((D, D), bf16),
                pltpu.VMEM((NC, D, FC), bf16), pltpu.VMEM((NC, D, FC), bf16), pltpu.VMEM((F, D), bf16),
                pltpu.SemaphoreType.DMA((4, 4)), pltpu.SemaphoreType.DMA((3, NC)),
                pltpu.VMEM((NB, 8 * GP, 128), f32), pltpu.VMEM((2, TM, D), f32),
                pltpu.VMEM((3, TM + HALO, D), f32),
                pltpu.VMEM((2, HALO, D), f32), pltpu.VMEM((2, HALO, D), f32),
                pltpu.VMEM((TM, D), bf16), pltpu.VMEM((TM, D), bf16), pltpu.SemaphoreType.DMA((2,)),
                pltpu.VMEM((4, 7, HD // 2, HD), u32), pltpu.VMEM((NC, 7, HD // 2, HF), u32), pltpu.VMEM((NC, 7, HD // 2, HF), u32),
                pltpu.VMEM((7, F // 4, HD), u32),
                pltpu.VMEM((7, HM // 2, HD), u32), pltpu.VMEM((7, HM // 2, HD), u32), pltpu.VMEM((7, HM // 2, HD), u32),
                pltpu.VMEM((7, HM // 2, F // 2), u32),
            ],
            compiler_params=pltpu.CompilerParams(
                vmem_limit_bytes=120 * 1024 * 1024, flags=flags),
        )(x, A_wqkv, A_wo, B_w1, B_w3, B_w2)
        return out.reshape(1, S, D)
    return fn


_kernel = make()


def pallas_interleave_layers__sliding_local_dilated__glu_gated_swiglu__prompt_kernel(A_x, A_wqkv, A_wo, B_x, B_w1, B_w3, B_w2):
    return _kernel(A_x, A_wqkv, A_wo, B_x, B_w1, B_w3, B_w2)
```

```python
import functools
import jax
import jax.numpy as jnp
from jax import lax
import jax.experimental.pallas as pl
import jax.experimental.pallas.tpu as pltpu

S, D, H, DH, WIN, DIL, F = 2048, 1024, 32, 32, 8, 2, 3584
NB = D // 128
SH = 8 * DIL
HALO = (WIN - 1) * SH
f32, bf16, u32 = jnp.float32, jnp.bfloat16, jnp.uint32


def _dot(a, b):
    return jnp.dot(a, b, preferred_element_type=f32)


def _ln(x):
    m = jnp.mean(x, axis=-1, keepdims=True)
    xc = x - m
    v = jnp.mean(xc * xc, axis=-1, keepdims=True)
    return xc * lax.rsqrt(v + 1e-5)


def _swiglu(g, u, th):
    if th:
        hg = 0.5 * g
        return (hg + hg * jnp.tanh(hg)) * u
    return g * jax.nn.sigmoid(g) * u


def _tree(t):
    while len(t) > 1:
        t = [t[j] + t[j + 1] for j in range(0, len(t), 2)]
    return t[0]


def _pack(v):
    return pltpu.bitcast(v.astype(bf16), jnp.uint32)


def _pdot(a, b):
    return _dot(a, pltpu.bitcast(b, bf16))


def _a_terms(a11, a12, a21, a22):
    return (a11 + a22, a21 + a22, a11, a22, a11 + a12, a21 - a11, a12 - a22)


def _b_terms(b11, b12, b21, b22):
    return (b11 + b22, b11, b12 - b22, b21 - b11, b22, b11 + b12, b21 + b22)


def _strassen(prod):
    m1 = prod(0)
    m2 = prod(1)
    t22 = m1 - m2
    m4 = prod(3)
    c21 = m2 + m4
    t11 = m1 + m4 + prod(6)
    m5 = prod(4)
    c11 = t11 - m5
    m3 = prod(2)
    c12 = m3 + m5
    c22 = t22 + m3 + prod(5)
    return c11, c12, c21, c22


def _dst(src, i):
    g = (src >> 2) & 7
    return (src & 3) * 32 + (g ^ i) * 4 + (src >> 5)


def _butterfly(blocks, g):
    for b in range(3):
        m = ((g >> b) & 1) == 1
        blocks = [jnp.where(m, blocks[j ^ (1 << b)], blocks[j]) for j in range(NB)]
    return blocks


def _prep_proj(src, dst, it):
    RC, HD = 128, D // 2
    r = lax.broadcasted_iota(jnp.int32, (128, 128), 0)
    c = lax.broadcasted_iota(jnp.int32, (128, 128), 1)
    g = (lax.broadcasted_iota(jnp.int32, (RC, 128), 1) >> 2) & 7
    top, bot = (pl.ds(pl.multiple_of(h + it * RC, RC), RC) for h in (0, HD))
    blocks = [pltpu.bitcast(jnp.concatenate([src[top, 128 * b:128 * (b + 1)], src[bot, 128 * b:128 * (b + 1)]], axis=0), u32)
              for b in range(NB)]
    blocks = _butterfly(blocks, g)

    def perm(i):
        p = jnp.where(c == _dst(r, i), 1.0, 0.0).astype(bf16)
        return _dot(pltpu.bitcast(blocks[i], bf16), p)

    rows = pl.ds(pl.multiple_of(it * (RC // 2), RC // 2), RC // 2)
    for i in range(NB // 2):
        lo, hi = perm(i), perm(i + NB // 2)
        for t, v in enumerate(_b_terms(lo[:RC], hi[:RC], lo[RC:], hi[RC:])):
            dst[t, rows, 128 * i:128 * (i + 1)] = _pack(v)


def _prep_out(src, dst, it):
    CC, HD = 128, D // 2
    r = lax.broadcasted_iota(jnp.int32, (128, 128), 0)
    c = lax.broadcasted_iota(jnp.int32, (128, 128), 1)
    g = (lax.broadcasted_iota(jnp.int32, (64, 2 * CC), 0) >> 1) & 7
    left, right = (pl.ds(pl.multiple_of(h + it * CC, CC), CC) for h in (0, HD))
    blocks = [pltpu.bitcast(jnp.concatenate([src[128 * b:128 * (b + 1), left], src[128 * b:128 * (b + 1), right]], axis=1), u32)
              for b in range(NB)]
    blocks = _butterfly(blocks, g)

    def perm(i):
        pt = jnp.where(r == _dst(c, i), 1.0, 0.0).astype(bf16)
        return _dot(pt, pltpu.bitcast(blocks[i], bf16))

    for i in range(NB // 2):
        up, dn = perm(i), perm(i + NB // 2)
        for t, v in enumerate(_b_terms(up[:, :CC], up[:, CC:], dn[:, :CC], dn[:, CC:])):
            dst[t, 64 * i:64 * (i + 1), left] = _pack(v)


def _roll_in_groups(x):
    n = x.shape[0] // 8
    return pltpu.roll(x.reshape(n, 8, x.shape[1]), 1, 1).reshape(x.shape)


def make(TM=128, FC=512, AR=8, PRE=1, PAD=1, flags=None, SUB=2, order=12, nrun=None, FS=256, dbg=0, ARL=32, SER=2, TH=True, GATE=True, PR=16, G1=2, G2=1, CUT=5, L2=0):
    G = TM // 8
    GP = G + PAD
    T = S // TM
    NS = 2 * T + 1
    NC = F // FC
    ln = (lambda v: v) if dbg & 16 else _ln
    HM, HD, HF = TM // 2, D // 2, FC // 2

    def kern(x_h, wqkv_h, wo_h, w1_h, w3_h, w2_h, out_h,
             wqkv_r, wo_r, w1, w3, w2, sem_a, sem_f,
             pbuf, qbuf, qkv_s, hk, hv, x_ref, o_ref, sem_io,
             wa_c, w1_c, w3_c, w2_c, x1c, x2c, oc, hc):

        def cp_qkv(j, it):
            cols = pl.ds(pl.multiple_of(j * D, D), D)
            rows = [pl.ds(pl.multiple_of(h + it * 128, 128), 128) for h in (0, HD)]
            return [pltpu.make_async_copy(wqkv_h.at[r, cols], wqkv_r.at[j, r], sem_a.at[j, it]) for r in rows]

        def start_qkv(j):
            for it in range(4):
                for cp in cp_qkv(j, it):
                    cp.start()

        cp_wo = pltpu.make_async_copy(wo_h, wo_r, sem_a.at[3, 0])

        def cp_ffn(c):
            cols = pl.ds(pl.multiple_of(c * FC, FC), FC)
            return (pltpu.make_async_copy(w1_h.at[:, cols], w1.at[c], sem_f.at[0, c]),
                    pltpu.make_async_copy(w3_h.at[:, cols], w3.at[c], sem_f.at[1, c]),
                    pltpu.make_async_copy(w2_h.at[cols, :], w2.at[cols, :], sem_f.at[2, c]))

        def load_x():
            for c in range(8):
                for i in range(NB):
                    pbuf[i, GP * c:GP * c + G, :] = x_ref[G * c:G * (c + 1), 128 * i:128 * (i + 1)].astype(f32)

        def store_out():
            for c in range(8):
                for i in range(NB):
                    o_ref[G * c:G * (c + 1), 128 * i:128 * (i + 1)] = pbuf[i, GP * c:GP * c + G, :].astype(bf16)

        def prow(m):
            return pl.ds(8 * m, 8) if dbg & 2 else pl.ds(m, 8, stride=GP)

        def p_rows(m0, n):
            return jnp.concatenate(
                [jnp.concatenate([pbuf[i, prow(m0 + m), :] for i in range(NB)], axis=1) for m in range(n)], axis=0)

        def halo(s, j, r0, n):
            layer = (s >> 1) & 1
            hal = hk if j == 1 else hv
            cur = _roll_in_groups(qkv_s[j, TM + r0:TM + r0 + n, :])
            prev = hal[layer, r0:r0 + n, :]
            if j == 2:
                fresh = jnp.logical_or(s == 0, s == 2)
                prev = jnp.where(fresh, jnp.broadcast_to(qkv_s[j, HALO:HALO + 1, :], (n, D)), prev)
            c0 = (lax.broadcasted_iota(jnp.int32, (n, D), 0) & 7) == 0
            qkv_s[j, r0:r0 + n, :] = jnp.where(c0, prev, cur)
            hal[layer, r0:r0 + n, :] = cur

        def attn_rows(s, r0, AR, ser=0):
            fresh = jnp.logical_or(s == 0, s == 2)
            static = isinstance(r0, int)
            scale = DH ** -0.5
            zero = (s >> 10) * 8
            def rows(w, z=0):
                b = HALO + r0 - SH * w + z
                return pl.ds(b if isinstance(b, int) else pl.multiple_of(b, 8), AR)
            q = [qkv_s[0, rows(0), 128 * i:128 * (i + 1)] for i in range(NB)]
            l = []
            for w in range(WIN):
                t = [q[i] * qkv_s[1, rows(w), 128 * i:128 * (i + 1)] for i in range(NB)]
                a = _tree(t)
                if ser and w % ser == ser - 1:
                    qkv_s[0, pl.ds(pl.multiple_of(zero, 8), AR), 0:128] = a
                a = a + pltpu.roll(a, 64, 1)
                a = a + pltpu.roll(a, 32, 1)
                a = a * scale
                if w > 0 and (not static or r0 < SH * w):
                    row = lax.broadcasted_iota(jnp.int32, (AR, 128), 0) + r0
                    bad = jnp.logical_and(jnp.logical_and(row < SH * w, (row & 7) == 0), fresh)
                    a = jnp.where(bad, -1e9, a)
                l.append(a)
                if w == WIN // 2 - 1 and CUT & 1:
                    yield
            yield
            mx = functools.reduce(jnp.maximum, l)
            e = [jnp.exp(a - mx) for a in l]
            inv = 1.0 / _tree(e)
            p = [a * inv for a in e]
            if CUT & 2:
                yield
            for i in range(NB):
                if i == NB // 2 and CUT & 4:
                    yield
                cols = slice(128 * i, 128 * (i + 1))
                o = _tree([p[w] * qkv_s[2, rows(w), cols] for w in range(WIN)])
                qkv_s[0, rows(0, zero if ser and i % ser == ser - 1 else 0), cols] = o

        def finish(s, y):
            slot = s & 1
            for m in range(G):
                x2 = qbuf[1 - slot, 8 * m:8 * m + 8, :] + y[8 * m:8 * m + 8, :]
                for i in range(NB):
                    pbuf[i, prow(m), :] = x2[:, 128 * i:128 * (i + 1)]

        def prep(dst, get, rows):
            for r in range(0, rows, PR):
                blk = [pltpu.bitcast(get(i, j, r), u32) for i in range(2) for j in range(2)]
                even, odd = (_b_terms(*[pltpu.unpack_elementwise(v, index=h, packed_dtype=bf16, unpacked_dtype=f32) for v in blk])
                             for h in range(2))
                for t in range(7):
                    both = lambda: pltpu.pack_elementwise([even[t], odd[t]], packed_dtype=bf16).astype(u32)
                    dst(t, r // 2, blk[0] if t == 1 else blk[3] if t == 4 else both())

        def prep_up(c, w, wc):
            def dst(t, r, v):
                wc[c, t, r:r + PR // 2, :] = v
            prep(dst, lambda a, b, r: w[c, HD * a + r:HD * a + r + PR, HF * b:HF * (b + 1)], HD)

        def prep_down(c):
            def dst(t, r, v):
                w2_c[t, pl.ds(pl.multiple_of(c * (HF // 2) + r, PR // 2), PR // 2), :] = v
            prep(dst, lambda a, b, r: w2[pl.ds(pl.multiple_of(c * FC + HF * a + r, PR), PR), HD * b:HD * (b + 1)], HF)

        def put_terms(dst, r, top, bot):
            n = top.shape[0]
            for t, v in enumerate(_a_terms(top[:, :HD], top[:, HD:], bot[:, :HD], bot[:, HD:])):
                dst[t, r:r + n, :] = v.astype(bf16)

        def ln1(m):
            put_terms(x1c, 8 * m, ln(p_rows(m, 2)), ln(p_rows(G // 2 + m, 2)))

        def proj(j, hook):
            c11, c12, c21, c22 = _strassen(lambda t: hook(_pdot(x1c[t], wa_c[j, t])))
            qkv_s[j, HALO:HALO + HM, :HD] = c11
            qkv_s[j, HALO:HALO + HM, HD:] = c12
            qkv_s[j, HALO + HM:, :HD] = c21
            qkv_s[j, HALO + HM:, HD:] = c22

        def o_terms(r):
            put_terms(oc, r, qkv_s[0, HALO + r:HALO + r + 16, :], qkv_s[0, HALO + HM + r:HALO + HM + r + 16, :])

        def out_proj():
            return _strassen(lambda t: _pdot(oc[t], wa_c[3, t]))

        def ln2(s, z, m):
            c11, c12, c21, c22 = z
            r = slice(8 * m, 8 * m + 16)
            top = p_rows(m, 2) + jnp.concatenate([c11[r], c12[r]], axis=1)
            bot = p_rows(G // 2 + m, 2) + jnp.concatenate([c21[r], c22[r]], axis=1)
            qbuf[s & 1, r, :] = top
            qbuf[s & 1, HM + 8 * m:HM + 8 * m + 16, :] = bot
            put_terms(x2c, 8 * m, ln(top), ln(bot))

        def gate_up(c, hook):
            g = _strassen(lambda t: hook(_pdot(x2c[t], w1_c[c, t])))
            u = _strassen(lambda t: hook(_pdot(x2c[t], w3_c[c, t])))
            h = [a + b if dbg & 64 else _swiglu(a, b, TH) for a, b in zip(g, u)]
            cols = pl.ds(HF * c if isinstance(c, int) else pl.multiple_of(HF * c, HF), HF)
            for t, v in enumerate(_a_terms(*h)):
                hc[t, :, cols] = v.astype(bf16)

        def down(s, hook):
            c11, c12, c21, c22 = _strassen(lambda t: hook(_pdot(hc[t], w2_c[t])))
            finish(s, jnp.concatenate([jnp.concatenate([c11, c12], axis=1), jnp.concatenate([c21, c22], axis=1)], axis=0))

        def cp_x(t):
            return pltpu.make_async_copy(x_h.at[pl.ds(pl.multiple_of(t * TM, TM), TM), :], x_ref, sem_io.at[0])

        def cp_out(t):
            return pltpu.make_async_copy(o_ref, out_h.at[pl.ds(pl.multiple_of(t * TM, TM), TM), :], sem_io.at[1])

        def next_x(t):
            cp_x(t).wait()
            load_x()
            pl.when(t + 1 < T)(lambda: cp_x(t + 1).start())

        def start_ffn(cs):
            for c in cs:
                for cp in cp_ffn(c):
                    cp.start()

        def att_head(s):
            next_x(s)
            for m in range(0, G // 2, 2):
                ln1(m)
            def body(j, carry):
                @pl.when(s == 0)
                def _():
                    def strip(it, carry):
                        for cp in cp_qkv(j, it):
                            cp.wait()

                        @pl.when(it == 1)
                        def _():
                            pl.when(j < 2)(lambda: start_qkv(j + 1))
                            pl.when(j == 1)(lambda: cp_wo.start())
                            pl.when(j == 2)(lambda: start_ffn([0]))
                        _prep_proj(wqkv_r.at[j], wa_c.at[j], it)
                        return carry
                    lax.fori_loop(0, 4, strip, 0)
                proj(j, lambda v: v)
                return carry
            lax.fori_loop(0, 3, body, 0)
            halo(s, 1, 0, HALO)
            halo(s, 2, 0, HALO)
            lax.fori_loop(0, TM // ARL, lambda j, c: (list(attn_rows(s, j * ARL, ARL)), c)[1], 0)

            @pl.when(s == 0)
            def _():
                cp_wo.wait()
                start_ffn(range(1, NC))
                lax.fori_loop(0, 4, lambda it, c: (_prep_out(wo_r, wa_c.at[3], it), c)[1], 0)

        def att_tail(s):
            for r in range(0, HM, 16):
                o_terms(r)
            z = out_proj()
            for m in range(0, G // 2, 2):
                ln2(s, z, m)

        def ffn_head(s):
            def body(c, carry):
                @pl.when(s == 1)
                def _():
                    for cp in cp_ffn(c):
                        cp.wait()
                    prep_up(c, w1, w1_c)
                    prep_up(c, w3, w3_c)
                    prep_down(c)
                gate_up(c, lambda v: v)
                return carry
            lax.fori_loop(0, NC, body, 0)

        def steady(s, carry):
            zero = pl.ds(pl.multiple_of((s >> 10) * 8, 8), 8)

            def after(buf, jobs):
                jobs = list(jobs)
                def hook(val):
                    job = jobs.pop(0) if jobs else None
                    if job is not None:
                        tail = val[HM - 8:, val.shape[1] - 128:]
                        if buf is pbuf:
                            pbuf[NB, zero, :] = tail
                        else:
                            qkv_s[0, zero, 0:128] = tail
                        job()
                    return val
                return hook, jobs

            def spaced(jobs, gap):
                return [x for job in jobs for x in [job] + [None] * (gap - 1)]

            P = functools.partial
            hook, left = after(pbuf, spaced([P(ln1, m) for m in range(0, G // 2, 2)], G1))
            for c in range(PRE):
                gate_up(c, hook)
            assert not any(left)
            proj(1, lambda v: v)
            hook, left = after(qkv_s, [P(halo, s, 1, r, SH) for r in range(0, HALO, SH)])
            proj(2, hook)
            hook, left = after(qkv_s, [P(halo, s, 2, r, SH) for r in range(0, HALO, SH)])
            proj(0, hook)
            jobs = []
            for r in range(0, HM, 16):
                for h in (r, HM + r):
                    for r0 in range(h, h + 16, AR):
                        gen = attn_rows(s, r0, AR, SER)
                        jobs += spaced([P(next, gen, None)] * (2 + bin(CUT).count("1")), G2)
                jobs += [P(o_terms, r)]
            hook, left = after(qkv_s, jobs)
            for c in range(PRE, NC):
                gate_up(c, hook)
            assert not any(left)
            z = out_proj()
            jobs = [P(ln2, s, z, m) for m in range(0, G // 2, 2)]
            if not L2:
                for job in jobs:
                    job()
            hook, left = after(pbuf, jobs if L2 else [])
            down(s, hook)

            @pl.when(jnp.logical_or((s & 3) == 3, (s & 3) == 0))
            def _():
                t = (s - 2) >> 1
                pl.when(t > 0)(lambda: cp_out(t - 1).wait())
                store_out()
                cp_out(t).start()
                pl.when(t + 2 < T)(lambda: next_x(t + 2))
            return carry

        cp_x(0).start()
        start_qkv(0)
        hk[...] = jnp.zeros(hk.shape, f32)
        hv[...] = jnp.zeros(hv.shape, f32)

        def edge(p, carry):
            s = jnp.where(p == 2, NS - 1, p)
            pl.when(p < 2)(lambda: att_head(s))
            pl.when(p > 0)(lambda: ffn_head(s))
            pl.when(p < 2)(lambda: att_tail(s))
            pl.when(p > 0)(lambda: down(s, lambda v: v))

            @pl.when(p == 1)
            def _():
                lax.fori_loop(2, nrun or (NS - 1), steady, 0)
            return carry
        lax.fori_loop(0, 3, edge, 0)
        if nrun is None:
            cp_out(T - 2).wait()
        else:
            cp_out(0).wait()
            cp_x(0).wait()
        store_out()
        cp_out(T - 1).start()
        cp_out(T - 1).wait()

    @jax.jit
    def fn(A_x, A_wqkv, A_wo, B_x, B_w1, B_w3, B_w2):
        x = A_x.reshape(S, D)
        anyspec = pl.BlockSpec(memory_space=pl.ANY)
        out = pl.pallas_call(
            kern,
            in_specs=[anyspec] * 6,
            out_specs=anyspec,
            out_shape=jax.ShapeDtypeStruct((S, D), bf16),
            scratch_shapes=[
                pltpu.VMEM((3, D, D), bf16), pltpu.VMEM((D, D), bf16),
                pltpu.VMEM((NC, D, FC), bf16), pltpu.VMEM((NC, D, FC), bf16), pltpu.VMEM((F, D), bf16),
                pltpu.SemaphoreType.DMA((4, 4)), pltpu.SemaphoreType.DMA((3, NC)),
                pltpu.VMEM((NB + 1, 8 * GP, 128), f32), pltpu.VMEM((2, TM, D), f32),
                pltpu.VMEM((3, TM + HALO, D), f32),
                pltpu.VMEM((2, HALO, D), f32), pltpu.VMEM((2, HALO, D), f32),
                pltpu.VMEM((TM, D), bf16), pltpu.VMEM((TM, D), bf16), pltpu.SemaphoreType.DMA((2,)),
                pltpu.VMEM((4, 7, HD // 2, HD), u32), pltpu.VMEM((NC, 7, HD // 2, HF), u32), pltpu.VMEM((NC, 7, HD // 2, HF), u32),
                pltpu.VMEM((7, F // 4, HD), u32),
                pltpu.VMEM((7, HM, HD), bf16), pltpu.VMEM((7, HM, HD), bf16), pltpu.VMEM((7, HM, HD), bf16),
                pltpu.VMEM((7, HM, F // 2), bf16),
            ],
            compiler_params=pltpu.CompilerParams(
                vmem_limit_bytes=120 * 1024 * 1024, flags=flags),
        )(x, A_wqkv, A_wo, B_w1, B_w3, B_w2)
        return out.reshape(1, S, D)
    return fn


_kernel = make()


def pallas_interleave_layers__sliding_local_dilated__glu_gated_swiglu__prompt_kernel(A_x, A_wqkv, A_wo, B_x, B_w1, B_w3, B_w2):
    return _kernel(A_x, A_wqkv, A_wo, B_x, B_w1, B_w3, B_w2)
```

```python
import functools
import jax
import jax.numpy as jnp
from jax import lax
import jax.experimental.pallas as pl
import jax.experimental.pallas.tpu as pltpu

S, D, H, DH, WIN, DIL, F = 2048, 1024, 32, 32, 8, 2, 3584
NB = D // 128
SH = 8 * DIL
HALO = (WIN - 1) * SH
f32, bf16, u32 = jnp.float32, jnp.bfloat16, jnp.uint32


def _dot(a, b):
    return jnp.dot(a, b, preferred_element_type=f32)


def _ln(x):
    m = jnp.mean(x, axis=-1, keepdims=True)
    xc = x - m
    v = jnp.mean(xc * xc, axis=-1, keepdims=True)
    return xc * lax.rsqrt(v + 1e-5)


def _swiglu(g, u, th):
    if th:
        hg = 0.5 * g
        return (hg + hg * jnp.tanh(hg)) * u
    return g * jax.nn.sigmoid(g) * u


def _tree(t):
    while len(t) > 1:
        t = [t[j] + t[j + 1] for j in range(0, len(t), 2)]
    return t[0]


def _pack(v):
    return pltpu.bitcast(v.astype(bf16), jnp.uint32)


def _pdot(a, b):
    return _dot(a, pltpu.bitcast(b, bf16))


def _a_terms(a11, a12, a21, a22):
    return (a11 + a22, a21 + a22, a11, a22, a11 + a12, a21 - a11, a12 - a22)


def _b_terms(b11, b12, b21, b22):
    return (b11 + b22, b11, b12 - b22, b21 - b11, b22, b11 + b12, b21 + b22)


def _strassen(prod):
    m1 = prod(0)
    m2 = prod(1)
    t22 = m1 - m2
    m4 = prod(3)
    c21 = m2 + m4
    t11 = m1 + m4 + prod(6)
    m5 = prod(4)
    c11 = t11 - m5
    m3 = prod(2)
    c12 = m3 + m5
    c22 = t22 + m3 + prod(5)
    return c11, c12, c21, c22


def _dst(src, i):
    g = (src >> 2) & 7
    return (src & 3) * 32 + (g ^ i) * 4 + (src >> 5)


def _butterfly(blocks, g):
    for b in range(3):
        m = ((g >> b) & 1) == 1
        blocks = [jnp.where(m, blocks[j ^ (1 << b)], blocks[j]) for j in range(NB)]
    return blocks


def _prep_proj(src, dst, it):
    RC, HD = 128, D // 2
    r = lax.broadcasted_iota(jnp.int32, (128, 128), 0)
    c = lax.broadcasted_iota(jnp.int32, (128, 128), 1)
    g = (lax.broadcasted_iota(jnp.int32, (RC, 128), 1) >> 2) & 7
    top, bot = (pl.ds(pl.multiple_of(h + it * RC, RC), RC) for h in (0, HD))
    blocks = [pltpu.bitcast(jnp.concatenate([src[top, 128 * b:128 * (b + 1)], src[bot, 128 * b:128 * (b + 1)]], axis=0), u32)
              for b in range(NB)]
    blocks = _butterfly(blocks, g)

    def perm(i):
        p = jnp.where(c == _dst(r, i), 1.0, 0.0).astype(bf16)
        return _dot(pltpu.bitcast(blocks[i], bf16), p)

    rows = pl.ds(pl.multiple_of(it * (RC // 2), RC // 2), RC // 2)
    for i in range(NB // 2):
        lo, hi = perm(i), perm(i + NB // 2)
        for t, v in enumerate(_b_terms(lo[:RC], hi[:RC], lo[RC:], hi[RC:])):
            dst[t, rows, 128 * i:128 * (i + 1)] = _pack(v)


def _prep_out(src, dst, it):
    CC, HD = 128, D // 2
    r = lax.broadcasted_iota(jnp.int32, (128, 128), 0)
    c = lax.broadcasted_iota(jnp.int32, (128, 128), 1)
    g = (lax.broadcasted_iota(jnp.int32, (64, 2 * CC), 0) >> 1) & 7
    left, right = (pl.ds(pl.multiple_of(h + it * CC, CC), CC) for h in (0, HD))
    blocks = [pltpu.bitcast(jnp.concatenate([src[128 * b:128 * (b + 1), left], src[128 * b:128 * (b + 1), right]], axis=1), u32)
              for b in range(NB)]
    blocks = _butterfly(blocks, g)

    def perm(i):
        pt = jnp.where(r == _dst(c, i), 1.0, 0.0).astype(bf16)
        return _dot(pt, pltpu.bitcast(blocks[i], bf16))

    for i in range(NB // 2):
        up, dn = perm(i), perm(i + NB // 2)
        for t, v in enumerate(_b_terms(up[:, :CC], up[:, CC:], dn[:, :CC], dn[:, CC:])):
            dst[t, 64 * i:64 * (i + 1), left] = _pack(v)


def _roll_in_groups(x):
    n = x.shape[0] // 8
    return pltpu.roll(x.reshape(n, 8, x.shape[1]), 1, 1).reshape(x.shape)


def make(TM=128, FC=512, AR=8, PRE=1, PAD=1, flags=None, SUB=2, order=12, nrun=None, FS=256, dbg=0, ARL=32, SER=2, TH=True, GATE=True, PR=16, G1=2, G2=1, CUT=7, L2=0, D0=0):
    G = TM // 8
    GP = G + PAD
    T = S // TM
    NS = 2 * T + 1
    NC = F // FC
    ln = (lambda v: v) if dbg & 16 else _ln
    HM, HD, HF = TM // 2, D // 2, FC // 2

    def kern(x_h, wqkv_h, wo_h, w1_h, w3_h, w2_h, out_h,
             wqkv_r, wo_r, w1, w3, w2, sem_a, sem_f,
             pbuf, qbuf, qkv_s, hk, hv, x_ref, o_ref, sem_io,
             wa_c, w1_c, w3_c, w2_c, x1c, x2c, oc, hc):

        def cp_qkv(j, it):
            cols = pl.ds(pl.multiple_of(j * D, D), D)
            rows = [pl.ds(pl.multiple_of(h + it * 128, 128), 128) for h in (0, HD)]
            return [pltpu.make_async_copy(wqkv_h.at[r, cols], wqkv_r.at[j, r], sem_a.at[j, it]) for r in rows]

        def start_qkv(j):
            for it in range(4):
                for cp in cp_qkv(j, it):
                    cp.start()

        cp_wo = pltpu.make_async_copy(wo_h, wo_r, sem_a.at[3, 0])

        def cp_ffn(c):
            cols = pl.ds(pl.multiple_of(c * FC, FC), FC)
            return (pltpu.make_async_copy(w1_h.at[:, cols], w1.at[c], sem_f.at[0, c]),
                    pltpu.make_async_copy(w3_h.at[:, cols], w3.at[c], sem_f.at[1, c]),
                    pltpu.make_async_copy(w2_h.at[cols, :], w2.at[cols, :], sem_f.at[2, c]))

        def load_x():
            for c in range(8):
                for i in range(NB):
                    pbuf[i, GP * c:GP * c + G, :] = x_ref[G * c:G * (c + 1), 128 * i:128 * (i + 1)].astype(f32)

        def store_out():
            for c in range(8):
                for i in range(NB):
                    o_ref[G * c:G * (c + 1), 128 * i:128 * (i + 1)] = pbuf[i, GP * c:GP * c + G, :].astype(bf16)

        def prow(m):
            return pl.ds(8 * m, 8) if dbg & 2 else pl.ds(m, 8, stride=GP)

        def p_rows(m0, n):
            return jnp.concatenate(
                [jnp.concatenate([pbuf[i, prow(m0 + m), :] for i in range(NB)], axis=1) for m in range(n)], axis=0)

        def halo(s, j, r0, n):
            layer = (s >> 1) & 1
            hal = hk if j == 1 else hv
            cur = _roll_in_groups(qkv_s[j, TM + r0:TM + r0 + n, :])
            prev = hal[layer, r0:r0 + n, :]
            if j == 2:
                fresh = jnp.logical_or(s == 0, s == 2)
                prev = jnp.where(fresh, jnp.broadcast_to(qkv_s[j, HALO:HALO + 1, :], (n, D)), prev)
            c0 = (lax.broadcasted_iota(jnp.int32, (n, D), 0) & 7) == 0
            qkv_s[j, r0:r0 + n, :] = jnp.where(c0, prev, cur)
            hal[layer, r0:r0 + n, :] = cur

        def attn_rows(s, r0, AR, ser=0):
            fresh = jnp.logical_or(s == 0, s == 2)
            static = isinstance(r0, int)
            scale = DH ** -0.5
            zero = (s >> 10) * 8
            def rows(w, z=0):
                b = HALO + r0 - SH * w + z
                return pl.ds(b if isinstance(b, int) else pl.multiple_of(b, 8), AR)
            q = [qkv_s[0, rows(0), 128 * i:128 * (i + 1)] for i in range(NB)]
            l = []
            for w in range(WIN):
                t = [q[i] * qkv_s[1, rows(w), 128 * i:128 * (i + 1)] for i in range(NB)]
                a = _tree(t)
                if ser and w % ser == ser - 1:
                    qkv_s[0, pl.ds(pl.multiple_of(zero, 8), AR), 0:128] = a
                a = a + pltpu.roll(a, 64, 1)
                a = a + pltpu.roll(a, 32, 1)
                a = a * scale
                if w > 0 and (not static or r0 < SH * w):
                    row = lax.broadcasted_iota(jnp.int32, (AR, 128), 0) + r0
                    bad = jnp.logical_and(jnp.logical_and(row < SH * w, (row & 7) == 0), fresh)
                    a = jnp.where(bad, -1e9, a)
                l.append(a)
                if w == WIN // 2 - 1 and CUT & 1:
                    yield
            yield
            mx = functools.reduce(jnp.maximum, l)
            e = [jnp.exp(a - mx) for a in l]
            inv = 1.0 / _tree(e)
            p = [a * inv for a in e]
            if CUT & 2:
                yield
            for i in range(NB):
                if i == NB // 2 and CUT & 4:
                    yield
                cols = slice(128 * i, 128 * (i + 1))
                o = _tree([p[w] * qkv_s[2, rows(w), cols] for w in range(WIN)])
                qkv_s[0, rows(0, zero if ser and i % ser == ser - 1 else 0), cols] = o

        def finish(s, y):
            slot = s & 1
            for m in range(G):
                x2 = qbuf[1 - slot, 8 * m:8 * m + 8, :] + y[8 * m:8 * m + 8, :]
                for i in range(NB):
                    pbuf[i, prow(m), :] = x2[:, 128 * i:128 * (i + 1)]

        def prep(dst, get, rows):
            for r in range(0, rows, PR):
                blk = [pltpu.bitcast(get(i, j, r), u32) for i in range(2) for j in range(2)]
                even, odd = (_b_terms(*[pltpu.unpack_elementwise(v, index=h, packed_dtype=bf16, unpacked_dtype=f32) for v in blk])
                             for h in range(2))
                for t in range(7):
                    both = lambda: pltpu.pack_elementwise([even[t], odd[t]], packed_dtype=bf16).astype(u32)
                    dst(t, r // 2, blk[0] if t == 1 else blk[3] if t == 4 else both())

        def prep_up(c, w, wc):
            def dst(t, r, v):
                wc[c, t, r:r + PR // 2, :] = v
            prep(dst, lambda a, b, r: w[c, HD * a + r:HD * a + r + PR, HF * b:HF * (b + 1)], HD)

        def prep_down(c):
            def dst(t, r, v):
                w2_c[t, pl.ds(pl.multiple_of(c * (HF // 2) + r, PR // 2), PR // 2), :] = v
            prep(dst, lambda a, b, r: w2[pl.ds(pl.multiple_of(c * FC + HF * a + r, PR), PR), HD * b:HD * (b + 1)], HF)

        def put_terms(dst, r, top, bot):
            n = top.shape[0]
            for t, v in enumerate(_a_terms(top[:, :HD], top[:, HD:], bot[:, :HD], bot[:, HD:])):
                dst[t, r:r + n, :] = v.astype(bf16)

        def ln1(m):
            put_terms(x1c, 8 * m, ln(p_rows(m, 2)), ln(p_rows(G // 2 + m, 2)))

        def proj(j, hook):
            c11, c12, c21, c22 = _strassen(lambda t: hook(_pdot(x1c[t], wa_c[j, t])))
            qkv_s[j, HALO:HALO + HM, :HD] = c11
            qkv_s[j, HALO:HALO + HM, HD:] = c12
            qkv_s[j, HALO + HM:, :HD] = c21
            qkv_s[j, HALO + HM:, HD:] = c22

        def o_terms(r):
            put_terms(oc, r, qkv_s[0, HALO + r:HALO + r + 16, :], qkv_s[0, HALO + HM + r:HALO + HM + r + 16, :])

        def out_proj():
            return _strassen(lambda t: _pdot(oc[t], wa_c[3, t]))

        def ln2(s, z, m):
            c11, c12, c21, c22 = z
            r = slice(8 * m, 8 * m + 16)
            top = p_rows(m, 2) + jnp.concatenate([c11[r], c12[r]], axis=1)
            bot = p_rows(G // 2 + m, 2) + jnp.concatenate([c21[r], c22[r]], axis=1)
            qbuf[s & 1, r, :] = top
            qbuf[s & 1, HM + 8 * m:HM + 8 * m + 16, :] = bot
            put_terms(x2c, 8 * m, ln(top), ln(bot))

        def resid(s, z, m):
            c11, c12, c21, c22 = z
            r = slice(8 * m, 8 * m + 16)
            qbuf[s & 1, r, :] = p_rows(m, 2) + jnp.concatenate([c11[r], c12[r]], axis=1)
            qbuf[s & 1, HM + 8 * m:HM + 8 * m + 16, :] = p_rows(G // 2 + m, 2) + jnp.concatenate([c21[r], c22[r]], axis=1)

        def norm2(s, m):
            put_terms(x2c, 8 * m, ln(qbuf[s & 1, 8 * m:8 * m + 16, :]), ln(qbuf[s & 1, HM + 8 * m:HM + 8 * m + 16, :]))

        def gate_up(c, hook):
            g = _strassen(lambda t: hook(_pdot(x2c[t], w1_c[c, t])))
            u = _strassen(lambda t: hook(_pdot(x2c[t], w3_c[c, t])))
            h = [a + b if dbg & 64 else _swiglu(a, b, TH) for a, b in zip(g, u)]
            cols = pl.ds(HF * c if isinstance(c, int) else pl.multiple_of(HF * c, HF), HF)
            for t, v in enumerate(_a_terms(*h)):
                hc[t, :, cols] = v.astype(bf16)

        def down(s, hook):
            c11, c12, c21, c22 = _strassen(lambda t: hook(_pdot(hc[t], w2_c[t])))
            finish(s, jnp.concatenate([jnp.concatenate([c11, c12], axis=1), jnp.concatenate([c21, c22], axis=1)], axis=0))

        def cp_x(t):
            return pltpu.make_async_copy(x_h.at[pl.ds(pl.multiple_of(t * TM, TM), TM), :], x_ref, sem_io.at[0])

        def cp_out(t):
            return pltpu.make_async_copy(o_ref, out_h.at[pl.ds(pl.multiple_of(t * TM, TM), TM), :], sem_io.at[1])

        def next_x(t):
            cp_x(t).wait()
            load_x()
            pl.when(t + 1 < T)(lambda: cp_x(t + 1).start())

        def start_ffn(cs):
            for c in cs:
                for cp in cp_ffn(c):
                    cp.start()

        def att_head(s):
            next_x(s)
            for m in range(0, G // 2, 2):
                ln1(m)
            def body(j, carry):
                @pl.when(s == 0)
                def _():
                    def strip(it, carry):
                        for cp in cp_qkv(j, it):
                            cp.wait()

                        n = 4 * j + it
                        pl.when(jnp.logical_or(n == 0, n == 3))(lambda: start_qkv((n + 5) >> 2))
                        pl.when(n == 5)(lambda: cp_wo.start())
                        pl.when(jnp.logical_and(n >= 7, (n & 1) == 1))(lambda: start_ffn([(n - 7) >> 1]))
                        _prep_proj(wqkv_r.at[j], wa_c.at[j], it)
                        return carry
                    lax.fori_loop(0, 4, strip, 0)
                proj(j, lambda v: v)
                return carry
            pl.when(s == 1)(lambda: start_ffn([5]))
            lax.fori_loop(0, 3, body, 0)
            pl.when(s == 1)(lambda: start_ffn([6]))
            halo(s, 1, 0, HALO)
            halo(s, 2, 0, HALO)
            lax.fori_loop(0, TM // ARL, lambda j, c: (list(attn_rows(s, j * ARL, ARL)), c)[1], 0)

            @pl.when(s == 0)
            def _():
                cp_wo.wait()
                start_ffn([3])
                lax.fori_loop(0, 4, lambda it, c: (_prep_out(wo_r, wa_c.at[3], it), c)[1], 0)
                start_ffn([4])

        def att_tail(s):
            for r in range(0, HM, 16):
                o_terms(r)
            z = out_proj()
            for m in range(0, G // 2, 2):
                ln2(s, z, m)

        def ffn_head(s):
            def body(c, carry):
                @pl.when(s == 1)
                def _():
                    for cp in cp_ffn(c):
                        cp.wait()
                    prep_up(c, w1, w1_c)
                    prep_up(c, w3, w3_c)
                    prep_down(c)
                gate_up(c, lambda v: v)
                return carry
            lax.fori_loop(0, NC, body, 0)

        def steady(s, carry):
            zero = pl.ds(pl.multiple_of((s >> 10) * 8, 8), 8)

            def after(buf, jobs):
                jobs = list(jobs)
                def hook(val):
                    job = jobs.pop(0) if jobs else None
                    if job is not None:
                        tail = val[HM - 8:, val.shape[1] - 128:]
                        if buf is pbuf:
                            pbuf[NB, zero, :] = tail
                        elif buf is qbuf:
                            qbuf[2, zero, 0:128] = tail
                        else:
                            qkv_s[0, zero, 0:128] = tail
                        job()
                    return val
                return hook, jobs

            def spaced(jobs, gap):
                return [x for job in jobs for x in [job] + [None] * (gap - 1)]

            P = functools.partial
            hook, left = after(pbuf, spaced([P(ln1, m) for m in range(0, G // 2, 2)], G1))
            for c in range(PRE):
                gate_up(c, hook)
            assert not any(left)
            proj(1, lambda v: v)
            hook, left = after(qkv_s, [P(halo, s, 1, r, SH) for r in range(0, HALO, SH)])
            proj(2, hook)
            hook, left = after(qkv_s, [P(halo, s, 2, r, SH) for r in range(0, HALO, SH)])
            proj(0, hook)
            jobs = [None] * D0
            for r in range(0, HM, 16):
                for h in (r, HM + r):
                    for r0 in range(h, h + 16, AR):
                        gen = attn_rows(s, r0, AR, SER)
                        jobs += spaced([P(next, gen, None)] * (2 + bin(CUT).count("1")), G2)
                jobs += [P(o_terms, r)]
            hook, left = after(qkv_s, jobs)
            for c in range(PRE, NC):
                gate_up(c, hook)
            assert not any(left)
            z = out_proj()
            jobs = [P(ln2, s, z, m) for m in range(0, G // 2, 2)]
            if L2 >= 2:
                for m in range(0, G // 2, 2):
                    resid(s, z, m)
                jobs = [P(norm2, s, m) for m in range(0, G // 2, 2)]
                hook, left = after(qbuf, jobs if L2 == 2 else [])
                if L2 == 3:
                    for job in jobs:
                        job()
            elif not L2:
                for job in jobs:
                    job()
            if L2 < 2:
                hook, left = after(pbuf, jobs if L2 else [])
            down(s, hook)

            @pl.when(jnp.logical_or((s & 3) == 3, (s & 3) == 0))
            def _():
                t = (s - 2) >> 1
                pl.when(t > 0)(lambda: cp_out(t - 1).wait())
                store_out()
                cp_out(t).start()
                pl.when(t + 2 < T)(lambda: next_x(t + 2))
            return carry

        cp_x(0).start()
        start_qkv(0)
        hk[...] = jnp.zeros(hk.shape, f32)
        hv[...] = jnp.zeros(hv.shape, f32)

        def edge(p, carry):
            s = jnp.where(p == 2, NS - 1, p)
            pl.when(p < 2)(lambda: att_head(s))
            pl.when(p > 0)(lambda: ffn_head(s))
            pl.when(p < 2)(lambda: att_tail(s))
            pl.when(p > 0)(lambda: down(s, lambda v: v))

            @pl.when(p == 1)
            def _():
                lax.fori_loop(2, nrun or (NS - 1), steady, 0)
            return carry
        lax.fori_loop(0, 3, edge, 0)
        if nrun is None:
            cp_out(T - 2).wait()
        else:
            cp_out(0).wait()
            cp_x(0).wait()
        store_out()
        cp_out(T - 1).start()
        cp_out(T - 1).wait()

    @jax.jit
    def fn(A_x, A_wqkv, A_wo, B_x, B_w1, B_w3, B_w2):
        x = A_x.reshape(S, D)
        anyspec = pl.BlockSpec(memory_space=pl.ANY)
        out = pl.pallas_call(
            kern,
            in_specs=[anyspec] * 6,
            out_specs=anyspec,
            out_shape=jax.ShapeDtypeStruct((S, D), bf16),
            scratch_shapes=[
                pltpu.VMEM((3, D, D), bf16), pltpu.VMEM((D, D), bf16),
                pltpu.VMEM((NC, D, FC), bf16), pltpu.VMEM((NC, D, FC), bf16), pltpu.VMEM((F, D), bf16),
                pltpu.SemaphoreType.DMA((4, 4)), pltpu.SemaphoreType.DMA((3, NC)),
                pltpu.VMEM((NB + 1, 8 * GP, 128), f32), pltpu.VMEM((3, TM, D), f32),
                pltpu.VMEM((3, TM + HALO, D), f32),
                pltpu.VMEM((2, HALO, D), f32), pltpu.VMEM((2, HALO, D), f32),
                pltpu.VMEM((TM, D), bf16), pltpu.VMEM((TM, D), bf16), pltpu.SemaphoreType.DMA((2,)),
                pltpu.VMEM((4, 7, HD // 2, HD), u32), pltpu.VMEM((NC, 7, HD // 2, HF), u32), pltpu.VMEM((NC, 7, HD // 2, HF), u32),
                pltpu.VMEM((7, F // 4, HD), u32),
                pltpu.VMEM((7, HM, HD), bf16), pltpu.VMEM((7, HM, HD), bf16), pltpu.VMEM((7, HM, HD), bf16),
                pltpu.VMEM((7, HM, F // 2), bf16),
            ],
            compiler_params=pltpu.CompilerParams(
                vmem_limit_bytes=120 * 1024 * 1024, flags=flags),
        )(x, A_wqkv, A_wo, B_w1, B_w3, B_w2)
        return out.reshape(1, S, D)
    return fn


_kernel = make()


def pallas_interleave_layers__sliding_local_dilated__glu_gated_swiglu__prompt_kernel(A_x, A_wqkv, A_wo, B_x, B_w1, B_w3, B_w2):
    return _kernel(A_x, A_wqkv, A_wo, B_x, B_w1, B_w3, B_w2)
```

```python
import functools

import jax
import jax.numpy as jnp
from jax import lax
import jax.experimental.pallas as pl
import jax.experimental.pallas.tpu as pltpu

S, D, DH, WIN, DIL, F = 2048, 1024, 32, 8, 2, 3584
NB = D // 128
SH = 8 * DIL
HALO = (WIN - 1) * SH
TM = 128
G = TM // 8
GP = G + 1
T = S // TM
NS = 2 * T + 1
FC = 512
NC = F // FC
HM, HD, HF = TM // 2, D // 2, FC // 2
PR = 16
f32, bf16, u32 = jnp.float32, jnp.bfloat16, jnp.uint32


def _dot(a, b):
    return jnp.dot(a, b, preferred_element_type=f32)


def _pack(v):
    return pltpu.bitcast(v.astype(bf16), u32)


def _pdot(a, b):
    return _dot(a, pltpu.bitcast(b, bf16))


def _ln(x):
    xc = x - jnp.mean(x, axis=-1, keepdims=True)
    return xc * lax.rsqrt(jnp.mean(xc * xc, axis=-1, keepdims=True) + 1e-5)


def _swiglu(g, u):
    hg = 0.5 * g
    return (hg + hg * jnp.tanh(hg)) * u


def _tree(t):
    while len(t) > 1:
        t = [t[j] + t[j + 1] for j in range(0, len(t), 2)]
    return t[0]


def _a_terms(a11, a12, a21, a22):
    return (a11 + a22, a21 + a22, a11, a22, a11 + a12, a21 - a11, a12 - a22)


def _b_terms(b11, b12, b21, b22):
    return (b11 + b22, b11, b12 - b22, b21 - b11, b22, b11 + b12, b21 + b22)


def _strassen(prod, emit=lambda i, j, v: v):
    m1 = prod(0)
    m2 = prod(1)
    t22 = m1 - m2
    m4 = prod(3)
    c21 = emit(1, 0, m2 + m4)
    t11 = m1 + m4 + prod(6)
    m5 = prod(4)
    c11 = emit(0, 0, t11 - m5)
    m3 = prod(2)
    c12 = emit(0, 1, m3 + m5)
    c22 = emit(1, 1, t22 + m3 + prod(5))
    return c11, c12, c21, c22


def _same(v):
    return v


def _dst(src, i):
    g = (src >> 2) & 7
    return (src & 3) * 32 + (g ^ i) * 4 + (src >> 5)


def _butterfly(blocks, g):
    for b in range(3):
        m = ((g >> b) & 1) == 1
        blocks = [jnp.where(m, blocks[j ^ (1 << b)], blocks[j]) for j in range(NB)]
    return blocks


def _prep_proj(src, dst, it):
    r = lax.broadcasted_iota(jnp.int32, (128, 128), 0)
    c = lax.broadcasted_iota(jnp.int32, (128, 128), 1)
    top, bot = (pl.ds(pl.multiple_of(h + it * 128, 128), 128) for h in (0, HD))
    blocks = [pltpu.bitcast(jnp.concatenate([src[top, 128 * b:128 * (b + 1)], src[bot, 128 * b:128 * (b + 1)]], axis=0), u32)
              for b in range(NB)]
    blocks = _butterfly(blocks, (c >> 2) & 7)

    def perm(i):
        p = jnp.where(c == _dst(r, i), 1.0, 0.0).astype(bf16)
        return _dot(pltpu.bitcast(blocks[i], bf16), p)

    rows = pl.ds(pl.multiple_of(it * 64, 64), 64)
    for i in range(NB // 2):
        lo, hi = perm(i), perm(i + NB // 2)
        for t, v in enumerate(_b_terms(lo[:128], hi[:128], lo[128:], hi[128:])):
            dst[t, rows, 128 * i:128 * (i + 1)] = _pack(v)


def _prep_out(src, dst, it):
    r = lax.broadcasted_iota(jnp.int32, (128, 128), 0)
    c = lax.broadcasted_iota(jnp.int32, (128, 128), 1)
    left, right = (pl.ds(pl.multiple_of(h + it * 128, 128), 128) for h in (0, HD))
    blocks = [pltpu.bitcast(jnp.concatenate([src[128 * b:128 * (b + 1), left], src[128 * b:128 * (b + 1), right]], axis=1), u32)
              for b in range(NB)]
    blocks = _butterfly(blocks, (lax.broadcasted_iota(jnp.int32, (64, 256), 0) >> 1) & 7)

    def perm(i):
        pt = jnp.where(r == _dst(c, i), 1.0, 0.0).astype(bf16)
        return _dot(pt, pltpu.bitcast(blocks[i], bf16))

    for i in range(NB // 2):
        up, dn = perm(i), perm(i + NB // 2)
        for t, v in enumerate(_b_terms(up[:, :128], up[:, 128:], dn[:, :128], dn[:, 128:])):
            dst[t, 64 * i:64 * (i + 1), left] = _pack(v)


def _prep_strip(get, put):
    blk = [pltpu.bitcast(get(i, j), u32) for i in range(2) for j in range(2)]
    even, odd = (_b_terms(*[pltpu.unpack_elementwise(v, index=h, packed_dtype=bf16, unpacked_dtype=f32) for v in blk])
                 for h in range(2))
    for t in range(7):
        if t in (1, 4):
            put(t, blk[0 if t == 1 else 3])
        else:
            put(t, pltpu.pack_elementwise([even[t], odd[t]], packed_dtype=bf16).astype(u32))


def _roll_in_groups(x):
    n = x.shape[0] // 8
    return pltpu.roll(x.reshape(n, 8, x.shape[1]), 1, 1).reshape(x.shape)


def _kernel(x_h, wqkv_h, wo_h, w1_h, w3_h, w2_h, out_h,
            wqkv_r, wo_r, w1_r, w3_r, w2_r, wa_c, w1_c, w3_c, w2_c,
            x_buf, o_buf, pbuf, qbuf, qkv, hk, hv, x1c, x2c, oc, hc,
            sem_a, sem_f, sem_io):

    def cp_qkv(j, it):
        cols = pl.ds(pl.multiple_of(j * D, D), D)
        rows = [pl.ds(pl.multiple_of(h + it * 128, 128), 128) for h in (0, HD)]
        return [pltpu.make_async_copy(wqkv_h.at[r, cols], wqkv_r.at[j, r], sem_a.at[j, it]) for r in rows]

    def start_qkv(j):
        for it in range(4):
            for cp in cp_qkv(j, it):
                cp.start()

    cp_wo = pltpu.make_async_copy(wo_h, wo_r, sem_a.at[3, 0])

    def cp_ffn(c):
        cols = pl.ds(pl.multiple_of(c * FC, FC), FC)
        return (pltpu.make_async_copy(w1_h.at[:, cols], w1_r.at[c], sem_f.at[0, c]),
                pltpu.make_async_copy(w3_h.at[:, cols], w3_r.at[c], sem_f.at[1, c]),
                pltpu.make_async_copy(w2_h.at[cols, :], w2_r.at[cols, :], sem_f.at[2, c]))

    def start_ffn(c):
        for cp in cp_ffn(c):
            cp.start()

    def cp_x(t, buf):
        return pltpu.make_async_copy(x_h.at[pl.ds(pl.multiple_of(t * TM, TM), TM), :], x_buf.at[buf], sem_io.at[0, buf])

    def cp_out(t, buf):
        return pltpu.make_async_copy(o_buf.at[buf], out_h.at[pl.ds(pl.multiple_of(t * TM, TM), TM), :], sem_io.at[1, buf])

    def next_tiles(p):
        return cp_x(2 * p + 2, 1), cp_x(2 * p + 3, 0)

    def load_x(buf, c):
        for i in range(NB):
            pbuf[1, i, GP * c:GP * c + G, :] = x_buf[buf, G * c:G * (c + 1), 128 * i:128 * (i + 1)].astype(f32)

    def store_out(buf, c):
        for i in range(NB):
            o_buf[buf, G * c:G * (c + 1), 128 * i:128 * (i + 1)] = pbuf[0, i, GP * c:GP * c + G, :].astype(bf16)

    def prep_ffn(c):
        for w, wc in ((w1_r, w1_c), (w3_r, w3_c)):
            for r in range(0, HD, PR):
                def put(t, v):
                    wc[c, t, r // 2:(r + PR) // 2, :] = v
                _prep_strip(lambda a, b: w[c, HD * a + r:HD * a + r + PR, HF * b:HF * (b + 1)], put)
        for r in range(0, HF, PR):
            def put(t, v):
                w2_c[t, pl.ds(pl.multiple_of(c * (HF // 2) + r // 2, PR // 2), PR // 2), :] = v
            _prep_strip(lambda a, b: w2_r[pl.ds(pl.multiple_of(c * FC + HF * a + r, PR), PR), HD * b:HD * (b + 1)], put)

    def in_rows(s, m):
        src = 1 - ((s >> 1) & 1)
        return jnp.concatenate(
            [jnp.concatenate([pbuf[src, i, pl.ds(m + k, 8, stride=GP), :] for i in range(NB)], axis=1) for k in range(2)],
            axis=0)

    def put_terms(dst, r, top, bot):
        for t, v in enumerate(_a_terms(top[:, :HD], top[:, HD:], bot[:, :HD], bot[:, HD:])):
            dst[t, r:r + 16, :] = v.astype(bf16)

    def ln1(s, m):
        top = _ln(in_rows(s, m))
        yield
        bot = _ln(in_rows(s, G // 2 + m))
        yield
        put_terms(x1c, 8 * m, top, bot)

    def proj(j, hook):
        def emit(a, b, v):
            qkv[j, HALO + HM * a:HALO + HM * (a + 1), HD * b:HD * (b + 1)] = v
        _strassen(lambda t: hook(_pdot(x1c[t], wa_c[j, t])), emit)

    def first_tile(s):
        return jnp.logical_or(s == 0, s == 2)

    def halo(s, j, r0, n):
        layer = (s >> 1) & 1
        hal = hk if j == 1 else hv
        cur = _roll_in_groups(qkv[j, TM + r0:TM + r0 + n, :])
        prev = hal[layer, r0:r0 + n, :]
        if j == 2:
            prev = jnp.where(first_tile(s), jnp.broadcast_to(qkv[j, HALO:HALO + 1, :], (n, D)), prev)
        chunk0 = (lax.broadcasted_iota(jnp.int32, (n, D), 0) & 7) == 0
        qkv[j, r0:r0 + n, :] = jnp.where(chunk0, prev, cur)
        hal[layer, r0:r0 + n, :] = cur

    def attend(s, r0, n, zero=None):
        def rows(w, z=0):
            b = HALO + r0 - SH * w + z
            return pl.ds(b if isinstance(b, int) else pl.multiple_of(b, 8), n)
        q = [qkv[0, rows(0), 128 * i:128 * (i + 1)] for i in range(NB)]
        logits = []
        for w in range(WIN):
            a = _tree([q[i] * qkv[1, rows(w), 128 * i:128 * (i + 1)] for i in range(NB)])
            if zero is not None and w % 2 == 1:
                qkv[0, pl.ds(pl.multiple_of(zero, 8), n), 0:128] = a
            a = a + pltpu.roll(a, 64, 1)
            a = a + pltpu.roll(a, 32, 1)
            a = a * DH ** -0.5
            if w > 0 and (not isinstance(r0, int) or r0 < SH * w):
                row = lax.broadcasted_iota(jnp.int32, (n, 128), 0) + r0
                masked = jnp.logical_and(jnp.logical_and(row < SH * w, (row & 7) == 0), first_tile(s))
                a = jnp.where(masked, -1e9, a)
            logits.append(a)
            if w == WIN // 2 - 1:
                yield
        yield
        mx = functools.reduce(jnp.maximum, logits)
        e = [jnp.exp(a - mx) for a in logits]
        inv = 1.0 / _tree(e)
        p = [a * inv for a in e]
        yield
        for i in range(NB):
            if i == NB // 2:
                yield
            cols = slice(128 * i, 128 * (i + 1))
            o = _tree([p[w] * qkv[2, rows(w), cols] for w in range(WIN)])
            qkv[0, rows(0, zero if zero is not None and i % 2 == 1 else 0), cols] = o

    def o_terms(r):
        put_terms(oc, r, qkv[0, HALO + r:HALO + r + 16, :], qkv[0, HALO + HM + r:HALO + HM + r + 16, :])

    def out_proj_ln2(s):
        c11, c12, c21, c22 = _strassen(lambda t: _pdot(oc[t], wa_c[3, t]))
        for m in range(0, G // 2, 2):
            r = slice(8 * m, 8 * m + 16)
            top = in_rows(s, m) + jnp.concatenate([c11[r], c12[r]], axis=1)
            bot = in_rows(s, G // 2 + m) + jnp.concatenate([c21[r], c22[r]], axis=1)
            qbuf[s & 1, r, :] = top
            qbuf[s & 1, HM + 8 * m:HM + 8 * m + 16, :] = bot
            put_terms(x2c, 8 * m, _ln(top), _ln(bot))

    def gate_up(c, hook):
        g = _strassen(lambda t: hook(_pdot(x2c[t], w1_c[c, t])))
        u = _strassen(lambda t: hook(_pdot(x2c[t], w3_c[c, t])))
        cols = pl.ds(HF * c if isinstance(c, int) else pl.multiple_of(HF * c, HF), HF)
        for t, v in enumerate(_a_terms(*[_swiglu(a, b) for a, b in zip(g, u)])):
            hc[t, :, cols] = v.astype(bf16)

    def down(s, hook):
        def emit(a, b, v):
            for m in range(G // 2):
                r = HM * a + 8 * m
                x2 = qbuf[1 - (s & 1), r:r + 8, HD * b:HD * (b + 1)] + v[8 * m:8 * m + 8, :]
                for i in range(NB // 2):
                    pbuf[0, NB // 2 * b + i, pl.ds(r // 8, 8, stride=GP), :] = x2[:, 128 * i:128 * (i + 1)]
        _strassen(lambda t: hook(_pdot(hc[t], w2_c[t])), emit)

    def att_head(s):
        cp_x(s, s).wait()
        for c in range(8):
            load_x(s, c)

        @pl.when(s == 1)
        def _():
            for cp in next_tiles(0):
                cp.start()
            start_ffn(5)
        for m in range(0, G // 2, 2):
            list(ln1(s, m))

        def body(j, carry):
            @pl.when(s == 0)
            def _():
                def strip(it, carry):
                    for cp in cp_qkv(j, it):
                        cp.wait()
                    n = 4 * j + it
                    pl.when(jnp.logical_or(n == 0, n == 3))(lambda: start_qkv((n + 5) >> 2))
                    pl.when(n == 5)(lambda: cp_wo.start())
                    pl.when(jnp.logical_and(n >= 7, (n & 1) == 1))(lambda: start_ffn((n - 7) >> 1))
                    _prep_proj(wqkv_r.at[j], wa_c.at[j], it)
                    return carry
                lax.fori_loop(0, 4, strip, 0)
            proj(j, _same)
            return carry
        lax.fori_loop(0, 3, body, 0)
        pl.when(s == 1)(lambda: start_ffn(6))
        halo(s, 1, 0, HALO)
        halo(s, 2, 0, HALO)
        lax.fori_loop(0, TM // 32, lambda j, c: (list(attend(s, j * 32, 32)), c)[1], 0)

        @pl.when(s == 0)
        def _():
            cp_wo.wait()
            start_ffn(3)
            lax.fori_loop(0, 4, lambda it, c: (_prep_out(wo_r, wa_c.at[3], it), c)[1], 0)
            start_ffn(4)

    def att_tail(s):
        for r in range(0, HM, 16):
            o_terms(r)
        out_proj_ln2(s)

    def ffn_head(s):
        def body(c, carry):
            @pl.when(s == 1)
            def _():
                for cp in cp_ffn(c):
                    cp.wait()
                prep_ffn(c)
            gate_up(c, _same)
            return carry
        lax.fori_loop(0, NC, body, 0)

    def steady(s, carry):
        zero = (s >> 10) * 8

        def after(buf, jobs):
            jobs = list(jobs)

            def hook(val):
                if jobs:
                    tail = val[HM - 8:, val.shape[1] - 128:]
                    if buf is pbuf:
                        pbuf[0, NB, pl.ds(pl.multiple_of(zero, 8), 8), :] = tail
                    else:
                        qkv[0, pl.ds(pl.multiple_of(zero, 8), 8), 0:128] = tail
                    jobs.pop(0)()
                return val
            return hook, jobs

        P = functools.partial
        phase = s & 3
        o_sel = jnp.where(phase < 2, phase, 2)
        x_sel = jnp.where(jnp.logical_and(jnp.logical_or(phase == 3, phase == 0), s < NS - 2), s & 1, 2)

        def pairs(fn, buf):
            return [P(lambda c: (fn(buf, c), fn(buf, c + 1)), c) for c in range(0, 8, 2)]

        att = []
        for r in range(0, HM, 16):
            for r0 in (r, r + 8, HM + r, HM + r + 8):
                att += [P(next, attend(s, r0, 8, zero), None)] * 5
            att += [P(o_terms, r)]
        plan = [after(pbuf, [P(next, g, None) for g in [ln1(s, m) for m in range(0, G // 2, 2)] for _ in range(3)]),
                after(pbuf, pairs(store_out, o_sel)),
                after(qkv, [P(halo, s, 1, r, SH) for r in range(0, HALO, SH)]),
                after(qkv, [P(halo, s, 2, r, SH) for r in range(0, HALO, SH)]),
                after(qkv, att),
                after(pbuf, pairs(load_x, x_sel))]
        gate_up(0, plan[0][0])
        assert not plan[0][1]
        for k, j in enumerate((1, 2, 0)):
            proj(j, plan[1 + k][0])
            assert not plan[1 + k][1]
        for c in range(1, NC):
            gate_up(c, plan[4][0])
        assert not plan[4][1]
        out_proj_ln2(s)
        down(s, plan[5][0])
        assert not plan[5][1]

        tile = (s >> 1) - 2 + (s & 1)
        pl.when(phase < 2)(lambda: cp_out(tile, phase).start())
        pl.when(jnp.logical_and(phase >= 2, s > 4))(lambda: cp_out(tile - 1, phase - 2).wait())

        @pl.when(jnp.logical_and(phase == 1, s < NS - 4))
        def _():
            for cp in next_tiles(s >> 2):
                cp.start()

        @pl.when(jnp.logical_and(phase == 2, s < NS - 3))
        def _():
            for cp in next_tiles(s >> 2):
                cp.wait()
        return carry

    cp_x(0, 0).start()
    start_qkv(0)
    cp_x(1, 1).start()
    x_buf[2] = jnp.zeros((TM, D), bf16)
    hk[...] = jnp.zeros(hk.shape, f32)
    hv[...] = jnp.zeros(hv.shape, f32)

    def edge(p, carry):
        s = jnp.where(p == 2, NS - 1, p)
        pl.when(p < 2)(lambda: att_head(s))

        @pl.when(p == 2)
        def _():
            for c in range(8):
                store_out(0, c)
            cp_out(T - 2, 0).start()
        pl.when(p > 0)(lambda: ffn_head(s))
        pl.when(p < 2)(lambda: att_tail(s))
        pl.when(p > 0)(lambda: down(s, _same))

        @pl.when(p == 1)
        def _():
            lax.fori_loop(2, NS - 1, steady, 0)
        return carry
    lax.fori_loop(0, 3, edge, 0)
    for c in range(8):
        store_out(1, c)
    cp_out(T - 1, 1).start()
    cp_out(T - 2, 0).wait()
    cp_out(T - 1, 1).wait()


@jax.jit
def pallas_interleave_layers__sliding_local_dilated__glu_gated_swiglu__prompt_kernel(
    A_x: jax.Array,
    A_wqkv: jax.Array,
    A_wo: jax.Array,
    B_x: jax.Array,
    B_w1: jax.Array,
    B_w3: jax.Array,
    B_w2: jax.Array,
):
    del B_x
    hbm = pl.BlockSpec(memory_space=pl.ANY)
    V = pltpu.VMEM
    out = pl.pallas_call(
        _kernel,
        in_specs=[hbm] * 6,
        out_specs=hbm,
        out_shape=jax.ShapeDtypeStruct((S, D), bf16),
        scratch_shapes=[
            V((3, D, D), bf16), V((D, D), bf16), V((NC, D, FC), bf16), V((NC, D, FC), bf16), V((F, D), bf16),
            V((4, 7, HD // 2, HD), u32), V((NC, 7, HD // 2, HF), u32), V((NC, 7, HD // 2, HF), u32),
            V((7, F // 4, HD), u32),
            V((3, TM, D), bf16), V((3, TM, D), bf16), V((2, NB + 1, 8 * GP, 128), f32), V((2, TM, D), f32),
            V((3, HALO + TM, D), f32), V((2, HALO, D), f32), V((2, HALO, D), f32),
            V((7, HM, HD), bf16), V((7, HM, HD), bf16), V((7, HM, HD), bf16), V((7, HM, F // 2), bf16),
            pltpu.SemaphoreType.DMA((4, 4)), pltpu.SemaphoreType.DMA((3, NC)), pltpu.SemaphoreType.DMA((2, 2)),
        ],
        compiler_params=pltpu.CompilerParams(vmem_limit_bytes=120 * 1024 * 1024),
    )(A_x.reshape(S, D), A_wqkv, A_wo, B_w1, B_w3, B_w2)
    return out.reshape(1, S, D)
```

```python
import functools

import jax
import jax.numpy as jnp
from jax import lax
import jax.experimental.pallas as pl
import jax.experimental.pallas.tpu as pltpu

S, D, DH, WIN, DIL, F = 2048, 1024, 32, 8, 2, 3584
NB = D // 128
SH = 8 * DIL
HALO = (WIN - 1) * SH
TM = 128
G = TM // 8
GP = G + 1
T = S // TM
NS = 2 * T + 1
FC = 512
NC = F // FC
HM, HD, HF = TM // 2, D // 2, FC // 2
PR = 16
f32, bf16, u32 = jnp.float32, jnp.bfloat16, jnp.uint32


def _dot(a, b):
    return jnp.dot(a, b, preferred_element_type=f32)


def _pack(v):
    return pltpu.bitcast(v.astype(bf16), u32)


def _pdot(a, b):
    return _dot(a, pltpu.bitcast(b, bf16))


def _ln(x):
    xc = x - jnp.mean(x, axis=-1, keepdims=True)
    return xc * lax.rsqrt(jnp.mean(xc * xc, axis=-1, keepdims=True) + 1e-5)


def _silu(g):
    hg = 0.5 * g
    return hg + hg * jnp.tanh(hg)


def _tree(t):
    while len(t) > 1:
        t = [t[j] + t[j + 1] for j in range(0, len(t), 2)]
    return t[0]


def _a_terms(a11, a12, a21, a22):
    return (a11 + a22, a21 + a22, a11, a22, a11 + a12, a21 - a11, a12 - a22)


def _b_terms(b11, b12, b21, b22):
    return (b11 + b22, b11, b12 - b22, b21 - b11, b22, b11 + b12, b21 + b22)


def _strassen(prod, emit=lambda i, j, v: v):
    m1 = prod(0)
    m2 = prod(1)
    t22 = m1 - m2
    m4 = prod(3)
    c21 = emit(1, 0, m2 + m4)
    t11 = m1 + m4 + prod(6)
    m5 = prod(4)
    c11 = emit(0, 0, t11 - m5)
    m3 = prod(2)
    c12 = emit(0, 1, m3 + m5)
    c22 = emit(1, 1, t22 + m3 + prod(5))
    return c11, c12, c21, c22


def _same(v):
    return v


def _dst(src, i):
    g = (src >> 2) & 7
    return (src & 3) * 32 + (g ^ i) * 4 + (src >> 5)


def _butterfly(blocks, g):
    for b in range(3):
        m = ((g >> b) & 1) == 1
        blocks = [jnp.where(m, blocks[j ^ (1 << b)], blocks[j]) for j in range(NB)]
    return blocks


def _prep_proj(src, dst, it):
    r = lax.broadcasted_iota(jnp.int32, (128, 128), 0)
    c = lax.broadcasted_iota(jnp.int32, (128, 128), 1)
    top, bot = (pl.ds(pl.multiple_of(h + it * 128, 128), 128) for h in (0, HD))
    blocks = [pltpu.bitcast(jnp.concatenate([src[top, 128 * b:128 * (b + 1)], src[bot, 128 * b:128 * (b + 1)]], axis=0), u32)
              for b in range(NB)]
    blocks = _butterfly(blocks, (c >> 2) & 7)

    def perm(i):
        p = jnp.where(c == _dst(r, i), 1.0, 0.0).astype(bf16)
        return _dot(pltpu.bitcast(blocks[i], bf16), p)

    rows = pl.ds(pl.multiple_of(it * 64, 64), 64)
    for i in range(NB // 2):
        lo, hi = perm(i), perm(i + NB // 2)
        for t, v in enumerate(_b_terms(lo[:128], hi[:128], lo[128:], hi[128:])):
            dst[t, rows, 128 * i:128 * (i + 1)] = _pack(v)


def _prep_out(src, dst, it):
    r = lax.broadcasted_iota(jnp.int32, (128, 128), 0)
    c = lax.broadcasted_iota(jnp.int32, (128, 128), 1)
    left, right = (pl.ds(pl.multiple_of(h + it * 128, 128), 128) for h in (0, HD))
    blocks = [pltpu.bitcast(jnp.concatenate([src[128 * b:128 * (b + 1), left], src[128 * b:128 * (b + 1), right]], axis=1), u32)
              for b in range(NB)]
    blocks = _butterfly(blocks, (lax.broadcasted_iota(jnp.int32, (64, 256), 0) >> 1) & 7)

    def perm(i):
        pt = jnp.where(r == _dst(c, i), 1.0, 0.0).astype(bf16)
        return _dot(pt, pltpu.bitcast(blocks[i], bf16))

    for i in range(NB // 2):
        up, dn = perm(i), perm(i + NB // 2)
        for t, v in enumerate(_b_terms(up[:, :128], up[:, 128:], dn[:, :128], dn[:, 128:])):
            dst[t, 64 * i:64 * (i + 1), left] = _pack(v)


def _prep_strip(get, put):
    blk = [pltpu.bitcast(get(i, j), u32) for i in range(2) for j in range(2)]
    even, odd = (_b_terms(*[pltpu.unpack_elementwise(v, index=h, packed_dtype=bf16, unpacked_dtype=f32) for v in blk])
                 for h in range(2))
    for t in range(7):
        if t in (1, 4):
            put(t, blk[0 if t == 1 else 3])
        else:
            put(t, pltpu.pack_elementwise([even[t], odd[t]], packed_dtype=bf16).astype(u32))


def _roll_in_groups(x):
    n = x.shape[0] // 8
    return pltpu.roll(x.reshape(n, 8, x.shape[1]), 1, 1).reshape(x.shape)


def _kernel(x_h, wqkv_h, wo_h, w1_h, w3_h, w2_h, out_h,
            wqkv_r, wo_r, w1_r, w3_r, w2_r, wa_c, w1_c, w3_c, w2_c,
            x_buf, o_buf, pbuf, qbuf, qkv, hk, hv, x1c, x2c, oc, hc,
            sem_a, sem_f, sem_io):

    def cp_qkv(j, it):
        cols = pl.ds(pl.multiple_of(j * D, D), D)
        rows = [pl.ds(pl.multiple_of(h + it * 128, 128), 128) for h in (0, HD)]
        return [pltpu.make_async_copy(wqkv_h.at[r, cols], wqkv_r.at[j, r], sem_a.at[j, it]) for r in rows]

    def start_qkv(j):
        for it in range(4):
            for cp in cp_qkv(j, it):
                cp.start()

    cp_wo = pltpu.make_async_copy(wo_h, wo_r, sem_a.at[3, 0])

    def cp_ffn(c):
        cols = pl.ds(pl.multiple_of(c * FC, FC), FC)
        return (pltpu.make_async_copy(w1_h.at[:, cols], w1_r.at[c], sem_f.at[0, c]),
                pltpu.make_async_copy(w3_h.at[:, cols], w3_r.at[c], sem_f.at[1, c]),
                pltpu.make_async_copy(w2_h.at[cols, :], w2_r.at[cols, :], sem_f.at[2, c]))

    def start_ffn(c):
        for cp in cp_ffn(c):
            cp.start()

    def cp_x(t, buf):
        return pltpu.make_async_copy(x_h.at[pl.ds(pl.multiple_of(t * TM, TM), TM), :], x_buf.at[buf], sem_io.at[0, buf])

    def cp_out(t, buf):
        return pltpu.make_async_copy(o_buf.at[buf], out_h.at[pl.ds(pl.multiple_of(t * TM, TM), TM), :], sem_io.at[1, buf])

    def next_tiles(p):
        return cp_x(2 * p + 2, 1), cp_x(2 * p + 3, 0)

    def load_x(buf, c):
        for i in range(NB):
            pbuf[1, i, GP * c:GP * c + G, :] = x_buf[buf, G * c:G * (c + 1), 128 * i:128 * (i + 1)].astype(f32)

    def store_out(buf, c):
        for i in range(NB):
            o_buf[buf, G * c:G * (c + 1), 128 * i:128 * (i + 1)] = pbuf[0, i, GP * c:GP * c + G, :].astype(bf16)

    def prep_ffn(c):
        for w, wc in ((w1_r, w1_c), (w3_r, w3_c)):
            for r in range(0, HD, PR):
                def put(t, v):
                    wc[c, t, r // 2:(r + PR) // 2, :] = v
                _prep_strip(lambda a, b: w[c, HD * a + r:HD * a + r + PR, HF * b:HF * (b + 1)], put)
        for r in range(0, HF, PR):
            def put(t, v):
                w2_c[t, pl.ds(pl.multiple_of(c * (HF // 2) + r // 2, PR // 2), PR // 2), :] = v
            _prep_strip(lambda a, b: w2_r[pl.ds(pl.multiple_of(c * FC + HF * a + r, PR), PR), HD * b:HD * (b + 1)], put)

    def in_rows(s, m):
        src = 1 - ((s >> 1) & 1)
        return jnp.concatenate(
            [jnp.concatenate([pbuf[src, i, pl.ds(m + k, 8, stride=GP), :] for i in range(NB)], axis=1) for k in range(2)],
            axis=0)

    def put_terms(dst, r, top, bot):
        for t, v in enumerate(_a_terms(top[:, :HD], top[:, HD:], bot[:, :HD], bot[:, HD:])):
            dst[t, r:r + 16, :] = v.astype(bf16)

    def ln1(s, m):
        top = _ln(in_rows(s, m))
        yield
        bot = _ln(in_rows(s, G // 2 + m))
        yield
        put_terms(x1c, 8 * m, top, bot)

    def proj(j, hook):
        def emit(a, b, v):
            qkv[j, HALO + HM * a:HALO + HM * (a + 1), HD * b:HD * (b + 1)] = v
        _strassen(lambda t: hook(_pdot(x1c[t], wa_c[j, t])), emit)

    def first_tile(s):
        return jnp.logical_or(s == 0, s == 2)

    def halo(s, j, r0, n):
        layer = (s >> 1) & 1
        hal = hk if j == 1 else hv
        cur = _roll_in_groups(qkv[j, TM + r0:TM + r0 + n, :])
        prev = hal[layer, r0:r0 + n, :]
        if j == 2:
            prev = jnp.where(first_tile(s), jnp.broadcast_to(qkv[j, HALO:HALO + 1, :], (n, D)), prev)
        chunk0 = (lax.broadcasted_iota(jnp.int32, (n, D), 0) & 7) == 0
        qkv[j, r0:r0 + n, :] = jnp.where(chunk0, prev, cur)
        hal[layer, r0:r0 + n, :] = cur

    def attend(s, r0, n, zero=None):
        def rows(w, z=0):
            b = HALO + r0 - SH * w + z
            return pl.ds(b if isinstance(b, int) else pl.multiple_of(b, 8), n)
        q = [qkv[0, rows(0), 128 * i:128 * (i + 1)] for i in range(NB)]
        logits = []
        for w in range(WIN):
            a = _tree([q[i] * qkv[1, rows(w), 128 * i:128 * (i + 1)] for i in range(NB)])
            if zero is not None and w % 4 == 1:
                qkv[0, pl.ds(pl.multiple_of(zero, 8), n), 0:128] = a
            a = a + pltpu.roll(a, 64, 1)
            a = a + pltpu.roll(a, 32, 1)
            a = a * DH ** -0.5
            if w > 0 and (not isinstance(r0, int) or r0 < SH * w):
                row = lax.broadcasted_iota(jnp.int32, (n, 128), 0) + r0
                masked = jnp.logical_and(jnp.logical_and(row < SH * w, (row & 7) == 0), first_tile(s))
                a = jnp.where(masked, -1e9, a)
            logits.append(a)
            if w == WIN // 2 - 1:
                yield
        yield
        mx = functools.reduce(jnp.maximum, logits)
        e = [jnp.exp(a - mx) for a in logits]
        inv = 1.0 / _tree(e)
        p = [a * inv for a in e]
        yield
        for i in range(NB):
            if i == NB // 2:
                yield
            cols = slice(128 * i, 128 * (i + 1))
            o = _tree([p[w] * qkv[2, rows(w), cols] for w in range(WIN)])
            qkv[0, rows(0, zero if zero is not None and i % 2 == 1 else 0), cols] = o

    def o_terms(r):
        put_terms(oc, r, qkv[0, HALO + r:HALO + r + 16, :], qkv[0, HALO + HM + r:HALO + HM + r + 16, :])

    def out_proj_ln2(s):
        c11, c12, c21, c22 = _strassen(lambda t: _pdot(oc[t], wa_c[3, t]))
        for m in range(0, G // 2, 2):
            r = slice(8 * m, 8 * m + 16)
            top = in_rows(s, m) + jnp.concatenate([c11[r], c12[r]], axis=1)
            bot = in_rows(s, G // 2 + m) + jnp.concatenate([c21[r], c22[r]], axis=1)
            qbuf[s & 1, r, :] = top
            qbuf[s & 1, HM + 8 * m:HM + 8 * m + 16, :] = bot
            put_terms(x2c, 8 * m, _ln(top), _ln(bot))

    def gate_up(c, hook):
        cols = pl.ds(HF * c if isinstance(c, int) else pl.multiple_of(HF * c, HF), HF)
        g11, g12, g21, g22 = _strassen(lambda t: hook(_pdot(x2c[t], w1_c[c, t])), lambda i, j, v: _silu(v))
        act, h = ((g11, g12), (g21, g22)), {}

        def emit(i, j, v):
            h[i, j] = act[i][j] * v
            ready = {(1, 0): {},
                     (0, 0): {2: lambda: h[0, 0], 5: lambda: h[1, 0] - h[0, 0]},
                     (0, 1): {4: lambda: h[0, 0] + h[0, 1]},
                     (1, 1): {0: lambda: h[0, 0] + h[1, 1], 1: lambda: h[1, 0] + h[1, 1],
                              3: lambda: h[1, 1], 6: lambda: h[0, 1] - h[1, 1]}}[i, j]
            for t, term in ready.items():
                hc[t, :, cols] = term().astype(bf16)
        _strassen(lambda t: hook(_pdot(x2c[t], w3_c[c, t])), emit)

    def down(s, hook):
        def emit(a, b, v):
            for m in range(G // 2):
                r = HM * a + 8 * m
                x2 = qbuf[1 - (s & 1), r:r + 8, HD * b:HD * (b + 1)] + v[8 * m:8 * m + 8, :]
                for i in range(NB // 2):
                    pbuf[0, NB // 2 * b + i, pl.ds(r // 8, 8, stride=GP), :] = x2[:, 128 * i:128 * (i + 1)]
        _strassen(lambda t: hook(_pdot(hc[t], w2_c[t])), emit)

    def att_head(s):
        cp_x(s, s).wait()
        for c in range(8):
            load_x(s, c)

        @pl.when(s == 1)
        def _():
            for cp in next_tiles(0):
                cp.start()
            start_ffn(5)
        for m in range(0, G // 2, 2):
            list(ln1(s, m))

        def body(j, carry):
            @pl.when(s == 0)
            def _():
                def strip(it, carry):
                    for cp in cp_qkv(j, it):
                        cp.wait()
                    n = 4 * j + it
                    pl.when(jnp.logical_or(n == 0, n == 3))(lambda: start_qkv((n + 5) >> 2))
                    pl.when(n == 5)(lambda: cp_wo.start())
                    pl.when(jnp.logical_and(n >= 7, (n & 1) == 1))(lambda: start_ffn((n - 7) >> 1))
                    _prep_proj(wqkv_r.at[j], wa_c.at[j], it)
                    return carry
                lax.fori_loop(0, 4, strip, 0)
            proj(j, _same)
            return carry
        lax.fori_loop(0, 3, body, 0)
        pl.when(s == 1)(lambda: start_ffn(6))
        halo(s, 1, 0, HALO)
        halo(s, 2, 0, HALO)
        lax.fori_loop(0, TM // 32, lambda j, c: (list(attend(s, j * 32, 32)), c)[1], 0)

        @pl.when(s == 0)
        def _():
            cp_wo.wait()
            start_ffn(3)
            lax.fori_loop(0, 4, lambda it, c: (_prep_out(wo_r, wa_c.at[3], it), c)[1], 0)
            start_ffn(4)

    def att_tail(s):
        for r in range(0, HM, 16):
            o_terms(r)
        out_proj_ln2(s)

    def ffn_head(s):
        def body(c, carry):
            @pl.when(s == 1)
            def _():
                for cp in cp_ffn(c):
                    cp.wait()
                prep_ffn(c)
            gate_up(c, _same)
            return carry
        lax.fori_loop(0, NC, body, 0)

    def steady(s, carry):
        zero = (s >> 10) * 8

        def after(buf, jobs):
            jobs = list(jobs)

            def hook(val):
                if jobs:
                    tail = val[:8, :128]
                    if buf is pbuf:
                        pbuf[0, NB, pl.ds(pl.multiple_of(zero, 8), 8), :] = tail
                    else:
                        qkv[0, pl.ds(pl.multiple_of(zero, 8), 8), 0:128] = tail
                    jobs.pop(0)()
                return val
            return hook, jobs

        P = functools.partial
        phase = s & 3
        o_sel = jnp.where(phase < 2, phase, 2)
        x_sel = jnp.where(jnp.logical_and(jnp.logical_or(phase == 3, phase == 0), s < NS - 2), s & 1, 2)

        def pairs(fn, buf):
            return [P(lambda c: (fn(buf, c), fn(buf, c + 1)), c) for c in range(0, 8, 2)]

        att = []
        for r in range(0, HM, 16):
            for r0 in (r, r + 8, HM + r, HM + r + 8):
                att += [P(next, attend(s, r0, 8, zero), None)] * 5
            att += [P(o_terms, r)]
        plan = [after(pbuf, [P(next, g, None) for g in [ln1(s, m) for m in range(0, G // 2, 2)] for _ in range(3)]),
                after(pbuf, pairs(store_out, o_sel)),
                after(qkv, [P(halo, s, 1, r, SH) for r in range(0, HALO, SH)]),
                after(qkv, [P(halo, s, 2, r, SH) for r in range(0, HALO, SH)]),
                after(qkv, att),
                after(pbuf, pairs(load_x, x_sel))]
        gate_up(0, plan[0][0])
        assert not plan[0][1]
        for k, j in enumerate((1, 2, 0)):
            proj(j, plan[1 + k][0])
            assert not plan[1 + k][1]
        for c in range(1, NC):
            gate_up(c, plan[4][0])
        assert not plan[4][1]
        out_proj_ln2(s)
        down(s, plan[5][0])
        assert not plan[5][1]

        tile = (s >> 1) - 2 + (s & 1)
        pl.when(phase < 2)(lambda: cp_out(tile, phase).start())
        pl.when(jnp.logical_and(phase >= 2, s > 4))(lambda: cp_out(tile - 1, phase - 2).wait())

        @pl.when(jnp.logical_and(phase == 1, s < NS - 4))
        def _():
            for cp in next_tiles(s >> 2):
                cp.start()

        @pl.when(jnp.logical_and(phase == 2, s < NS - 3))
        def _():
            for cp in next_tiles(s >> 2):
                cp.wait()
        return carry

    cp_x(0, 0).start()
    start_qkv(0)
    cp_x(1, 1).start()
    x_buf[2] = jnp.zeros((TM, D), bf16)
    hk[...] = jnp.zeros(hk.shape, f32)
    hv[...] = jnp.zeros(hv.shape, f32)

    def edge(p, carry):
        s = jnp.where(p == 2, NS - 1, p)
        pl.when(p < 2)(lambda: att_head(s))

        @pl.when(p == 2)
        def _():
            for c in range(8):
                store_out(0, c)
            cp_out(T - 2, 0).start()
        pl.when(p > 0)(lambda: ffn_head(s))
        pl.when(p < 2)(lambda: att_tail(s))
        pl.when(p > 0)(lambda: down(s, _same))

        @pl.when(p == 1)
        def _():
            lax.fori_loop(2, NS - 1, steady, 0)
        return carry
    lax.fori_loop(0, 3, edge, 0)
    for c in range(8):
        store_out(1, c)
    cp_out(T - 1, 1).start()
    cp_out(T - 2, 0).wait()
    cp_out(T - 1, 1).wait()


@jax.jit
def pallas_interleave_layers__sliding_local_dilated__glu_gated_swiglu__prompt_kernel(
    A_x: jax.Array,
    A_wqkv: jax.Array,
    A_wo: jax.Array,
    B_x: jax.Array,
    B_w1: jax.Array,
    B_w3: jax.Array,
    B_w2: jax.Array,
):
    del B_x
    hbm = pl.BlockSpec(memory_space=pl.ANY)
    V = pltpu.VMEM
    out = pl.pallas_call(
        _kernel,
        in_specs=[hbm] * 6,
        out_specs=hbm,
        out_shape=jax.ShapeDtypeStruct((S, D), bf16),
        scratch_shapes=[
            V((3, D, D), bf16), V((D, D), bf16), V((NC, D, FC), bf16), V((NC, D, FC), bf16), V((F, D), bf16),
            V((4, 7, HD // 2, HD), u32), V((NC, 7, HD // 2, HF), u32), V((NC, 7, HD // 2, HF), u32),
            V((7, F // 4, HD), u32),
            V((3, TM, D), bf16), V((3, TM, D), bf16), V((2, NB + 1, 8 * GP, 128), f32), V((2, TM, D), f32),
            V((3, HALO + TM, D), f32), V((2, HALO, D), f32), V((2, HALO, D), f32),
            V((7, HM, HD), bf16), V((7, HM, HD), bf16), V((7, HM, HD), bf16), V((7, HM, F // 2), bf16),
            pltpu.SemaphoreType.DMA((4, 4)), pltpu.SemaphoreType.DMA((3, NC)), pltpu.SemaphoreType.DMA((2, 2)),
        ],
        compiler_params=pltpu.CompilerParams(vmem_limit_bytes=120 * 1024 * 1024),
    )(A_x.reshape(S, D), A_wqkv, A_wo, B_w1, B_w3, B_w2)
    return out.reshape(1, S, D)
```

```python
import functools

import jax
import jax.numpy as jnp
from jax import lax
import jax.experimental.pallas as pl
import jax.experimental.pallas.tpu as pltpu

S, D, DH, WIN, DIL, F = 2048, 1024, 32, 8, 2, 3584
NB = D // 128
SH = 8 * DIL
HALO = (WIN - 1) * SH
TM = 128
G = TM // 8
GP = G + 1
T = S // TM
NS = 2 * T + 1
FC = 512
NC = F // FC
HM, HD, HF = TM // 2, D // 2, FC // 2
PR = 16
f32, bf16, u32 = jnp.float32, jnp.bfloat16, jnp.uint32


def _dot(a, b):
    return jnp.dot(a, b, preferred_element_type=f32)


def _pack(v):
    return pltpu.bitcast(v.astype(bf16), u32)


def _pdot(a, b):
    return _dot(a, pltpu.bitcast(b, bf16))


def _ln(x):
    xc = x - jnp.mean(x, axis=-1, keepdims=True)
    return xc * lax.rsqrt(jnp.mean(xc * xc, axis=-1, keepdims=True) + 1e-5)


def _silu(g):
    hg = 0.5 * g
    return hg + hg * jnp.tanh(hg)


def _tree(t):
    while len(t) > 1:
        t = [t[j] + t[j + 1] for j in range(0, len(t), 2)]
    return t[0]


def _a_terms(a11, a12, a21, a22):
    return (a11 + a22, a21 + a22, a11, a22, a11 + a12, a21 - a11, a12 - a22)


def _b_terms(b11, b12, b21, b22):
    return (b11 + b22, b11, b12 - b22, b21 - b11, b22, b11 + b12, b21 + b22)


def _strassen(prod, emit=lambda i, j, v: v):
    m1 = prod(0)
    m2 = prod(1)
    t22 = m1 - m2
    m4 = prod(3)
    c21 = emit(1, 0, m2 + m4)
    t11 = m1 + m4 + prod(6)
    m5 = prod(4)
    c11 = emit(0, 0, t11 - m5)
    m3 = prod(2)
    c12 = emit(0, 1, m3 + m5)
    c22 = emit(1, 1, t22 + m3 + prod(5))
    return c11, c12, c21, c22


def _same(v):
    return v


def _dst(src, i):
    g = (src >> 2) & 7
    return (src & 3) * 32 + (g ^ i) * 4 + (src >> 5)


def _butterfly(blocks, g):
    for b in range(3):
        m = ((g >> b) & 1) == 1
        blocks = [jnp.where(m, blocks[j ^ (1 << b)], blocks[j]) for j in range(NB)]
    return blocks


def _prep_proj(src, dst, it):
    r = lax.broadcasted_iota(jnp.int32, (128, 128), 0)
    c = lax.broadcasted_iota(jnp.int32, (128, 128), 1)
    top, bot = (pl.ds(pl.multiple_of(h + it * 128, 128), 128) for h in (0, HD))
    blocks = [pltpu.bitcast(jnp.concatenate([src[top, 128 * b:128 * (b + 1)], src[bot, 128 * b:128 * (b + 1)]], axis=0), u32)
              for b in range(NB)]
    blocks = _butterfly(blocks, (c >> 2) & 7)

    def perm(i):
        p = jnp.where(c == _dst(r, i), 1.0, 0.0).astype(bf16)
        return _dot(pltpu.bitcast(blocks[i], bf16), p)

    rows = pl.ds(pl.multiple_of(it * 64, 64), 64)
    for i in range(NB // 2):
        lo, hi = perm(i), perm(i + NB // 2)
        for t, v in enumerate(_b_terms(lo[:128], hi[:128], lo[128:], hi[128:])):
            dst[t, rows, 128 * i:128 * (i + 1)] = _pack(v)


def _prep_out(src, dst, it):
    r = lax.broadcasted_iota(jnp.int32, (128, 128), 0)
    c = lax.broadcasted_iota(jnp.int32, (128, 128), 1)
    left, right = (pl.ds(pl.multiple_of(h + it * 128, 128), 128) for h in (0, HD))
    blocks = [pltpu.bitcast(jnp.concatenate([src[128 * b:128 * (b + 1), left], src[128 * b:128 * (b + 1), right]], axis=1), u32)
              for b in range(NB)]
    blocks = _butterfly(blocks, (lax.broadcasted_iota(jnp.int32, (64, 256), 0) >> 1) & 7)

    def perm(i):
        pt = jnp.where(r == _dst(c, i), 1.0, 0.0).astype(bf16)
        return _dot(pt, pltpu.bitcast(blocks[i], bf16))

    for i in range(NB // 2):
        up, dn = perm(i), perm(i + NB // 2)
        for t, v in enumerate(_b_terms(up[:, :128], up[:, 128:], dn[:, :128], dn[:, 128:])):
            dst[t, 64 * i:64 * (i + 1), left] = _pack(v)


def _prep_strip(get, put):
    blk = [get(i, j) for i in range(2) for j in range(2)]
    terms = _b_terms(*[v.astype(f32) for v in blk])
    for t in range(7):
        put(t, _pack(blk[0] if t == 1 else blk[3] if t == 4 else terms[t]))


def _roll_in_groups(x):
    n = x.shape[0] // 8
    return pltpu.roll(x.reshape(n, 8, x.shape[1]), 1, 1).reshape(x.shape)


def _kernel(x_h, wqkv_h, wo_h, w1_h, w3_h, w2_h, out_h,
            wqkv_r, wo_r, w1_r, w3_r, w2_r, wa_c, w1_c, w3_c, w2_c,
            x_buf, o_buf, pbuf, qbuf, qkv, hk, hv, x1c, x2c, oc, hc,
            sem_a, sem_f, sem_io):

    def cp_qkv(j, it):
        cols = pl.ds(pl.multiple_of(j * D, D), D)
        rows = [pl.ds(pl.multiple_of(h + it * 128, 128), 128) for h in (0, HD)]
        return [pltpu.make_async_copy(wqkv_h.at[r, cols], wqkv_r.at[j, r], sem_a.at[j, it]) for r in rows]

    def start_qkv(j):
        for it in range(4):
            for cp in cp_qkv(j, it):
                cp.start()

    cp_wo = pltpu.make_async_copy(wo_h, wo_r, sem_a.at[3, 0])

    def cp_ffn(c):
        cols = pl.ds(pl.multiple_of(c * FC, FC), FC)
        return (pltpu.make_async_copy(w1_h.at[:, cols], w1_r.at[c], sem_f.at[0, c]),
                pltpu.make_async_copy(w3_h.at[:, cols], w3_r.at[c], sem_f.at[1, c]),
                pltpu.make_async_copy(w2_h.at[cols, :], w2_r.at[cols, :], sem_f.at[2, c]))

    def start_ffn(c):
        for cp in cp_ffn(c):
            cp.start()

    def cp_x(t, buf):
        return pltpu.make_async_copy(x_h.at[pl.ds(pl.multiple_of(t * TM, TM), TM), :], x_buf.at[buf], sem_io.at[0, buf])

    def cp_out(t, buf):
        return pltpu.make_async_copy(o_buf.at[buf], out_h.at[pl.ds(pl.multiple_of(t * TM, TM), TM), :], sem_io.at[1, buf])

    def next_tiles(p):
        return cp_x(2 * p + 2, 1), cp_x(2 * p + 3, 0)

    def load_x(buf, c):
        for i in range(NB):
            pbuf[1, i, GP * c:GP * c + G, :] = x_buf[buf, G * c:G * (c + 1), 128 * i:128 * (i + 1)].astype(f32)

    def store_out(buf, c):
        for i in range(NB):
            o_buf[buf, G * c:G * (c + 1), 128 * i:128 * (i + 1)] = pbuf[0, i, GP * c:GP * c + G, :].astype(bf16)

    def prep_ffn(c):
        for w, wc in ((w1_r, w1_c), (w3_r, w3_c)):
            for r in range(0, HD, PR):
                def put(t, v):
                    wc[c, t, r // 2:(r + PR) // 2, :] = v
                _prep_strip(lambda a, b: w[c, HD * a + r:HD * a + r + PR, HF * b:HF * (b + 1)], put)
        for r in range(0, HF, PR):
            def put(t, v):
                w2_c[t, pl.ds(pl.multiple_of(c * (HF // 2) + r // 2, PR // 2), PR // 2), :] = v
            _prep_strip(lambda a, b: w2_r[pl.ds(pl.multiple_of(c * FC + HF * a + r, PR), PR), HD * b:HD * (b + 1)], put)

    def in_rows(s, m):
        src = 1 - ((s >> 1) & 1)
        return jnp.concatenate(
            [jnp.concatenate([pbuf[src, i, pl.ds(m + k, 8, stride=GP), :] for i in range(NB)], axis=1) for k in range(2)],
            axis=0)

    def put_terms(dst, r, top, bot):
        for t, v in enumerate(_a_terms(top[:, :HD], top[:, HD:], bot[:, :HD], bot[:, HD:])):
            dst[t, r:r + 16, :] = v.astype(bf16)

    def ln1(s, m):
        top = _ln(in_rows(s, m))
        yield
        bot = _ln(in_rows(s, G // 2 + m))
        yield
        put_terms(x1c, 8 * m, top, bot)

    def proj(j, hook):
        def emit(a, b, v):
            qkv[j, HALO + HM * a:HALO + HM * (a + 1), HD * b:HD * (b + 1)] = v
        _strassen(lambda t: hook(_pdot(x1c[t], wa_c[j, t])), emit)

    def first_tile(s):
        return jnp.logical_or(s == 0, s == 2)

    def halo(s, j, r0, n):
        layer = (s >> 1) & 1
        hal = hk if j == 1 else hv
        cur = _roll_in_groups(qkv[j, TM + r0:TM + r0 + n, :])
        prev = hal[layer, r0:r0 + n, :]
        if j == 2:
            prev = jnp.where(first_tile(s), jnp.broadcast_to(qkv[j, HALO:HALO + 1, :], (n, D)), prev)
        chunk0 = (lax.broadcasted_iota(jnp.int32, (n, D), 0) & 7) == 0
        qkv[j, r0:r0 + n, :] = jnp.where(chunk0, prev, cur)
        hal[layer, r0:r0 + n, :] = cur

    def attend(s, r0, n, zero=None):
        def rows(w, z=0):
            b = HALO + r0 - SH * w + z
            return pl.ds(b if isinstance(b, int) else pl.multiple_of(b, 8), n)
        q = [qkv[0, rows(0), 128 * i:128 * (i + 1)] for i in range(NB)]
        logits = []
        for w in range(WIN):
            a = _tree([q[i] * qkv[1, rows(w), 128 * i:128 * (i + 1)] for i in range(NB)])
            if zero is not None and w % 4 == 1:
                qkv[0, pl.ds(pl.multiple_of(zero, 8), n), 0:128] = a
            a = a + pltpu.roll(a, 64, 1)
            a = a + pltpu.roll(a, 32, 1)
            a = a * DH ** -0.5
            if w > 0 and (not isinstance(r0, int) or r0 < SH * w):
                row = lax.broadcasted_iota(jnp.int32, (n, 128), 0) + r0
                masked = jnp.logical_and(jnp.logical_and(row < SH * w, (row & 7) == 0), first_tile(s))
                a = jnp.where(masked, -1e9, a)
            logits.append(a)
            if w == WIN // 2 - 1:
                yield
        yield
        mx = functools.reduce(jnp.maximum, logits)
        e = [jnp.exp(a - mx) for a in logits]
        inv = 1.0 / _tree(e)
        p = [a * inv for a in e]
        yield
        for i in range(NB):
            if i == NB // 2:
                yield
            cols = slice(128 * i, 128 * (i + 1))
            o = _tree([p[w] * qkv[2, rows(w), cols] for w in range(WIN)])
            qkv[0, rows(0, zero if zero is not None and i % 2 == 1 else 0), cols] = o

    def o_terms(r):
        put_terms(oc, r, qkv[0, HALO + r:HALO + r + 16, :], qkv[0, HALO + HM + r:HALO + HM + r + 16, :])

    def out_proj_ln2(s):
        c11, c12, c21, c22 = _strassen(lambda t: _pdot(oc[t], wa_c[3, t]))
        for m in range(0, G // 2, 2):
            r = slice(8 * m, 8 * m + 16)
            top = in_rows(s, m) + jnp.concatenate([c11[r], c12[r]], axis=1)
            bot = in_rows(s, G // 2 + m) + jnp.concatenate([c21[r], c22[r]], axis=1)
            qbuf[s & 1, r, :] = top
            qbuf[s & 1, HM + 8 * m:HM + 8 * m + 16, :] = bot
            put_terms(x2c, 8 * m, _ln(top), _ln(bot))

    def gate_up(c, hook):
        cols = pl.ds(HF * c if isinstance(c, int) else pl.multiple_of(HF * c, HF), HF)
        g11, g12, g21, g22 = _strassen(lambda t: hook(_pdot(x2c[t], w1_c[c, t])), lambda i, j, v: _silu(v))
        act, h = ((g11, g12), (g21, g22)), {}

        def emit(i, j, v):
            h[i, j] = act[i][j] * v
            ready = {(1, 0): {},
                     (0, 0): {2: lambda: h[0, 0], 5: lambda: h[1, 0] - h[0, 0]},
                     (0, 1): {4: lambda: h[0, 0] + h[0, 1]},
                     (1, 1): {0: lambda: h[0, 0] + h[1, 1], 1: lambda: h[1, 0] + h[1, 1],
                              3: lambda: h[1, 1], 6: lambda: h[0, 1] - h[1, 1]}}[i, j]
            for t, term in ready.items():
                hc[t, :, cols] = term().astype(bf16)
        _strassen(lambda t: hook(_pdot(x2c[t], w3_c[c, t])), emit)

    def down(s, hook):
        def emit(a, b, v):
            for m in range(G // 2):
                r = HM * a + 8 * m
                x2 = qbuf[1 - (s & 1), r:r + 8, HD * b:HD * (b + 1)] + v[8 * m:8 * m + 8, :]
                for i in range(NB // 2):
                    pbuf[0, NB // 2 * b + i, pl.ds(r // 8, 8, stride=GP), :] = x2[:, 128 * i:128 * (i + 1)]
        _strassen(lambda t: hook(_pdot(hc[t], w2_c[t])), emit)

    def att_head(s):
        cp_x(s, s).wait()
        for c in range(8):
            load_x(s, c)

        @pl.when(s == 1)
        def _():
            for cp in next_tiles(0):
                cp.start()
            start_ffn(5)
        for m in range(0, G // 2, 2):
            list(ln1(s, m))

        def body(j, carry):
            @pl.when(s == 0)
            def _():
                def strip(it, carry):
                    for cp in cp_qkv(j, it):
                        cp.wait()
                    n = 4 * j + it
                    pl.when(jnp.logical_or(n == 0, n == 3))(lambda: start_qkv((n + 5) >> 2))
                    pl.when(n == 5)(lambda: cp_wo.start())
                    pl.when(jnp.logical_and(n >= 7, (n & 1) == 1))(lambda: start_ffn((n - 7) >> 1))
                    _prep_proj(wqkv_r.at[j], wa_c.at[j], it)
                    return carry
                lax.fori_loop(0, 4, strip, 0)
            proj(j, _same)
            return carry
        lax.fori_loop(0, 3, body, 0)
        pl.when(s == 1)(lambda: start_ffn(6))
        halo(s, 1, 0, HALO)
        halo(s, 2, 0, HALO)
        lax.fori_loop(0, TM // 32, lambda j, c: (list(attend(s, j * 32, 32)), c)[1], 0)

        @pl.when(s == 0)
        def _():
            cp_wo.wait()
            start_ffn(3)
            lax.fori_loop(0, 4, lambda it, c: (_prep_out(wo_r, wa_c.at[3], it), c)[1], 0)
            start_ffn(4)

    def att_tail(s):
        for r in range(0, HM, 16):
            o_terms(r)
        out_proj_ln2(s)

    def ffn_head(s):
        def body(c, carry):
            @pl.when(s == 1)
            def _():
                for cp in cp_ffn(c):
                    cp.wait()
                prep_ffn(c)
            gate_up(c, _same)
            return carry
        lax.fori_loop(0, NC, body, 0)

    def steady(s, carry):
        zero = (s >> 10) * 8

        def after(buf, jobs):
            jobs = list(jobs)

            def hook(val):
                if jobs:
                    tail = val[:8, :128]
                    if buf is pbuf:
                        pbuf[0, NB, pl.ds(pl.multiple_of(zero, 8), 8), :] = tail
                    else:
                        qkv[0, pl.ds(pl.multiple_of(zero, 8), 8), 0:128] = tail
                    jobs.pop(0)()
                return val
            return hook, jobs

        P = functools.partial
        phase = s & 3
        o_sel = jnp.where(phase < 2, phase, 2)
        x_sel = jnp.where(jnp.logical_and(jnp.logical_or(phase == 3, phase == 0), s < NS - 2), s & 1, 2)

        def pairs(fn, buf):
            return [P(lambda c: (fn(buf, c), fn(buf, c + 1)), c) for c in range(0, 8, 2)]

        att = []
        for r in range(0, HM, 16):
            for r0 in (r, r + 8, HM + r, HM + r + 8):
                att += [P(next, attend(s, r0, 8, zero), None)] * 5
            att += [P(o_terms, r)]
        plan = [after(pbuf, [P(next, g, None) for g in [ln1(s, m) for m in range(0, G // 2, 2)] for _ in range(3)]),
                after(pbuf, pairs(store_out, o_sel)),
                after(qkv, [P(halo, s, 1, r, SH) for r in range(0, HALO, SH)]),
                after(qkv, [P(halo, s, 2, r, SH) for r in range(0, HALO, SH)]),
                after(qkv, att),
                after(pbuf, pairs(load_x, x_sel))]
        gate_up(0, plan[0][0])
        assert not plan[0][1]
        for k, j in enumerate((1, 2, 0)):
            proj(j, plan[1 + k][0])
            assert not plan[1 + k][1]
        for c in range(1, NC):
            gate_up(c, plan[4][0])
        assert not plan[4][1]
        out_proj_ln2(s)
        down(s, plan[5][0])
        assert not plan[5][1]

        tile = (s >> 1) - 2 + (s & 1)
        pl.when(phase < 2)(lambda: cp_out(tile, phase).start())
        pl.when(jnp.logical_and(phase >= 2, s > 4))(lambda: cp_out(tile - 1, phase - 2).wait())

        @pl.when(jnp.logical_and(phase == 1, s < NS - 4))
        def _():
            for cp in next_tiles(s >> 2):
                cp.start()

        @pl.when(jnp.logical_and(phase == 2, s < NS - 3))
        def _():
            for cp in next_tiles(s >> 2):
                cp.wait()
        return carry

    cp_x(0, 0).start()
    start_qkv(0)
    cp_x(1, 1).start()
    x_buf[2] = jnp.zeros((TM, D), bf16)
    hk[...] = jnp.zeros(hk.shape, f32)
    hv[...] = jnp.zeros(hv.shape, f32)

    def edge(p, carry):
        s = jnp.where(p == 2, NS - 1, p)
        pl.when(p < 2)(lambda: att_head(s))

        @pl.when(p == 2)
        def _():
            for c in range(8):
                store_out(0, c)
            cp_out(T - 2, 0).start()
        pl.when(p > 0)(lambda: ffn_head(s))
        pl.when(p < 2)(lambda: att_tail(s))
        pl.when(p > 0)(lambda: down(s, _same))

        @pl.when(p == 1)
        def _():
            lax.fori_loop(2, NS - 1, steady, 0)
        return carry
    lax.fori_loop(0, 3, edge, 0)
    for c in range(8):
        store_out(1, c)
    cp_out(T - 1, 1).start()
    cp_out(T - 2, 0).wait()
    cp_out(T - 1, 1).wait()


@jax.jit
def pallas_interleave_layers__sliding_local_dilated__glu_gated_swiglu__prompt_kernel(
    A_x: jax.Array,
    A_wqkv: jax.Array,
    A_wo: jax.Array,
    B_x: jax.Array,
    B_w1: jax.Array,
    B_w3: jax.Array,
    B_w2: jax.Array,
):
    del B_x
    hbm = pl.BlockSpec(memory_space=pl.ANY)
    V = pltpu.VMEM
    out = pl.pallas_call(
        _kernel,
        in_specs=[hbm] * 6,
        out_specs=hbm,
        out_shape=jax.ShapeDtypeStruct((S, D), bf16),
        scratch_shapes=[
            V((3, D, D), bf16), V((D, D), bf16), V((NC, D, FC), bf16), V((NC, D, FC), bf16), V((F, D), bf16),
            V((4, 7, HD // 2, HD), u32), V((NC, 7, HD // 2, HF), u32), V((NC, 7, HD // 2, HF), u32),
            V((7, F // 4, HD), u32),
            V((3, TM, D), bf16), V((3, TM, D), bf16), V((2, NB + 1, 8 * GP, 128), f32), V((2, TM, D), f32),
            V((3, HALO + TM, D), f32), V((2, HALO, D), f32), V((2, HALO, D), f32),
            V((7, HM, HD), bf16), V((7, HM, HD), bf16), V((7, HM, HD), bf16), V((7, HM, F // 2), bf16),
            pltpu.SemaphoreType.DMA((4, 4)), pltpu.SemaphoreType.DMA((3, NC)), pltpu.SemaphoreType.DMA((2, 2)),
        ],
        compiler_params=pltpu.CompilerParams(vmem_limit_bytes=120 * 1024 * 1024),
    )(A_x.reshape(S, D), A_wqkv, A_wo, B_w1, B_w3, B_w2)
    return out.reshape(1, S, D)
```

```python
import functools

import jax
import jax.numpy as jnp
from jax import lax
import jax.experimental.pallas as pl
import jax.experimental.pallas.tpu as pltpu

S, D, DH, WIN, DIL, F = 2048, 1024, 32, 8, 2, 3584
NB = D // 128
SH = 8 * DIL
HALO = (WIN - 1) * SH
TM = 128
G = TM // 8
GP = G + 1
T = S // TM
NS = 2 * T + 1
FC = 512
NC = F // FC
HM, HD, HF = TM // 2, D // 2, FC // 2
PR = 16
f32, bf16, u32 = jnp.float32, jnp.bfloat16, jnp.uint32


def _dot(a, b):
    return jnp.dot(a, b, preferred_element_type=f32)


def _pack(v):
    return pltpu.bitcast(v.astype(bf16), u32)


def _pdot(a, b):
    return _dot(a, pltpu.bitcast(b, bf16))


def _ln(x):
    xc = x - jnp.mean(x, axis=-1, keepdims=True)
    return xc * lax.rsqrt(jnp.mean(xc * xc, axis=-1, keepdims=True) + 1e-5)


def _silu(g):
    hg = 0.5 * g
    return hg + hg * jnp.tanh(hg)


def _tree(t):
    while len(t) > 1:
        t = [t[j] + t[j + 1] for j in range(0, len(t), 2)]
    return t[0]


def _a_terms(a11, a12, a21, a22):
    return (a11 + a22, a21 + a22, a11, a22, a11 + a12, a21 - a11, a12 - a22)


def _b_terms(b11, b12, b21, b22):
    return (b11 + b22, b11, b12 - b22, b21 - b11, b22, b11 + b12, b21 + b22)


def _strassen(prod, emit=lambda i, j, v: v):
    m1 = prod(0)
    m2 = prod(1)
    t22 = m1 - m2
    m4 = prod(3)
    c21 = emit(1, 0, m2 + m4)
    t11 = m1 + m4 + prod(6)
    m5 = prod(4)
    c11 = emit(0, 0, t11 - m5)
    m3 = prod(2)
    c12 = emit(0, 1, m3 + m5)
    c22 = emit(1, 1, t22 + m3 + prod(5))
    return c11, c12, c21, c22


def _same(v):
    return v


def _dst(src, i):
    g = (src >> 2) & 7
    return (src & 3) * 32 + (g ^ i) * 4 + (src >> 5)


def _butterfly(blocks, g):
    for b in range(3):
        m = ((g >> b) & 1) == 1
        blocks = [jnp.where(m, blocks[j ^ (1 << b)], blocks[j]) for j in range(NB)]
    return blocks


def _prep_proj(src, dst, perm_mats, it):
    c = lax.broadcasted_iota(jnp.int32, (128, 128), 1)
    top, bot = (pl.ds(pl.multiple_of(h + it * 128, 128), 128) for h in (0, HD))
    blocks = [pltpu.bitcast(jnp.concatenate([src[top, 128 * b:128 * (b + 1)], src[bot, 128 * b:128 * (b + 1)]], axis=0), u32)
              for b in range(NB)]
    blocks = _butterfly(blocks, (c >> 2) & 7)

    def perm(i):
        return _dot(pltpu.bitcast(blocks[i], bf16), perm_mats[0, i])

    rows = pl.ds(pl.multiple_of(it * 64, 64), 64)
    for i in range(NB // 2):
        lo, hi = perm(i), perm(i + NB // 2)
        for t, v in enumerate(_b_terms(lo[:128], hi[:128], lo[128:], hi[128:])):
            dst[t, rows, 128 * i:128 * (i + 1)] = _pack(v)


def _prep_out(src, dst, perm_mats, it):
    left, right = (pl.ds(pl.multiple_of(h + it * 128, 128), 128) for h in (0, HD))
    blocks = [pltpu.bitcast(jnp.concatenate([src[128 * b:128 * (b + 1), left], src[128 * b:128 * (b + 1), right]], axis=1), u32)
              for b in range(NB)]
    blocks = _butterfly(blocks, (lax.broadcasted_iota(jnp.int32, (64, 256), 0) >> 1) & 7)

    def perm(i):
        return _dot(perm_mats[1, i], pltpu.bitcast(blocks[i], bf16))

    for i in range(NB // 2):
        up, dn = perm(i), perm(i + NB // 2)
        for t, v in enumerate(_b_terms(up[:, :128], up[:, 128:], dn[:, :128], dn[:, 128:])):
            dst[t, 64 * i:64 * (i + 1), left] = _pack(v)


def _prep_strip(get, put):
    blk = [get(i, j) for i in range(2) for j in range(2)]
    terms = _b_terms(*[v.astype(f32) for v in blk])
    for t in range(7):
        put(t, _pack(blk[0] if t == 1 else blk[3] if t == 4 else terms[t]))


def _roll_in_groups(x):
    n = x.shape[0] // 8
    return pltpu.roll(x.reshape(n, 8, x.shape[1]), 1, 1).reshape(x.shape)


def _kernel(x_h, wqkv_h, wo_h, w1_h, w3_h, w2_h, out_h,
            wqkv_r, wo_r, w1_r, w3_r, w2_r, wa_c, w1_c, w3_c, w2_c, perm_mats,
            x_buf, o_buf, pbuf, qbuf, qkv, hk, hv, x1c, x2c, oc, hc,
            sem_a, sem_f, sem_io):

    def cp_qkv(j, it):
        cols = pl.ds(pl.multiple_of(j * D, D), D)
        rows = [pl.ds(pl.multiple_of(h + it * 128, 128), 128) for h in (0, HD)]
        return [pltpu.make_async_copy(wqkv_h.at[r, cols], wqkv_r.at[j, r], sem_a.at[j, it]) for r in rows]

    def start_qkv(j):
        for it in range(4):
            for cp in cp_qkv(j, it):
                cp.start()

    cp_wo = pltpu.make_async_copy(wo_h, wo_r, sem_a.at[3, 0])

    def cp_ffn(c):
        cols = pl.ds(pl.multiple_of(c * FC, FC), FC)
        return (pltpu.make_async_copy(w1_h.at[:, cols], w1_r.at[c], sem_f.at[0, c]),
                pltpu.make_async_copy(w3_h.at[:, cols], w3_r.at[c], sem_f.at[1, c]),
                pltpu.make_async_copy(w2_h.at[cols, :], w2_r.at[cols, :], sem_f.at[2, c]))

    def start_ffn(c):
        for cp in cp_ffn(c):
            cp.start()

    def cp_x(t, buf):
        return pltpu.make_async_copy(x_h.at[pl.ds(pl.multiple_of(t * TM, TM), TM), :], x_buf.at[buf], sem_io.at[0, buf])

    def cp_out(t, buf):
        return pltpu.make_async_copy(o_buf.at[buf], out_h.at[pl.ds(pl.multiple_of(t * TM, TM), TM), :], sem_io.at[1, buf])

    def next_tiles(p):
        return cp_x(2 * p + 2, 1), cp_x(2 * p + 3, 0)

    def load_x(buf, c):
        for i in range(NB):
            pbuf[1, i, GP * c:GP * c + G, :] = x_buf[buf, G * c:G * (c + 1), 128 * i:128 * (i + 1)].astype(f32)

    def store_out(buf, c):
        for i in range(NB):
            o_buf[buf, G * c:G * (c + 1), 128 * i:128 * (i + 1)] = pbuf[0, i, GP * c:GP * c + G, :].astype(bf16)

    def prep_ffn(c):
        for w, wc in ((w1_r, w1_c), (w3_r, w3_c)):
            for r in range(0, HD, PR):
                def put(t, v):
                    wc[c, t, r // 2:(r + PR) // 2, :] = v
                _prep_strip(lambda a, b: w[c, HD * a + r:HD * a + r + PR, HF * b:HF * (b + 1)], put)
        for r in range(0, HF, PR):
            def put(t, v):
                w2_c[t, pl.ds(pl.multiple_of(c * (HF // 2) + r // 2, PR // 2), PR // 2), :] = v
            _prep_strip(lambda a, b: w2_r[pl.ds(pl.multiple_of(c * FC + HF * a + r, PR), PR), HD * b:HD * (b + 1)], put)

    def in_rows(s, m):
        src = 1 - ((s >> 1) & 1)
        return jnp.concatenate(
            [jnp.concatenate([pbuf[src, i, pl.ds(m + k, 8, stride=GP), :] for i in range(NB)], axis=1) for k in range(2)],
            axis=0)

    def put_terms(dst, r, top, bot):
        for t, v in enumerate(_a_terms(top[:, :HD], top[:, HD:], bot[:, :HD], bot[:, HD:])):
            dst[t, r:r + 16, :] = v.astype(bf16)

    def ln1(s, m):
        top = _ln(in_rows(s, m))
        yield
        bot = _ln(in_rows(s, G // 2 + m))
        yield
        put_terms(x1c, 8 * m, top, bot)

    def proj(j, hook):
        def emit(a, b, v):
            qkv[j, HALO + HM * a:HALO + HM * (a + 1), HD * b:HD * (b + 1)] = v
        _strassen(lambda t: hook(_pdot(x1c[t], wa_c[j, t])), emit)

    def first_tile(s):
        return jnp.logical_or(s == 0, s == 2)

    def halo(s, j, r0, n):
        layer = (s >> 1) & 1
        hal = hk if j == 1 else hv
        cur = _roll_in_groups(qkv[j, TM + r0:TM + r0 + n, :])
        prev = hal[layer, r0:r0 + n, :]
        if j == 2:
            prev = jnp.where(first_tile(s), jnp.broadcast_to(qkv[j, HALO:HALO + 1, :], (n, D)), prev)
        chunk0 = (lax.broadcasted_iota(jnp.int32, (n, D), 0) & 7) == 0
        qkv[j, r0:r0 + n, :] = jnp.where(chunk0, prev, cur)
        hal[layer, r0:r0 + n, :] = cur

    def attend(s, r0, n, zero=None):
        def rows(w, z=0):
            b = HALO + r0 - SH * w + z
            return pl.ds(b if isinstance(b, int) else pl.multiple_of(b, 8), n)
        q = [qkv[0, rows(0), 128 * i:128 * (i + 1)] for i in range(NB)]
        logits = []
        for w in range(WIN):
            a = _tree([q[i] * qkv[1, rows(w), 128 * i:128 * (i + 1)] for i in range(NB)])
            if zero is not None and w % 4 == 1:
                qkv[0, pl.ds(pl.multiple_of(zero, 8), n), 0:128] = a
            a = a + pltpu.roll(a, 64, 1)
            a = a + pltpu.roll(a, 32, 1)
            a = a * DH ** -0.5
            if w > 0 and (not isinstance(r0, int) or r0 < SH * w):
                row = lax.broadcasted_iota(jnp.int32, (n, 128), 0) + r0
                masked = jnp.logical_and(jnp.logical_and(row < SH * w, (row & 7) == 0), first_tile(s))
                a = jnp.where(masked, -1e9, a)
            logits.append(a)
            if w == WIN // 2 - 1:
                yield
        yield
        mx = functools.reduce(jnp.maximum, logits)
        e = [jnp.exp(a - mx) for a in logits]
        inv = 1.0 / _tree(e)
        p = [a * inv for a in e]
        yield
        for i in range(NB):
            if i == NB // 2:
                yield
            cols = slice(128 * i, 128 * (i + 1))
            o = _tree([p[w] * qkv[2, rows(w), cols] for w in range(WIN)])
            qkv[0, rows(0, zero if zero is not None and i % 2 == 1 else 0), cols] = o

    def o_terms(r):
        put_terms(oc, r, qkv[0, HALO + r:HALO + r + 16, :], qkv[0, HALO + HM + r:HALO + HM + r + 16, :])

    def out_proj_ln2(s):
        c11, c12, c21, c22 = _strassen(lambda t: _pdot(oc[t], wa_c[3, t]))
        for m in range(0, G // 2, 2):
            r = slice(8 * m, 8 * m + 16)
            top = in_rows(s, m) + jnp.concatenate([c11[r], c12[r]], axis=1)
            bot = in_rows(s, G // 2 + m) + jnp.concatenate([c21[r], c22[r]], axis=1)
            qbuf[s & 1, r, :] = top
            qbuf[s & 1, HM + 8 * m:HM + 8 * m + 16, :] = bot
            put_terms(x2c, 8 * m, _ln(top), _ln(bot))

    def gate_up(c, hook):
        cols = pl.ds(HF * c if isinstance(c, int) else pl.multiple_of(HF * c, HF), HF)
        g11, g12, g21, g22 = _strassen(lambda t: hook(_pdot(x2c[t], w1_c[c, t])), lambda i, j, v: _silu(v))
        act, h = ((g11, g12), (g21, g22)), {}

        def emit(i, j, v):
            h[i, j] = act[i][j] * v
            ready = {(1, 0): {},
                     (0, 0): {2: lambda: h[0, 0], 5: lambda: h[1, 0] - h[0, 0]},
                     (0, 1): {4: lambda: h[0, 0] + h[0, 1]},
                     (1, 1): {0: lambda: h[0, 0] + h[1, 1], 1: lambda: h[1, 0] + h[1, 1],
                              3: lambda: h[1, 1], 6: lambda: h[0, 1] - h[1, 1]}}[i, j]
            for t, term in ready.items():
                hc[t, :, cols] = term().astype(bf16)
        _strassen(lambda t: hook(_pdot(x2c[t], w3_c[c, t])), emit)

    def down(s, hook):
        def emit(a, b, v):
            for m in range(G // 2):
                r = HM * a + 8 * m
                x2 = qbuf[1 - (s & 1), r:r + 8, HD * b:HD * (b + 1)] + v[8 * m:8 * m + 8, :]
                for i in range(NB // 2):
                    pbuf[0, NB // 2 * b + i, pl.ds(r // 8, 8, stride=GP), :] = x2[:, 128 * i:128 * (i + 1)]
        _strassen(lambda t: hook(_pdot(hc[t], w2_c[t])), emit)

    def att_head(s):
        cp_x(s, s).wait()
        for c in range(8):
            load_x(s, c)

        @pl.when(s == 1)
        def _():
            for cp in next_tiles(0):
                cp.start()
            start_ffn(5)
        for m in range(0, G // 2, 2):
            list(ln1(s, m))

        def body(j, carry):
            @pl.when(s == 0)
            def _():
                def strip(it, carry):
                    for cp in cp_qkv(j, it):
                        cp.wait()
                    n = 4 * j + it
                    pl.when(jnp.logical_or(n == 0, n == 3))(lambda: start_qkv((n + 5) >> 2))
                    pl.when(n == 5)(lambda: cp_wo.start())
                    pl.when(jnp.logical_and(n >= 7, (n & 1) == 1))(lambda: start_ffn((n - 7) >> 1))
                    _prep_proj(wqkv_r.at[j], wa_c.at[j], perm_mats, it)
                    return carry
                lax.fori_loop(0, 4, strip, 0)
            proj(j, _same)
            return carry
        lax.fori_loop(0, 3, body, 0)
        pl.when(s == 1)(lambda: start_ffn(6))
        halo(s, 1, 0, HALO)
        halo(s, 2, 0, HALO)
        lax.fori_loop(0, TM // 32, lambda j, c: (list(attend(s, j * 32, 32)), c)[1], 0)

        @pl.when(s == 0)
        def _():
            cp_wo.wait()
            start_ffn(3)
            lax.fori_loop(0, 4, lambda it, c: (_prep_out(wo_r, wa_c.at[3], perm_mats, it), c)[1], 0)
            start_ffn(4)

    def att_tail(s):
        for r in range(0, HM, 16):
            o_terms(r)
        out_proj_ln2(s)

    def ffn_head(s):
        def body(c, carry):
            @pl.when(s == 1)
            def _():
                for cp in cp_ffn(c):
                    cp.wait()
                prep_ffn(c)
            gate_up(c, _same)
            return carry
        lax.fori_loop(0, NC, body, 0)

    def steady(s, carry):
        zero = (s >> 10) * 8

        def after(buf, jobs):
            jobs = list(jobs)

            def hook(val):
                if jobs:
                    tail = val[:8, :128]
                    if buf is pbuf:
                        pbuf[0, NB, pl.ds(pl.multiple_of(zero, 8), 8), :] = tail
                    else:
                        qkv[0, pl.ds(pl.multiple_of(zero, 8), 8), 0:128] = tail
                    jobs.pop(0)()
                return val
            return hook, jobs

        P = functools.partial
        phase = s & 3
        o_sel = jnp.where(phase < 2, phase, 2)
        x_sel = jnp.where(jnp.logical_and(jnp.logical_or(phase == 3, phase == 0), s < NS - 2), s & 1, 2)

        def pairs(fn, buf):
            return [P(lambda c: (fn(buf, c), fn(buf, c + 1)), c) for c in range(0, 8, 2)]

        att = []
        for r in range(0, HM, 16):
            for r0 in (r, r + 8, HM + r, HM + r + 8):
                att += [P(next, attend(s, r0, 8, zero), None)] * 5
            att += [P(o_terms, r)]
        plan = [after(pbuf, [P(next, g, None) for g in [ln1(s, m) for m in range(0, G // 2, 2)] for _ in range(3)]),
                after(pbuf, pairs(store_out, o_sel)),
                after(qkv, [P(halo, s, 1, r, SH) for r in range(0, HALO, SH)]),
                after(qkv, [P(halo, s, 2, r, SH) for r in range(0, HALO, SH)]),
                after(qkv, att),
                after(pbuf, pairs(load_x, x_sel))]
        gate_up(0, plan[0][0])
        assert not plan[0][1]
        for k, j in enumerate((1, 2, 0)):
            proj(j, plan[1 + k][0])
            assert not plan[1 + k][1]
        for c in range(1, NC):
            gate_up(c, plan[4][0])
        assert not plan[4][1]
        out_proj_ln2(s)
        down(s, plan[5][0])
        assert not plan[5][1]

        tile = (s >> 1) - 2 + (s & 1)
        pl.when(phase < 2)(lambda: cp_out(tile, phase).start())
        pl.when(jnp.logical_and(phase >= 2, s > 4))(lambda: cp_out(tile - 1, phase - 2).wait())

        @pl.when(jnp.logical_and(phase == 1, s < NS - 4))
        def _():
            for cp in next_tiles(s >> 2):
                cp.start()

        @pl.when(jnp.logical_and(phase == 2, s < NS - 3))
        def _():
            for cp in next_tiles(s >> 2):
                cp.wait()
        return carry

    cp_x(0, 0).start()
    start_qkv(0)
    cp_x(1, 1).start()
    x_buf[2] = jnp.zeros((TM, D), bf16)
    row, col = (lax.broadcasted_iota(jnp.int32, (128, 128), a) for a in range(2))
    for i in range(NB):
        perm_mats[0, i] = jnp.where(col == _dst(row, i), 1.0, 0.0).astype(bf16)
        perm_mats[1, i] = jnp.where(row == _dst(col, i), 1.0, 0.0).astype(bf16)
    hk[...] = jnp.zeros(hk.shape, f32)
    hv[...] = jnp.zeros(hv.shape, f32)

    def edge(p, carry):
        s = jnp.where(p == 2, NS - 1, p)
        pl.when(p < 2)(lambda: att_head(s))

        @pl.when(p == 2)
        def _():
            for c in range(8):
                store_out(0, c)
            cp_out(T - 2, 0).start()
        pl.when(p > 0)(lambda: ffn_head(s))
        pl.when(p < 2)(lambda: att_tail(s))
        pl.when(p > 0)(lambda: down(s, _same))

        @pl.when(p == 1)
        def _():
            lax.fori_loop(2, NS - 1, steady, 0)
        return carry
    lax.fori_loop(0, 3, edge, 0)
    for c in range(8):
        store_out(1, c)
    cp_out(T - 1, 1).start()
    cp_out(T - 2, 0).wait()
    cp_out(T - 1, 1).wait()


@jax.jit
def pallas_interleave_layers__sliding_local_dilated__glu_gated_swiglu__prompt_kernel(
    A_x: jax.Array,
    A_wqkv: jax.Array,
    A_wo: jax.Array,
    B_x: jax.Array,
    B_w1: jax.Array,
    B_w3: jax.Array,
    B_w2: jax.Array,
):
    del B_x
    hbm = pl.BlockSpec(memory_space=pl.ANY)
    V = pltpu.VMEM
    out = pl.pallas_call(
        _kernel,
        in_specs=[hbm] * 6,
        out_specs=hbm,
        out_shape=jax.ShapeDtypeStruct((S, D), bf16),
        scratch_shapes=[
            V((3, D, D), bf16), V((D, D), bf16), V((NC, D, FC), bf16), V((NC, D, FC), bf16), V((F, D), bf16),
            V((4, 7, HD // 2, HD), u32), V((NC, 7, HD // 2, HF), u32), V((NC, 7, HD // 2, HF), u32),
            V((7, F // 4, HD), u32), V((2, NB, 128, 128), bf16),
            V((3, TM, D), bf16), V((3, TM, D), bf16), V((2, NB + 1, 8 * GP, 128), f32), V((2, TM, D), f32),
            V((3, HALO + TM, D), f32), V((2, HALO, D), f32), V((2, HALO, D), f32),
            V((7, HM, HD), bf16), V((7, HM, HD), bf16), V((7, HM, HD), bf16), V((7, HM, F // 2), bf16),
            pltpu.SemaphoreType.DMA((4, 4)), pltpu.SemaphoreType.DMA((3, NC)), pltpu.SemaphoreType.DMA((2, 2)),
        ],
        compiler_params=pltpu.CompilerParams(vmem_limit_bytes=120 * 1024 * 1024),
    )(A_x.reshape(S, D), A_wqkv, A_wo, B_w1, B_w3, B_w2)
    return out.reshape(1, S, D)
```
